```python
import jax
import jax.numpy as jnp

def _softmax(x, axis=-1):
    return jax.nn.softmax(x, axis=axis)

def _gelu(x):
    return jax.nn.gelu(x, approximate=True)

def _silu(x):
    return jax.nn.silu(x)

def _sigmoid(x):
    return jax.nn.sigmoid(x)

def _layernorm(x, axis=-1, eps=1e-05):
    m = jnp.mean(x, axis=axis, keepdims=True)
    v = jnp.var(x, axis=axis, keepdims=True)
    return (x - m) / jnp.sqrt(v + eps)

def _scatter_add(tgt, idx, src, axis=0):
    return tgt.at[idx].add(src)

def _segment_sum(src, seg, n):
    return jax.ops.segment_sum(src, seg, n)

class _Rng:

    def __init__(self, key):
        self._k = key

    def _next(self):
        self._k, sub = jax.random.split(self._k)
        return sub

    def normal(self, shape):
        return jax.random.normal(self._next(), shape, dtype=jnp.bfloat16)

    def randint(self, lo, hi, shape):
        return jax.random.randint(self._next(), shape, lo, hi, dtype=jnp.int32)

    def uniform(self, shape, lo=0.0, hi=1.0):
        return jax.random.uniform(self._next(), shape, jnp.bfloat16, lo, hi)

    def permutation(self, n):
        return jax.random.permutation(self._next(), n)
kernel_name = 'sequential_preLN__memory_aug_recurrent_mem_tr__mixer_s_mlp__prompt'

def setup_inputs():
    _rng = _Rng(jax.random.key(int.from_bytes(__import__("os").urandom(4), "little")))
    _w = lambda a: (lambda t: t.astype(jnp.bfloat16) if jnp.issubdtype(t.dtype, jnp.floating) else t)(jnp.asarray(a))

    def _A_setup():
        B, S, Dm = (1, 2048, 1024)
        H, Dh = (32, 128)
        M, seg = (8, 32)
        seg = min(seg, S)
        S = S // seg * seg
        return {'x': _w((lambda *s: _rng.normal(s) * 0.05)(B, S, Dm)), 'mem0': _w((lambda *s: _rng.normal(s) * 0.05)(B, M, Dm)), 'Wq': _w((lambda *s: _rng.normal(s) * 0.05)(Dm, H, Dh) * Dm ** (-0.5)), 'Wk': _w((lambda *s: _rng.normal(s) * 0.05)(Dm, H, Dh) * Dm ** (-0.5)), 'Wv': _w((lambda *s: _rng.normal(s) * 0.05)(Dm, H, Dh) * Dm ** (-0.5)), 'Wo': _w((lambda *s: _rng.normal(s) * 0.05)(H, Dh, Dm) * (H * Dh) ** (-0.5)), 'seg_len': seg}
    _A_in = _A_setup()

    def _B_setup():
        B, S, D, F = (1, 2048, 1024, 3584)
        return {'x': _w((lambda *s: _rng.normal(s) * 0.05)(B, S, D)), 'w1': _w((lambda *s: _rng.normal(s) * 0.05)(D, D) * D ** (-0.5)), 'w2': _w((lambda *s: _rng.normal(s) * 0.05)(D, D) * D ** (-0.5)), 'w3': _w((lambda *s: _rng.normal(s) * 0.05)(D, F) * D ** (-0.5)), 'w4': _w((lambda *s: _rng.normal(s) * 0.05)(F, D) * F ** (-0.5))}
    _B_in = _B_setup()
    return {'A_x': _A_in['x'], 'A_mem0': _A_in['mem0'], 'A_Wq': _A_in['Wq'], 'A_Wk': _A_in['Wk'], 'A_Wv': _A_in['Wv'], 'A_Wo': _A_in['Wo'], 'A_seg_len': _A_in['seg_len'], 'B_x': _B_in['x'], 'B_w1': _B_in['w1'], 'B_w2': _B_in['w2'], 'B_w3': _B_in['w3'], 'B_w4': _B_in['w4']}

def reference(A_x, A_mem0, A_Wq, A_Wk, A_Wv, A_Wo, A_seg_len, B_x, B_w1, B_w2, B_w3, B_w4):

    def _A_ref(x, mem0, Wq, Wk, Wv, Wo, seg_len):
        B, S, Dm = x.shape
        H, Dh = (Wq.shape[1], Wq.shape[2])
        M = mem0.shape[1]
        scale = Dh ** (-0.5)
        n_seg = S // seg_len
        L = M + seg_len
        idx = jnp.arange(L)
        mask = (idx[:, None] < M) | (idx[:, None] >= idx[None, :])
        mem = mem0
        outs = []
        for s in range(n_seg):
            xs = x[:, s * seg_len:(s + 1) * seg_len, :].copy()
            h = jnp.concatenate([mem, xs], axis=1)
            q = jnp.einsum('btd,dhe->bhte', h, Wq)
            k = jnp.einsum('btd,dhe->bhte', h, Wk)
            v = jnp.einsum('btd,dhe->bhte', h, Wv)
            scores = jnp.einsum('bhqe,bhke->bhqk', q, k) * scale
            scores = jnp.where(mask[None, None], scores, -1000000000.0)
            p = _softmax(scores, axis=-1)
            o = jnp.einsum('bhqk,bhke->bhqe', p, v)
            o = jnp.einsum('bhte,hed->btd', o, Wo)
            mem = o[:, :M, :].copy()
            outs.append(o[:, M:, :])
        return jnp.concatenate(outs, axis=1)

    def _B_ref(x, w1, w2, w3, w4):
        B, S, D = x.shape
        h = _gelu(_layernorm(x, axis=-1) @ w1)
        c = D // 4
        g0 = jnp.pad(h[:, :, 0 * c:1 * c], ((0, 0), (1, 0), (0, 0)))[:, :S, :]
        g1 = jnp.pad(h[:, :, 1 * c:2 * c], ((0, 0), (0, 1), (0, 0)))[:, 1:, :]
        g2 = jnp.pad(h[:, :, 2 * c:3 * c], ((0, 0), (2, 0), (0, 0)))[:, :S, :]
        g3 = jnp.pad(h[:, :, 3 * c:], ((0, 0), (0, 2), (0, 0)))[:, 2:, :]
        hs = jnp.concatenate([g0, g1, g2, g3], axis=-1) @ w2
        x1 = x + hs
        h2 = _gelu(_layernorm(x1, axis=-1) @ w3) @ w4
        return x1 + h2
    x = A_x
    h = x + _A_ref(_layernorm(x, axis=-1), A_mem0, A_Wq, A_Wk, A_Wv, A_Wo, A_seg_len)
    h2 = h + _B_ref(_layernorm(h, axis=-1), B_w1, B_w2, B_w3, B_w4)
    return h2
```

```python
import functools

import jax
import jax.numpy as jnp
from jax import lax
import jax.experimental.pallas as pl
import jax.experimental.pallas.tpu as pltpu

S = 2048
D = 1024
H = 32
DH = 128
MEM = 8
SEG = 32
F = 3584
NSEG = S // SEG
L = MEM + SEG
TOK = 24
P0 = S - TOK * NSEG
RING = 576
X0 = P0 + 128
C4 = D // 4
SHIFT = (-1, 1, -2, 2)
HALO = 8
RB = 256
R4 = RB // 4
NC = F // 512
NP = 49
EPS = 1e-5
NEG = -1000000000.0

LAG_QK, LAG_PV, LAG_WO = 2, 4, 6
FILL_AT = 18
UNROLL = 2
ENC = 5
SIDE_AT = 2
SIDE_N = 48
LN_ROWS = 16
NSPLIT = 14
KSPLIT = 4
POST_C = (0, 2, 4)
PRO_AT = 2
PRO_K = 4
POST_N = 33
POST_LAG = 6
POST_ROWS = 8
W4_SPLIT = (4, 4, 4, 0, 0, 4, 4, 4, 22)
W4_AT = 3

bf16 = jnp.bfloat16
f32 = jnp.float32
u32 = jnp.uint32

SEM_X0, SEM_X, SEM_W1, SEM_W23, SEM_W4, SEM_WO, SEM_OUT, SEM_W = 0, 1, 2, 3, 4, 5, 9, 17
NSEM = SEM_W + 12

SA = (((0, 0), 1, (1, 1)), ((1, 0), 1, (1, 1)), ((0, 0),), ((1, 1),),
      ((0, 0), 1, (0, 1)), ((1, 0), -1, (0, 0)), ((0, 1), -1, (1, 1)))
SB = (((0, 0), 1, (1, 1)), ((0, 0),), ((0, 1), -1, (1, 1)), ((1, 0), -1, (0, 0)),
      ((1, 1),), ((0, 0), 1, (0, 1)), ((1, 0), 1, (1, 1)))
SC = ((((0, 0), 1), ((1, 1), 1)), (((1, 0), 1), ((1, 1), -1)),
      (((0, 1), 1), ((1, 1), 1)), (((0, 0), 1), ((1, 0), 1)),
      (((0, 0), -1), ((0, 1), 1)), (((1, 1), 1),), (((0, 0), 1),))
ORDER_A = (2, 3, 0, 4, 6, 1, 5)
ORDER_B = (1, 4, 0, 2, 5, 3, 6)
QUAD = ((0, 0), (0, 1), (1, 0), (1, 1))


def _mult(i, n):
    return i if isinstance(i, int) else pl.multiple_of(i, n)


def _ln(x):
    m = jnp.mean(x, axis=-1, keepdims=True)
    d = x - m
    v = jnp.mean(d * d, axis=-1, keepdims=True)
    return d * lax.rsqrt(v + EPS)


def _gelu(x):
    c = 0.7978845608028654
    half = 0.5 * x
    return half * jnp.tanh(x * (c + c * 0.044715 * (x * x))) + half


def _pack(x):
    return pltpu.bitcast(x.astype(bf16), u32)


def _unpack(x):
    return pltpu.bitcast(x, bf16)


def _dot(a, b):
    return jnp.dot(a, b, preferred_element_type=f32)


def _zip(even, odd):
    return pltpu.bitcast(pltpu.pack_elementwise([even, odd], packed_dtype=bf16), u32)


def _unzip(w, k):
    return pltpu.unpack_elementwise(w, index=k, packed_dtype=bf16, unpacked_dtype=f32)


def _combine(get, term):
    if len(term) == 1:
        return get(*term[0])
    a, b = get(*term[0]), get(*term[2])
    return a + b if term[1] > 0 else a - b


def _encode7(tab, p, get):
    outer = [{(i, j): _combine(lambda a, b: get(k, 2 * a + i, 2 * b + j), tab[p])
              for i, j in QUAD} for k in range(2)]
    return [_zip(*[_combine(lambda a, b: o[a, b], tab[r]) for o in outer])
            for r in range(7)]


def _encode(tab, get):
    get = functools.cache(get)
    ops = {p: _encode7(tab, p, get) for p in (ORDER_A if tab is SA else ORDER_B)}
    return [w for p in range(7) for w in ops[p]]


def _accumulate(acc, key, sign, v):
    if key not in acc:
        acc[key] = v
    else:
        acc[key] = acc[key] + v if sign > 0 else acc[key] - v


def _decode7(p, prods, out):
    inner = {}
    for r in range(7):
        for key, sign in SC[r]:
            _accumulate(inner, key, sign, prods[r])
    for (a, b), sign in SC[p]:
        for (i, j), v in inner.items():
            _accumulate(out, (2 * a + i, 2 * b + j), sign, v)


def _decode(prods, r0):
    out = {}
    for p in range(7):
        _decode7(p, [pltpu.bitcast(m[r0:r0 + 8, :], f32) for m in prods[7 * p:7 * p + 7]],
                 out)
    return out


def _rows(ref, rows):
    return jnp.concatenate([ref[c, rows, :] for c in range(ref.shape[0])], axis=1)


def _set_rows(ref, rows, v):
    for c in range(ref.shape[0]):
        ref[c, rows, :] = v[:, c * 128:(c + 1) * 128]


class _Side:
    def __init__(self, zero, slots, *jobs):
        self.zero = zero
        self.slots = slots
        self.jobs = [[job, count, 0] for job, count in jobs]
        self.at = 0

    def tie(self, w, r0=0, c0=0):
        self.at += 1
        head = old = w[r0:r0 + 8, c0:c0 + 128]
        for job in self.jobs:
            while job[2] * self.slots < min(self.at, self.slots) * job[1]:
                job[2] += 1
                for ref, idx in next(job[0]):
                    row = pl.ds(pl.multiple_of(idx[-1] + 8 * self.zero, 8), 8)
                    seen = ref[idx[:-1] + (row, pl.ds(0, 128))]
                    head = jnp.where(self.zero == 0, head, pltpu.bitcast(seen, u32))
        if head is old:
            return w
        row = [v for v in (w[r0:r0 + 8, :c0] if c0 else None, head,
                           w[r0:r0 + 8, c0 + 128:] if c0 + 128 < w.shape[1] else None)
               if v is not None]
        rows = (w[:r0] if r0 else None, jnp.concatenate(row, axis=1),
                w[r0 + 8:] if r0 + 8 < w.shape[0] else None)
        return jnp.concatenate([v for v in rows if v is not None], axis=0)

    def after(self, ref, r):
        spare = pl.multiple_of(ref.shape[-2] - 8 - 8 * self.zero, 8)
        lead = tuple(n - 1 - self.zero for n in ref.shape[:-2])
        ref[lead + (pl.ds(spare, 8), pl.ds(0, 128))] = pltpu.bitcast(r[:8, :128], ref.dtype)

    def finish(self):
        for job in self.jobs:
            for _ in job[0]:
                pass


def _kernel(x_hbm, mem0_ref, wq_hbm, wk_hbm, wv_hbm, wo_hbm, w1_hbm, w2_hbm,
            w3_hbm, w4_hbm, out_hbm,
            wo_b, xs, hbuf, xg, w1b, we, sems, *q_rings):
    w_hbm = (wq_hbm, wk_hbm, wv_hbm)
    q_r = [q_rings[h % 8].at[h // 8] for h in range(H)]

    x0_copy = pltpu.make_async_copy(x_hbm.at[pl.ds(0, X0)], xs.at[pl.ds(0, X0)],
                                    sems.at[SEM_X0])
    x_copy = pltpu.make_async_copy(x_hbm.at[pl.ds(X0, S - X0)], xs.at[pl.ds(X0, S - X0)],
                                   sems.at[SEM_X])

    def wo_copy(i):
        rows = pl.ds(_mult(i * 512, 512), 512)
        return pltpu.make_async_copy(wo_hbm.bitcast(u32).at[rows], wo_b.at[rows],
                                     sems.at[SEM_WO + i])

    def w1_copy(i):
        cols = pl.ds(_mult(i * C4, C4), C4)
        return pltpu.make_async_copy(w1_hbm.bitcast(u32).at[:, cols], w1b.at[i],
                                     sems.at[SEM_W1])

    def w23_copies(c):
        src, first, step = (w3_hbm, 4 * c, 1) if c < NC else (w2_hbm, c - NC, 2)
        return [pltpu.make_async_copy(
            src.bitcast(u32).at[:, pl.ds((first + step * b) * 128, 128)],
            we.at[c, pl.ds(b * 512, 512)], sems.at[SEM_W23]) for b in range(4)]

    def out_copy(i):
        rows = pl.ds(_mult(i * RB, RB), RB)
        return pltpu.make_async_copy(xs.at[rows], out_hbm.at[rows], sems.at[SEM_OUT + i])

    def block_a(wq_s, wk_s, wv_s, ubuf, tokbuf, lnbuf, *kv_rings):
        w_s = (wq_s, wk_s, wv_s)
        rings = tuple(q_rings) + tuple(kv_rings)
        ring = [[rings[m * 8 + h % 8].at[h // 8] for h in range(H)] for m in range(3)]
        k_r, v_r = ring[1:]

        stg = [we.at[m, pl.ds(0, 4 * D)] for m in range(3)]
        xe = we.at[3]
        w_op = (hbuf, xg)

        def start_chunk(g, m):
            src = w_hbm[m].bitcast(u32)
            dst = stg[m].reshape(D // 2, 8, DH)
            for par in range(2):
                pltpu.make_async_copy(
                    src.at[:, pl.ds(_mult(16 * par + 4 * g, 4), 4), :],
                    dst.at[:, pl.ds(4 * par, 4), :],
                    sems.at[SEM_W + 3 * g + m]).start()

        def wait_chunk(g, m):
            pltpu.make_async_copy(stg[m], stg[m], sems.at[SEM_W + 3 * g + m]).wait()

        def encode_unit(g, m, half, slices):
            h0 = 8 * g + 4 * half
            for i0 in slices:
                blk = {}

                def get(k, a, b):
                    if (k, a, b) not in blk:
                        for par in range(2):
                            w = stg[m][pl.ds(8 * (128 * a + i0) + 4 * par + 2 * half + b // 2,
                                             8, stride=8), :]
                            for j in range(2):
                                blk[par, a, b - b % 2 + j] = _unzip(w, j)
                        for j in (b - b % 2, b - b % 2 + 1):
                            w_s[m][h0 + j, pl.ds(128 * a + i0, 8), :] = _zip(
                                blk[0, a, j], blk[1, a, j])
                    return blk[k, a, b]

                for p in ORDER_B:
                    known = len(blk)
                    for r, w in enumerate(_encode7(SB, p, get)):
                        q = 7 * p + r
                        if len(SB[p]) + len(SB[r]) > 2:
                            w_op[half][1 + q // 16, pl.ds(128 * (q % 16) + i0, 8), :] = (
                                pltpu.bitcast(w, f32))
                    yield [(w_op[half], (1, i0))] + [(w_s[m], (h0, i0))] * (len(blk) > known)

        def operand(g, m, half, q, zero):
            tp, tr = SB[q // 7], SB[q % 7]
            if len(tp) + len(tr) == 2:
                a, b = (2 * tp[0][n] + tr[0][n] for n in range(2))
                return w_s[m][8 * g + 4 * half + b, pl.ds(128 * a, 128), :]
            return w_op[half][1 + q // 16, pl.ds(
                pl.multiple_of(128 * (q % 16) + 8 * zero, 8), 128), :]

        def decode_unit(g, m, half, prods):
            for r0 in range(0, P0 // 4, 8):
                out = _decode(prods, r0)
                for i, j in QUAD:
                    for a, b in QUAD:
                        rings[8 * m + 4 * half + 2 * b + j][
                            g, pl.ds(P0 // 4 * (2 * a + i) + r0, 8), :] = out[2 * a + i, 2 * b + j]
                    yield [(rings[8 * m + 4 * half + 2 * b + j], (g, r0)) for b in range(2)]

        x0_copy.start()
        for m in range(3):
            start_chunk(0, m)
        x0_copy.wait()

        @pl.loop(0, P0 // 64)
        def _(s):
            for a in range(4):
                rows = pl.ds(pl.multiple_of(P0 // 4 * a + 16 * s, 16), 16)
                _set_rows(hbuf, rows, _ln(xs[rows, :].astype(f32)))
            for kt in range(2):
                ops = _encode(SA, lambda k, a, b: hbuf[
                    2 * b + kt, pl.ds(P0 // 4 * a + 16 * s + k, 8, stride=2), :])
                for p, w in enumerate(ops):
                    xe[pl.ds(pl.multiple_of(128 * p + 64 * kt + 8 * s, 8), 8), :] = w

        tokbuf[...] = _ln(xs[pl.ds(P0, UNROLL * TOK), :].astype(f32))
        wait_chunk(0, 0)

        @pl.loop(0, 16)
        def _(i):
            list(encode_unit(0, 0, 0, [pl.multiple_of(8 * i, 8)]))

        last = [we.at[4, pl.ds(128 * p, 128)] for p in range(NP)]

        @pl.loop(0, 4)
        def _(g):
            g1 = jnp.minimum(g + 1, 3)
            zero = g >> 2
            jobs = [(decode_unit((g + 3) & 3, 2, 1, last), 64)]
            for m in range(3):
                for half in range(2):
                    nxt = (g1, 0, 0) if (m, half) == (2, 1) else (g, m + half, 1 - half)
                    side = _Side(zero, (NP - PRO_AT - 1) * PRO_K,
                                 (encode_unit(*nxt, range(0, 128, 8)), 16 * 7), *jobs)
                    prods = []
                    for p in range(NP):
                        lhs = jnp.concatenate(
                            [xe[pl.ds(128 * p + 64 * kt, 64), :] for kt in range(2)], axis=1)
                        rhs = operand(g, m, half, p, zero)
                        if p > PRO_AT:
                            for k in range(PRO_K):
                                lhs = side.tie(lhs, 64 // PRO_K * k)
                        prods.append(_dot(_unpack(lhs), _unpack(rhs)))
                        if half == 1 and p == 1:
                            if m < 2:
                                wait_chunk(g, m + 1)
                            else:
                                pl.when(g < 3)(functools.partial(wait_chunk, g1, 0))
                            pl.when(g < 3)(functools.partial(start_chunk, g1, m))
                            if m == 0:
                                w1_copy(g).start()
                            if m == 1:
                                wo_copy(g).start()
                    jobs = [(decode_unit(g, m, half, prods), 64)]
            for p in range(NP):
                we[4, pl.ds(128 * p, 128), :] = pltpu.bitcast(prods[p], u32)

        list(decode_unit(3, 2, 1, last))

        x_copy.start()
        _set_rows(xg, pl.ds(0, HALO), jnp.zeros((HALO, D), f32))
        _set_rows(xg, pl.ds(HALO + S, HALO), jnp.zeros((HALO, D), f32))
        _set_rows(hbuf, pl.ds(0, UNROLL * TOK), jnp.zeros((UNROLL * TOK, D), f32))
        ubuf[...] = jnp.zeros(ubuf.shape, u32)
        for c in range(NC + 2):
            for cp in w23_copies(c):
                cp.start()
        for i in range(4):
            w1_copy(i).wait()
        for i in range(4):
            wo_copy(i).wait()

        def wrap(r):
            return jnp.where(r >= RING, r - RING, r)

        def step(s, carry, tok, side):
            mem, rp, ra, rw = carry
            ri = lax.broadcasted_iota(jnp.int32, (2 * MEM + SEG, 2 * L), 0)
            ci = lax.broadcasted_iota(jnp.int32, (2 * MEM + SEG, 2 * L), 1)
            key_b = ((ci >= MEM) & (ci < 2 * MEM)) | (ci >= 2 * MEM + SEG)
            same = key_b == ((ri >= MEM) & (ri < 2 * MEM))
            mask = same & ((ri < 2 * MEM) | (ri >= ci))
            fill = jnp.where(same, NEG, -jnp.inf)

            lhs = jnp.concatenate([mem, tok], axis=0).astype(bf16)
            rps = [pl.multiple_of(wrap(rp + 8 * i), 8) for i in range(3)]
            ra_ = pl.multiple_of(ra, SEG)
            rw_ = pl.multiple_of(rw, 8)

            col = s & 3
            group = jnp.maximum((s >> 2) - 1, 0)
            rb = pl.multiple_of(group * (4 * TOK), 8)

            def filler(j):
                u = ubuf[pl.ds(pl.multiple_of((group & 1) * (2 * TOK), 8), 2 * TOK), :]
                r = _dot(_unpack(u), _unpack(w1b[col, :, pl.ds(j * 128, 128)]))
                xg[2 * col + j, pl.ds(HALO + rb, 4 * TOK), :] = _gelu(r)

            mem_qkv = {}
            scores = {}
            o_mem = {}
            total = [None]

            def qkv(h):
                for m in range(3):
                    w = w_s[m][h]
                    r = _dot(lhs, _unpack(side.tie(w) if h >= SIDE_AT else w))
                    for i in range(3):
                        ring[m][h][pl.ds(rps[i], 8), :] = r[8 + 8 * i:16 + 8 * i]
                    mem_qkv[m, h] = r[:MEM]

            def segment(m, pair):
                a, b = 2 * pair, 2 * pair + 1
                ma, mb = mem_qkv.pop((m, a)), mem_qkv.pop((m, b))
                xa, xb = (ring[m][h][pl.ds(ra_, SEG), :] for h in (a, b))
                if m == 0:
                    parts = ((ma, mb, xa), (xb,))
                else:
                    parts = ((ma, mb, xa, xb), (mb, ma, xb))
                return [jnp.concatenate(v, axis=0).astype(bf16) for v in parts]

            def qk(pair):
                q, k = segment(0, pair), segment(1, pair)
                for n in (pair % 2, 1 - pair % 2):
                    scores[pair, n] = lax.dot_general(
                        q[n], k[n], (((1,), (1,)), ((), ())), preferred_element_type=f32)

            def pv(pair):
                v = segment(2, pair)
                for n in (pair % 2, 1 - pair % 2):
                    sc = scores.pop((pair, n)) * (DH ** -0.5)
                    if n == 0:
                        sc = jnp.where(mask, sc, fill)
                    else:
                        sc = jnp.where(mask[2 * MEM:, :2 * MEM + SEG], sc,
                                       fill[2 * MEM:, :2 * MEM + SEG])
                    mx = jnp.max(sc, axis=1, keepdims=True)
                    e = jnp.exp(sc - mx)
                    den = jnp.sum(e, axis=1, keepdims=True)
                    inv = pl.reciprocal(den, approx=True)
                    inv = inv * (2.0 - den * inv)
                    o = _dot(e.astype(bf16), v[n]) * inv
                    q_r[2 * pair + n][pl.ds(ra_, SEG), :] = o[-SEG:]
                    if n == 0:
                        o_mem[2 * pair], o_mem[2 * pair + 1] = o[:MEM], o[MEM:2 * MEM]

            def wo(h):
                lo = jnp.concatenate([o_mem.pop(h), q_r[h][pl.ds(rw_, TOK), :]],
                                     axis=0).astype(bf16)
                r = _dot(lo, _unpack(wo_b[pl.ds(h * DH // 2, DH // 2), :]))
                total[0] = r if total[0] is None else total[0] + r

            npair = H // 2
            for t in range(npair + LAG_WO):
                if 0 <= t - LAG_QK < npair:
                    qk(t - LAG_QK)
                if 0 <= t - LAG_PV < npair:
                    pv(t - LAG_PV)
                if t < npair:
                    qkv(2 * t)
                    qkv(2 * t + 1)
                if t == FILL_AT:
                    filler(0)
                if 0 <= t - LAG_WO < npair:
                    wo(2 * (t - LAG_WO))
                    wo(2 * (t - LAG_WO) + 1)
            filler(1)

            a = total[0]
            return (a[:MEM], wrap(rp + TOK), wrap(ra + SEG), wrap(rw + TOK)), a[MEM:]

        def steps(i, carry):
            n = UNROLL * TOK
            pl.when(i == 1)(x_copy.wait)

            @pl.when(i == 3)
            def _():
                for c in range(NC + 2):
                    for cp in w23_copies(c):
                        cp.wait()

            zero = i >> 5

            def norm_filler():
                prev = jnp.maximum(i - 1, 0)
                for r in range(0, n, LN_ROWS):
                    rows = pl.ds(pl.multiple_of(n * prev + r, 8), LN_ROWS)
                    lnbuf[pl.ds(r, LN_ROWS), :] = _ln(_rows(hbuf, rows))
                    yield [(lnbuf, (r,))]
                for r in range(0, n, LN_ROWS):
                    rows = pl.ds(pl.multiple_of(r + 16 * zero, 8), LN_ROWS)
                    dst = pl.multiple_of((n * (prev & 3) + r) // 2, 8)
                    ubuf[pl.ds(dst, LN_ROWS // 2), :] = _pack(_ln(lnbuf[rows, :]))
                    yield [(ubuf, (dst,))]

            def norm_tokens():
                nxt = jnp.minimum(P0 + n * (i + 1), S - n)
                for r in range(0, n, 16):
                    rows = pl.ds(pl.multiple_of(nxt + r, 16), 16)
                    tokbuf[pl.ds(r, 16), :] = _ln(xs[rows, :].astype(f32))
                    yield [(tokbuf, (r,))]

            def encode_w23():
                for k in range(ENC):
                    j = ENC * i + k
                    grp, i0 = jnp.where(j < 16, NC + 2, (j >> 4) - 1), 8 * (j & 15)
                    slot = lambda q: (grp, pl.ds(pl.multiple_of(128 * q + i0, 8), 8))
                    raw = {(a, b): we[slot(4 * b + a)] for a in range(4) for b in range(4)}
                    get = functools.cache(lambda k, a, b: _unzip(raw[a, b], k))
                    for p in ORDER_B:
                        for r, w in enumerate(_encode7(SB, p, get)):
                            we[slot(7 * p + r)] = w
                        yield [(we, (grp, i0))]

            jobs = [[(norm_filler(), 2 * n // LN_ROWS)],
                    [(encode_w23(), 7 * ENC), (norm_tokens(), n // 16)]]
            for k in range(UNROLL):
                s = i * UNROLL + k
                carry, o = step(s, carry, tokbuf[pl.ds(k * TOK, TOK), :],
                                _Side(zero, SIDE_N, *jobs[k]))
                lo = k * TOK // 16 * 16
                xv = xs[pl.ds(pl.multiple_of(n * i + lo, 16), 32), :].astype(f32)
                _set_rows(hbuf, pl.ds(pl.multiple_of(TOK * s, 8), TOK),
                          xv[k * TOK - lo:(k + 1) * TOK - lo] + o)
            return carry

        carry = (mem0_ref[...].astype(f32), jnp.int32(P0), jnp.int32(0), jnp.int32(0))
        carry = lax.fori_loop(0, NSEG // UNROLL, steps, carry)
        return carry[1] >> 16

    zero = pl.run_scoped(
        block_a,
        *[pltpu.VMEM((H, D // 2, DH), u32)] * 3,
        pltpu.VMEM((4 * TOK, D), u32),
        pltpu.VMEM((UNROLL * TOK, D), f32),
        pltpu.VMEM((UNROLL * TOK, D), f32),
        *[pltpu.VMEM((H // 8, RING, DH), f32)] * 16,
    )

    def tail(w4e, ye, res, ue, woe, *pairs):
        ge, oe = pairs[0:2], pairs[2:4]
        w4_copies = [
            pltpu.make_async_copy(w4_hbm.bitcast(u32).at[:, a, :, pl.ds(b * C4, C4)],
                                  w4e.at[4 * a + b], sems.at[SEM_W4])
            for a in range(4) for b in range(4)]
        for cp in w4_copies:
            cp.start()
        done = TOK * NSEG
        first = 4 * TOK * (NSEG // 4 - 1)

        def later(rows, n):
            return pl.ds(pl.multiple_of(rows + 8 * zero, 8), n)

        def run(dots, ties, *jobs, hold=(), lag=1):
            side = _Side(zero, len(dots) * len(ties), *jobs)
            prods = []
            for load in dots:
                lhs, rhs = load()
                for ref in hold if len(prods) >= lag else ():
                    side.after(ref, prods[-lag])
                for r0, c0 in ties:
                    lhs = side.tie(lhs, r0, c0)
                prods.append(_dot(_unpack(lhs), _unpack(rhs)))
            return prods

        hk, hn, hm = H * DH // 4, D // 2, P0 // 2
        wo_op = {0: (woe, 0, 0), 1: (wo_b, 0, 0), 2: (wo_b, 0, hn), 3: (wo_b, hk, 0),
                 4: (wo_b, hk, hn), 5: (woe, hk, 0), 6: (woe, 2 * hk, 0)}

        def encode_wo():
            for i0 in range(0, hk, 8):
                for c in range(0, hn, C4):
                    raw = {(a, b): wo_b[pl.ds(hk * a + i0, 8), pl.ds(hn * b + c, C4)]
                           for a, b in QUAD}
                    get = functools.cache(lambda k, a, b: _unzip(raw[a, b], k))
                    for p in (0, 2, 3, 5, 6):
                        ref, r0, c0 = wo_op[p]
                        ref[pl.ds(r0 + i0, 8), pl.ds(c0 + c, C4)] = _zip(
                            *[_combine(functools.partial(get, k), SB[p]) for k in range(2)])
                    yield [(woe, (0,))]

        def encode_o(n):
            for kt in range(H // 2):
                for s in range(hm // 16):
                    oe[n % 2][pl.ds(8 * s, 8), pl.ds(128 * kt, 128)] = _zip(*[_combine(
                        lambda a, b: q_r[H // 2 * b + kt][pl.ds(
                            (done + hm * a + 16 * s) % RING + k + n * zero, 8, stride=2), :],
                        SA[ORDER_B[n]]) for k in range(2)])
                    if s % 4 == 3:
                        yield [(oe[n % 2], (0,))]

        def wo_dots(n):
            ref, r0, c0 = wo_op[ORDER_B[n]]
            rows = lambda i: later(r0 + 8 * i * zero, hk) if n > 1 else pl.ds(r0, hk)
            return [lambda i=i, j=j: (oe[n % 2][later(hm // 4 * i + 8 * j * zero, hm // 4), :],
                                      ref[rows(i), pl.ds(c0 + C4 * j, C4)])
                    for j, i in QUAD]

        def decode_wo(n, prods):
            for (j, i), v in zip(QUAD, prods):
                for r in range(0, hm // 2, 16):
                    for (a, b), sign in SC[ORDER_B[n]]:
                        fresh = all(key != (a, b) for q in ORDER_B[:n] for key, _ in SC[q])
                        row = done + hm * a + hm // 2 * i + r
                        for k in range(2):
                            c = 4 * b + 2 * j + k
                            old = (xs[pl.ds(row, 16), pl.ds(128 * c, 128)].astype(f32) if fresh
                                   else hbuf[c, later(row + 8 * n * zero, 16), :])
                            new = v[r:r + 16, 128 * k:128 * (k + 1)]
                            hbuf[c, pl.ds(row, 16), :] = old + new if sign > 0 else old - new
                    yield [(hbuf, (0, 0))]

        hsb = wo_b

        def norm_in(r0):
            for r in range(r0, r0 + RB, 16):
                hsb[pl.ds(r, 16), :] = pltpu.bitcast(
                    _ln(_rows(hbuf, later(r + 56 * zero, 16))), u32)
                yield [(hsb, (r,))]
            for r in range(r0, r0 + RB, 16):
                ue[pl.ds((r - done) // 2, 8), :] = _pack(
                    _ln(pltpu.bitcast(hsb[later(r, 16), :], f32)))
                yield [(ue, (0,))]

        def in_dots(lhs, cols):
            return [lambda c=c: (lhs(), w1b[c // 2, :, pl.ds(128 * (c % 2), 128)])
                    for c in cols]

        def gelu_in(r0, cols, prods):
            for c, v in zip(cols, prods):
                for r in range(0, v.shape[0], 32):
                    xg[c, pl.ds(HALO + r0 + r, 32), :] = _gelu(v[r:r + 32])
                    yield [(xg, (c, HALO + r0))]

        def encode_g(i):
            for s in range(R4 // 16):
                for kt in range(2):
                    get = functools.cache(lambda k, a, b: xg[2 * b + kt, pl.ds(
                        HALO + i * RB + R4 * a + 16 * s + k + SHIFT[b], 8, stride=2), :])
                    for p in ORDER_A:
                        for r, w in enumerate(_encode7(SA, p, get)):
                            ge[i % 2][7 * p + r, pl.ds(8 * s, 8), pl.ds(128 * kt, 128)] = w
                        yield [(ge[i % 2], (0, 0))]

        def out_dots(i, j):
            return [lambda p=p: (ge[i % 2][p, later(8 * j * zero, R4 // 2), :],
                                 we[NC + j, later(128 * p + 8 * i * zero, 128), :])
                    for p in range(NP)]

        def decode_out(i, j, prods):
            for r0 in range(0, R4, 8):
                out = _decode(prods, r0)
                for ii, jj in QUAD:
                    for a, b in QUAD:
                        hsb[pl.ds(i * RB + R4 * (2 * a + ii) + r0, 8),
                            pl.ds(C4 * (2 * b + jj) + 128 * j, 128)] = pltpu.bitcast(
                                out[2 * a + ii, 2 * b + jj], u32)
                    yield [(hsb, (i * RB,))]

        def encode_w4():
            for c in range(NC):
                for i0 in range(0, 64, 8):
                    for j in range(2):
                        at = (c, pl.ds(i0, 8), pl.ds(128 * j, 128))
                        raw = {(a, b): w4e[(4 * a + b,) + at]
                               for a in range(4) for b in range(4)}
                        get = functools.cache(lambda k, a, b: _unzip(raw[a, b], k))
                        for p in ORDER_B:
                            for r, w in enumerate(_encode7(SB, p, get)):
                                w4e[(7 * p + r,) + at] = w
                            yield [(w4e, (0, c, i0))]

        def mixer_post(r0, zero):
            for r in range(0, RB, POST_ROWS):
                rows = pl.ds(_mult(r0 + r, 8), POST_ROWS)
                hv = _rows(hbuf, rows)
                x1 = _ln(hv) + pltpu.bitcast(hsb[rows, :], f32)
                _set_rows(res, pl.ds(r, POST_ROWS), hv + x1)
                hsb[rows, :] = pltpu.bitcast(x1, u32)
                yield [(res, (0, 0)), (hsb, (r0,))]
            for r in range(0, RB, POST_ROWS):
                rows = pl.ds(pl.multiple_of(r0 + r + 8 * zero, 8), POST_ROWS)
                _set_rows(hbuf, rows, _ln(pltpu.bitcast(hsb[rows, :], f32)))
                yield [(hbuf, (0, r0))]
            for s in range(R4 // 16):
                for kt in range(2):
                    get = functools.cache(lambda k, a, b: hbuf[2 * b + kt, pl.ds(
                        r0 + R4 * a + 32 * (s // 2) + 2 * k + s % 2, 8, stride=4), :])
                    for p in ORDER_A:
                        for r, w in enumerate(_encode7(SA, p, get)):
                            ye[7 * p + r, pl.ds(8 * s, 8), pl.ds(128 * kt, 128)] = w
                        if p in (0, 6, 5):
                            yield [(ye, (0, 8 * s))]

        n_g, n_out, n_o = 7 * R4 // 8, R4 // 2, H // 2 * hm // 64
        n_post = 2 * RB // POST_ROWS + 6 * R4 // 16
        out_ties = ((0, 0), (16, 0))
        wo_ties = [(r0, c0) for c0 in range(0, 2 * D, 512) for r0 in range(0, 64, 8)]
        in_ties = [(r0, c0) for c0 in (0, 512) for r0 in range(0, 128, 8)]
        w4_job, wo_job = encode_w4(), encode_wo()

        def mixer_out(i, pending, *jobs):
            for j in range(2):
                prods = run(out_dots(i, j), out_ties, pending,
                            *[(job, count // 2) for job, count in jobs],
                            hold=(w4e,) if i else (), lag=6)
                pending = (decode_out(i, j, prods), n_out)
            return pending

        u = _pack(_ln(_ln(_rows(hbuf, pl.ds(first, done - first)))))
        pending = (encode_o(0), n_o)
        list(pending[0])
        for n in range(7):
            jobs = [(encode_o(n + 1), n_o) if n < 6 else (encode_g(0), n_g)]
            if n:
                jobs.append(pending)
            if n < 2:
                jobs.append((wo_job, hk // 8))
            if n == W4_AT:
                for cp in w4_copies:
                    cp.wait()
            if n >= W4_AT:
                jobs.append((w4_job, 7 * W4_SPLIT[8]))
            prods = run(wo_dots(n), wo_ties, *jobs, hold=(w4e,) if n >= W4_AT else ())
            pending = (decode_wo(n, prods), hm // 8)
        prods = run(in_dots(lambda: u, range(8)), in_ties[:6], pending)
        pending = (gelu_in(first, range(8), prods), 24)
        for i in range(5):
            jobs = [(w4_job, 7 * W4_SPLIT[i])]
            if i < 4:
                jobs.append((encode_g(i + 1), n_g))
            if i > 2:
                jobs.append((norm_in(done + (i - 3) * RB), RB // 8))
            pending = mixer_out(i, pending, *jobs)
        post = mixer_post(0, zero)
        for n in range(8):
            r0, cols = done + n // 4 * RB, range(n % 4 * 2, n % 4 * 2 + 2)
            jobs = [pending]
            jobs.append((post, n_post // 8))
            if n == 6:
                jobs.append((encode_g(5), n_g))
            prods = run(in_dots(
                lambda: ue[later((r0 - done) // 2 + 8 * n * zero, RB // 2), :], cols), in_ties,
                *jobs)
            pending = (gelu_in(r0, cols, prods), RB // 16)
        list(pending[0])
        pending = (None, 0)
        for i in range(5, 8):
            jobs = [(w4_job, 7 * W4_SPLIT[i])]
            if i < 7:
                jobs.append((encode_g(i + 1), n_g))
            pending = mixer_out(i, pending, *jobs)
        list(pending[0])
        list(w4_job)

        def mlp_block(i, carry):
            te = []
            for c in range(NC):
                prods = [_dot(_unpack(ye[p]), _unpack(we[c, pl.ds(128 * p, 128), :]))
                         for p in range(NP)]
                ops = []
                for s in range(R4 // 16):
                    act = [{key: _gelu(v) for key, v in _decode(
                        prods, 32 * (s // 2) + 16 * k + 8 * (s % 2)).items()}
                        for k in range(2)]
                    ops.append(_encode(SA, lambda k, a, b: act[k][a, b]))
                te.append([jnp.concatenate([o[p] for o in ops], axis=0) for p in range(NP)])

            def down(p, lo, hi, tie=lambda w: w):
                lhs = jnp.concatenate([tie(te[c][p]) if c in POST_C else te[c][p]
                                       for c in range(lo, hi)], axis=1)
                return _dot(_unpack(lhs), _unpack(w4e[p, lo:hi].reshape((hi - lo) * 64, C4)))

            prods = [down(p, 0, KSPLIT) for p in range(NSPLIT)]
            prods = [m + down(p, KSPLIT, NC) for p, m in enumerate(prods)]
            out = {(a, b): jnp.concatenate(
                [res[2 * b + j, pl.ds(R4 * a, R4), :] for j in range(2)], axis=1)
                for a in range(4) for b in range(4)}
            side = _Side(i >> 3, POST_N * len(POST_C),
                         (mixer_post(jnp.minimum(i + 1, S // RB - 1) * RB, i >> 3), n_post))
            for p in range(7):
                for q in range(len(prods), 7 * p + 7):
                    side.after(hbuf, prods[q - POST_LAG])
                    prods.append(down(q, 0, NC, side.tie))
                _decode7(p, prods[7 * p:7 * p + 7], out)
            for (a, b), v in out.items():
                xs[pl.ds(pl.multiple_of(i * RB + R4 * a, R4), R4), pl.ds(C4 * b, C4)] = (
                    v.astype(bf16))
            out_copy(i).start()
            return carry

        lax.fori_loop(0, S // RB, mlp_block, 0)
        for i in range(S // RB):
            out_copy(i).wait()

    pl.run_scoped(
        tail,
        pltpu.VMEM((NP + 1, NC, 64, C4), u32),
        pltpu.VMEM((NP, R4 // 2, C4), u32),
        pltpu.VMEM((D // 128, RB, 128), f32),
        pltpu.VMEM((P0 // 2, D), u32),
        pltpu.VMEM((3 * H * DH // 4, D // 2), u32),
        *[pltpu.VMEM((NP, R4 // 2, C4), u32)] * 2,
        *[pltpu.VMEM((P0 // 4, H * DH // 2), u32)] * 2,
    )


@jax.jit
def pallas_sequential_preLN__memory_aug_recurrent_mem_tr__mixer_s_mlp__prompt_kernel(
    A_x: jax.Array,
    A_mem0: jax.Array,
    A_Wq: jax.Array,
    A_Wk: jax.Array,
    A_Wv: jax.Array,
    A_Wo: jax.Array,
    A_seg_len: jax.Array,
    B_x: jax.Array,
    B_w1: jax.Array,
    B_w2: jax.Array,
    B_w3: jax.Array,
    B_w4: jax.Array,
):
    del A_seg_len, B_x
    hbm = pl.BlockSpec(memory_space=pl.ANY)
    vmem = pl.BlockSpec(memory_space=pltpu.VMEM)
    scratch = [
        pltpu.VMEM((H * DH // 2, D), u32),
        pltpu.VMEM((S, D), bf16),
        pltpu.VMEM((D // 128, S + 8, 128), f32),
        pltpu.VMEM((D // 128, S + 2 * HALO, 128), f32),
        pltpu.VMEM((4, D // 2, C4), u32),
        pltpu.VMEM((NC + 3, NP * 128, 128), u32),
        pltpu.SemaphoreType.DMA((NSEM,)),
    ] + [pltpu.VMEM((H // 8, RING, DH), f32)] * 8
    out = pl.pallas_call(
        _kernel,
        out_shape=jax.ShapeDtypeStruct((S, D), A_x.dtype),
        in_specs=[hbm, vmem] + [hbm] * 8,
        out_specs=hbm,
        scratch_shapes=scratch,
        compiler_params=pltpu.CompilerParams(vmem_limit_bytes=int(127.9 * 1024 * 1024)),
    )(A_x.reshape(S, D), A_mem0.reshape(MEM, D),
      A_Wq.reshape(D // 2, 2 * H, DH), A_Wk.reshape(D // 2, 2 * H, DH),
      A_Wv.reshape(D // 2, 2 * H, DH),
      A_Wo.reshape(H * DH, D), B_w1, B_w2, B_w3, B_w4.reshape(NC, 4, 128, D))
    return out.reshape(A_x.shape)
```

```python
import functools

import jax
import jax.numpy as jnp
from jax import lax
import jax.experimental.pallas as pl
import jax.experimental.pallas.tpu as pltpu

S = 2048
D = 1024
H = 32
DH = 128
MEM = 8
SEG = 32
F = 3584
NSEG = S // SEG
L = MEM + SEG
TOK = 24
P0 = S - TOK * NSEG
RING = 576
X0 = P0 + 128
C4 = D // 4
SHIFT = (-1, 1, -2, 2)
HALO = 8
RB = 256
R4 = RB // 4
NC = F // 512
NP = 49
EPS = 1e-5
NEG = -1000000000.0

LAG_QK, LAG_PV, LAG_WO = 2, 4, 6
FILL_AT = 20
UNROLL = 2
ENC = 5
VMEM_LIMIT = 127 * 1024 * 1024 + 896 * 1024
ENC_R = (6,)
ENC0 = 0
SIDE_R = (0,)
SIDE_AT = 6
SIDE_N = 48
LN_ROWS = 16
NSPLIT = 7
KSPLIT = 4
POST_C = (0, 2, 4)
PRO_AT = 2
PRO_K = 8
POST_N = 40
POST_LAG = 7
POST_ROWS = 16
POST_P = (0, 6, 5)
W4_SPLIT = (10, 8, 8, 8, 10, 8, 8, 8, 14, 2)
W4_AT = 5

bf16 = jnp.bfloat16
f32 = jnp.float32
u32 = jnp.uint32

SEM_X0, SEM_X, SEM_W1, SEM_W23, SEM_W4, SEM_WO, SEM_OUT, SEM_W = 0, 1, 2, 3, 4, 5, 9, 25
NSEM = SEM_W + 12

SA = (((0, 0), 1, (1, 1)), ((1, 0), 1, (1, 1)), ((0, 0),), ((1, 1),),
      ((0, 0), 1, (0, 1)), ((1, 0), -1, (0, 0)), ((0, 1), -1, (1, 1)))
SB = (((0, 0), 1, (1, 1)), ((0, 0),), ((0, 1), -1, (1, 1)), ((1, 0), -1, (0, 0)),
      ((1, 1),), ((0, 0), 1, (0, 1)), ((1, 0), 1, (1, 1)))
SC = ((((0, 0), 1), ((1, 1), 1)), (((1, 0), 1), ((1, 1), -1)),
      (((0, 1), 1), ((1, 1), 1)), (((0, 0), 1), ((1, 0), 1)),
      (((0, 0), -1), ((0, 1), 1)), (((1, 1), 1),), (((0, 0), 1),))
ORDER_A = (2, 3, 0, 4, 6, 1, 5)
ORDER_B = (1, 4, 0, 2, 5, 3, 6)
QUAD = ((0, 0), (0, 1), (1, 0), (1, 1))


def _mult(i, n):
    return i if isinstance(i, int) else pl.multiple_of(i, n)


def _ln(x):
    m = jnp.mean(x, axis=-1, keepdims=True)
    d = x - m
    v = jnp.mean(d * d, axis=-1, keepdims=True)
    return d * lax.rsqrt(v + EPS)


def _gelu(x):
    c = 0.7978845608028654
    half = 0.5 * x
    return half * jnp.tanh(x * (c + c * 0.044715 * (x * x))) + half


def _pack(x):
    return pltpu.bitcast(x.astype(bf16), u32)


def _unpack(x):
    return pltpu.bitcast(x, bf16)


def _dot(a, b):
    return jnp.dot(a, b, preferred_element_type=f32)


def _zip(even, odd):
    return pltpu.bitcast(pltpu.pack_elementwise([even, odd], packed_dtype=bf16), u32)


def _unzip(w, k):
    return pltpu.unpack_elementwise(w, index=k, packed_dtype=bf16, unpacked_dtype=f32)


def _combine(get, term):
    if len(term) == 1:
        return get(*term[0])
    a, b = get(*term[0]), get(*term[2])
    return a + b if term[1] > 0 else a - b


def _encode7(tab, p, get):
    outer = [{(i, j): _combine(lambda a, b: get(k, 2 * a + i, 2 * b + j), tab[p])
              for i, j in QUAD} for k in range(2)]
    return [_zip(*[_combine(lambda a, b: o[a, b], tab[r]) for o in outer])
            for r in range(7)]


def _encode(tab, get):
    get = functools.cache(get)
    ops = {p: _encode7(tab, p, get) for p in (ORDER_A if tab is SA else ORDER_B)}
    return [w for p in range(7) for w in ops[p]]


def _accumulate(acc, key, sign, v):
    if key not in acc:
        acc[key] = v
    else:
        acc[key] = acc[key] + v if sign > 0 else acc[key] - v


def _decode7(p, prods, out):
    inner = {}
    for r in range(7):
        for key, sign in SC[r]:
            _accumulate(inner, key, sign, prods[r])
    for (a, b), sign in SC[p]:
        for (i, j), v in inner.items():
            _accumulate(out, (2 * a + i, 2 * b + j), sign, v)


def _decode(prods, r0):
    out = {}
    for p in range(7):
        _decode7(p, [pltpu.bitcast(m[r0:r0 + 8, :], f32) for m in prods[7 * p:7 * p + 7]],
                 out)
    return out


def _rows(ref, rows):
    return jnp.concatenate([ref[c, rows, :] for c in range(ref.shape[0])], axis=1)


def _set_rows(ref, rows, v):
    for c in range(ref.shape[0]):
        ref[c, rows, :] = v[:, c * 128:(c + 1) * 128]


class _Side:
    def __init__(self, zero, slots, *jobs):
        self.zero = zero
        self.slots = slots
        self.jobs = [[job, count, 0] for job, count in jobs]
        self.at = 0

    def tie(self, w, r0=0, c0=0):
        self.at += 1
        head = old = w[r0:r0 + 8, c0:c0 + 128]
        for job in self.jobs:
            while job[2] * self.slots < min(self.at, self.slots) * job[1]:
                job[2] += 1
                for ref, idx in next(job[0]):
                    row = pl.ds(pl.multiple_of(idx[-1] + 8 * self.zero, 8), 8)
                    seen = ref[idx[:-1] + (row, pl.ds(0, 128))]
                    head = jnp.where(self.zero == 0, head, pltpu.bitcast(seen, u32))
        if head is old:
            return w
        row = [v for v in (w[r0:r0 + 8, :c0] if c0 else None, head,
                           w[r0:r0 + 8, c0 + 128:] if c0 + 128 < w.shape[1] else None)
               if v is not None]
        rows = (w[:r0] if r0 else None, jnp.concatenate(row, axis=1),
                w[r0 + 8:] if r0 + 8 < w.shape[0] else None)
        return jnp.concatenate([v for v in rows if v is not None], axis=0)

    def after(self, ref, r):
        spare = pl.multiple_of(ref.shape[-2] - 8 - 8 * self.zero, 8)
        lead = tuple(n - 1 - self.zero for n in ref.shape[:-2])
        ref[lead + (pl.ds(spare, 8), pl.ds(0, 128))] = pltpu.bitcast(r[:8, :128], ref.dtype)

    def finish(self):
        for job in self.jobs:
            for _ in job[0]:
                pass


def _kernel(x_hbm, mem0_ref, wq_hbm, wk_hbm, wv_hbm, wo_hbm, w1_hbm, w2_hbm,
            w3_hbm, w4_hbm, out_hbm,
            wo_b, xs, hbuf, xg, w1b, we, sems, *q_rings):
    w_hbm = (wq_hbm, wk_hbm, wv_hbm)
    q_r = [q_rings[h % 8].at[h // 8] for h in range(H)]

    x0_copy = pltpu.make_async_copy(x_hbm.at[pl.ds(0, X0)], xs.at[pl.ds(0, X0)],
                                    sems.at[SEM_X0])
    x_copy = pltpu.make_async_copy(x_hbm.at[pl.ds(X0, S - X0)], xs.at[pl.ds(X0, S - X0)],
                                   sems.at[SEM_X])

    def wo_copy(i):
        rows = pl.ds(_mult(i * 512, 512), 512)
        return pltpu.make_async_copy(wo_hbm.bitcast(u32).at[rows], wo_b.at[rows],
                                     sems.at[SEM_WO + i])

    def w1_copy(i):
        cols = pl.ds(_mult(i * C4, C4), C4)
        return pltpu.make_async_copy(w1_hbm.bitcast(u32).at[:, cols], w1b.at[i],
                                     sems.at[SEM_W1])

    def w23_copies(c):
        src, first, step = (w3_hbm, 4 * c, 1) if c < NC else (w2_hbm, c - NC, 2)
        return [pltpu.make_async_copy(
            src.bitcast(u32).at[:, pl.ds((first + step * b) * 128, 128)],
            we.at[c, pl.ds(b * 512, 512)], sems.at[SEM_W23]) for b in range(4)]

    def block_a(wq_s, wk_s, wv_s, ubuf, tokbuf, lnbuf, *kv_rings):
        w_s = (wq_s, wk_s, wv_s)
        rings = tuple(q_rings) + tuple(kv_rings)
        ring = [[rings[m * 8 + h % 8].at[h // 8] for h in range(H)] for m in range(3)]
        k_r, v_r = ring[1:]

        stg = [we.at[m, pl.ds(0, 4 * D)] for m in range(3)]
        xe = we.at[3]
        w_op = (hbuf, xg)

        def start_chunk(g, m):
            src = w_hbm[m].bitcast(u32)
            dst = stg[m].reshape(D // 2, 8, DH)
            for par in range(2):
                pltpu.make_async_copy(
                    src.at[:, pl.ds(_mult(16 * par + 4 * g, 4), 4), :],
                    dst.at[:, pl.ds(4 * par, 4), :],
                    sems.at[SEM_W + 3 * g + m]).start()

        def wait_chunk(g, m):
            pltpu.make_async_copy(stg[m], stg[m], sems.at[SEM_W + 3 * g + m]).wait()

        def encode_unit(g, m, half, slices):
            h0 = 8 * g + 4 * half
            for i0 in slices:
                blk = {}

                def get(k, a, b):
                    if (k, a, b) not in blk:
                        for par in range(2):
                            w = stg[m][pl.ds(8 * (128 * a + i0) + 4 * par + 2 * half + b // 2,
                                             8, stride=8), :]
                            for j in range(2):
                                blk[par, a, b - b % 2 + j] = _unzip(w, j)
                        for j in (b - b % 2, b - b % 2 + 1):
                            w_s[m][h0 + j, pl.ds(128 * a + i0, 8), :] = _zip(
                                blk[0, a, j], blk[1, a, j])
                    return blk[k, a, b]

                for p in ORDER_B:
                    known = len(blk)
                    for r, w in enumerate(_encode7(SB, p, get)):
                        q = 7 * p + r
                        if len(SB[p]) + len(SB[r]) > 2:
                            w_op[half][1 + q // 16, pl.ds(128 * (q % 16) + i0, 8), :] = (
                                pltpu.bitcast(w, f32))
                    yield [(w_op[half], (1, i0))] + [(w_s[m], (h0, i0))] * (len(blk) > known)

        def operand(g, m, half, q, zero):
            tp, tr = SB[q // 7], SB[q % 7]
            if len(tp) + len(tr) == 2:
                a, b = (2 * tp[0][n] + tr[0][n] for n in range(2))
                return w_s[m][8 * g + 4 * half + b, pl.ds(128 * a, 128), :]
            return w_op[half][1 + q // 16, pl.ds(
                pl.multiple_of(128 * (q % 16) + 8 * zero, 8), 128), :]

        def decode_unit(g, m, half, prods):
            for r0 in range(0, P0 // 4, 8):
                out = _decode(prods, r0)
                for i, j in QUAD:
                    for a, b in QUAD:
                        rings[8 * m + 4 * half + 2 * b + j][
                            g, pl.ds(P0 // 4 * (2 * a + i) + r0, 8), :] = out[2 * a + i, 2 * b + j]
                    yield [(rings[8 * m + 4 * half + 2 * b + j], (g, r0)) for b in range(2)]

        x0_copy.start()
        for m in range(3):
            start_chunk(0, m)
        x0_copy.wait()

        @pl.loop(0, P0 // 64)
        def _(s):
            for a in range(4):
                rows = pl.ds(pl.multiple_of(P0 // 4 * a + 16 * s, 16), 16)
                _set_rows(hbuf, rows, _ln(xs[rows, :].astype(f32)))
            for kt in range(2):
                ops = _encode(SA, lambda k, a, b: hbuf[
                    2 * b + kt, pl.ds(P0 // 4 * a + 16 * s + k, 8, stride=2), :])
                for p, w in enumerate(ops):
                    xe[pl.ds(pl.multiple_of(128 * p + 64 * kt + 8 * s, 8), 8), :] = w

        tokbuf[...] = _ln(xs[pl.ds(P0, UNROLL * TOK), :].astype(f32))
        wait_chunk(0, 0)

        @pl.loop(0, 16)
        def _(i):
            list(encode_unit(0, 0, 0, [pl.multiple_of(8 * i, 8)]))

        last = [we.at[4, pl.ds(128 * p, 128)] for p in range(NP)]

        @pl.loop(0, 4)
        def _(g):
            g1 = jnp.minimum(g + 1, 3)
            zero = g >> 2
            jobs = [(decode_unit((g + 3) & 3, 2, 1, last), 64)]
            for m in range(3):
                for half in range(2):
                    nxt = (g1, 0, 0) if (m, half) == (2, 1) else (g, m + half, 1 - half)
                    side = _Side(zero, (NP - PRO_AT - 1) * PRO_K,
                                 (encode_unit(*nxt, range(0, 128, 8)), 16 * 7), *jobs)
                    prods = []
                    for p in range(NP):
                        lhs = jnp.concatenate(
                            [xe[pl.ds(128 * p + 64 * kt, 64), :] for kt in range(2)], axis=1)
                        rhs = operand(g, m, half, p, zero)
                        if p > PRO_AT:
                            for k in range(PRO_K):
                                lhs = side.tie(lhs, 64 // PRO_K * k)
                        prods.append(_dot(_unpack(lhs), _unpack(rhs)))
                        if half == 1 and p == 1:
                            if m < 2:
                                wait_chunk(g, m + 1)
                            else:
                                pl.when(g < 3)(functools.partial(wait_chunk, g1, 0))
                            pl.when(g < 3)(functools.partial(start_chunk, g1, m))
                            if m == 0:
                                w1_copy(g).start()
                            if m == 1:
                                wo_copy(g).start()
                    jobs = [(decode_unit(g, m, half, prods), 64)]
            for p in range(NP):
                we[4, pl.ds(128 * p, 128), :] = pltpu.bitcast(prods[p], u32)

        list(decode_unit(3, 2, 1, last))

        x_copy.start()
        _set_rows(xg, pl.ds(0, HALO), jnp.zeros((HALO, D), f32))
        _set_rows(xg, pl.ds(HALO + S, HALO), jnp.zeros((HALO, D), f32))
        _set_rows(hbuf, pl.ds(0, UNROLL * TOK), jnp.zeros((UNROLL * TOK, D), f32))
        ubuf[...] = jnp.zeros(ubuf.shape, u32)
        for c in range(NC + 2):
            for cp in w23_copies(c):
                cp.start()
        for i in range(4):
            w1_copy(i).wait()
        for i in range(4):
            wo_copy(i).wait()

        def wrap(r):
            return jnp.where(r >= RING, r - RING, r)

        def step(s, carry, tok, side):
            mem, rp, ra, rw = carry
            ri = lax.broadcasted_iota(jnp.int32, (2 * MEM + SEG, 2 * L), 0)
            ci = lax.broadcasted_iota(jnp.int32, (2 * MEM + SEG, 2 * L), 1)
            key_b = ((ci >= MEM) & (ci < 2 * MEM)) | (ci >= 2 * MEM + SEG)
            same = key_b == ((ri >= MEM) & (ri < 2 * MEM))
            mask = same & ((ri < 2 * MEM) | (ri >= ci))
            fill = jnp.where(same, NEG, -jnp.inf)

            lhs = jnp.concatenate([mem, tok], axis=0).astype(bf16)
            rps = [pl.multiple_of(wrap(rp + 8 * i), 8) for i in range(3)]
            ra_ = pl.multiple_of(ra, SEG)
            rw_ = pl.multiple_of(rw, 8)

            col = s & 3
            group = jnp.maximum((s >> 2) - 1, 0)
            rb = pl.multiple_of(group * (4 * TOK), 8)

            def filler(j):
                u = ubuf[pl.ds(pl.multiple_of((group & 1) * (2 * TOK), 8), 2 * TOK), :]
                r = _dot(_unpack(u), _unpack(w1b[col, :, pl.ds(j * 128, 128)]))
                xg[2 * col + j, pl.ds(HALO + rb, 4 * TOK), :] = _gelu(r)

            mem_qkv = {}
            scores = {}
            o_mem = {}
            total = [None]

            def qkv(h):
                for m in range(3):
                    w = w_s[m][h]
                    for r0 in SIDE_R if h >= SIDE_AT else ():
                        w = side.tie(w, r0)
                    r = _dot(lhs, _unpack(w))
                    for i in range(3):
                        ring[m][h][pl.ds(rps[i], 8), :] = r[8 + 8 * i:16 + 8 * i]
                    mem_qkv[m, h] = r[:MEM]

            def segment(m, pair):
                a, b = 2 * pair, 2 * pair + 1
                ma, mb = mem_qkv.pop((m, a)), mem_qkv.pop((m, b))
                xa, xb = (ring[m][h][pl.ds(ra_, SEG), :] for h in (a, b))
                if m == 0:
                    parts = ((ma, mb, xa), (xb,))
                else:
                    parts = ((ma, mb, xa, xb), (mb, ma, xb))
                return [jnp.concatenate(v, axis=0).astype(bf16) for v in parts]

            def qk(pair):
                q, k = segment(0, pair), segment(1, pair)
                for n in (pair % 2, 1 - pair % 2):
                    scores[pair, n] = lax.dot_general(
                        q[n], k[n], (((1,), (1,)), ((), ())), preferred_element_type=f32)

            def pv(pair):
                v = segment(2, pair)
                for n in (pair % 2, 1 - pair % 2):
                    sc = scores.pop((pair, n)) * (DH ** -0.5)
                    if n == 0:
                        sc = jnp.where(mask, sc, fill)
                    else:
                        sc = jnp.where(mask[2 * MEM:, :2 * MEM + SEG], sc,
                                       fill[2 * MEM:, :2 * MEM + SEG])
                    mx = jnp.max(sc, axis=1, keepdims=True)
                    e = jnp.exp(sc - mx)
                    den = jnp.sum(e, axis=1, keepdims=True)
                    inv = pl.reciprocal(den, approx=True)
                    inv = inv * (2.0 - den * inv)
                    o = _dot(e.astype(bf16), v[n]) * inv
                    q_r[2 * pair + n][pl.ds(ra_, SEG), :] = o[-SEG:]
                    if n == 0:
                        o_mem[2 * pair], o_mem[2 * pair + 1] = o[:MEM], o[MEM:2 * MEM]

            def wo(h):
                lo = jnp.concatenate([o_mem.pop(h), q_r[h][pl.ds(rw_, TOK), :]],
                                     axis=0).astype(bf16)
                r = _dot(lo, _unpack(wo_b[pl.ds(h * DH // 2, DH // 2), :]))
                total[0] = r if total[0] is None else total[0] + r

            npair = H // 2
            for t in range(npair + LAG_WO):
                if 0 <= t - LAG_QK < npair:
                    qk(t - LAG_QK)
                if 0 <= t - LAG_PV < npair:
                    pv(t - LAG_PV)
                if t < npair:
                    qkv(2 * t)
                    qkv(2 * t + 1)
                if t == FILL_AT:
                    filler(0)
                if 0 <= t - LAG_WO < npair:
                    wo(2 * (t - LAG_WO))
                    wo(2 * (t - LAG_WO) + 1)
            filler(1)

            a = total[0]
            return (a[:MEM], wrap(rp + TOK), wrap(ra + SEG), wrap(rw + TOK)), a[MEM:]

        def steps(i, carry):
            n = UNROLL * TOK
            pl.when(i == 1)(x_copy.wait)

            @pl.when(i == 3)
            def _():
                for c in range(NC + 2):
                    for cp in w23_copies(c):
                        cp.wait()

            zero = i >> 5

            def norm_filler():
                prev = jnp.maximum(i - 1, 0)
                for r in range(0, n, LN_ROWS):
                    rows = pl.ds(pl.multiple_of(n * prev + r, 8), LN_ROWS)
                    lnbuf[pl.ds(r, LN_ROWS), :] = _ln(_rows(hbuf, rows))
                    yield [(lnbuf, (r,))]
                for r in range(0, n, LN_ROWS):
                    rows = pl.ds(pl.multiple_of(r + 16 * zero, 8), LN_ROWS)
                    dst = pl.multiple_of((n * (prev & 3) + r) // 2, 8)
                    ubuf[pl.ds(dst, LN_ROWS // 2), :] = _pack(_ln(lnbuf[rows, :]))
                    yield [(ubuf, (dst,))]

            def norm_tokens():
                nxt = jnp.minimum(P0 + n * (i + 1), S - n)
                for r in range(0, n, 16):
                    rows = pl.ds(pl.multiple_of(nxt + r, 16), 16)
                    tokbuf[pl.ds(r, 16), :] = _ln(xs[rows, :].astype(f32))
                    yield [(tokbuf, (r,))]

            def encode_w23():
                for k in range(ENC):
                    j = ENC * i + k
                    grp, i0 = jnp.where(j < 16, NC + 2, (j >> 4) - 1), 8 * (j & 15)
                    slot = lambda q: (grp, pl.ds(pl.multiple_of(128 * q + i0, 8), 8))
                    raw = {(a, b): we[slot(4 * b + a)] for a in range(4) for b in range(4)}
                    get = functools.cache(lambda k, a, b: _unzip(raw[a, b], k))
                    for p in ORDER_B:
                        for r, w in enumerate(_encode7(SB, p, get)):
                            we[slot(7 * p + r)] = w
                            if r in ENC_R:
                                yield [(we, (grp, i0))]

            enc, n_enc = encode_w23(), 7 * len(ENC_R)
            jobs = [[(norm_filler(), 2 * n // LN_ROWS), (enc, n_enc * ENC0)],
                    [(enc, n_enc * (ENC - ENC0)), (norm_tokens(), n // 16)]]
            for k in range(UNROLL):
                s = i * UNROLL + k
                carry, o = step(s, carry, tokbuf[pl.ds(k * TOK, TOK), :],
                                _Side(zero, SIDE_N * len(SIDE_R), *jobs[k]))
                lo = k * TOK // 16 * 16
                xv = xs[pl.ds(pl.multiple_of(n * i + lo, 16), 32), :].astype(f32)
                _set_rows(hbuf, pl.ds(pl.multiple_of(TOK * s, 8), TOK),
                          xv[k * TOK - lo:(k + 1) * TOK - lo] + o)
            return carry

        carry = (mem0_ref[...].astype(f32), jnp.int32(P0), jnp.int32(0), jnp.int32(0))
        carry = lax.fori_loop(0, NSEG // UNROLL, steps, carry)
        return carry[1] >> 16

    zero = pl.run_scoped(
        block_a,
        *[pltpu.VMEM((H, D // 2, DH), u32)] * 3,
        pltpu.VMEM((4 * TOK, D), u32),
        pltpu.VMEM((UNROLL * TOK, D), f32),
        pltpu.VMEM((UNROLL * TOK, D), f32),
        *[pltpu.VMEM((H // 8, RING, DH), f32)] * 16,
    )

    def tail(w4e, ye, ybuf, ue, *bufs):
        woe, pool = bufs[:3], bufs[3:]
        w4_copies = [
            pltpu.make_async_copy(w4_hbm.bitcast(u32).at[:, a, :, pl.ds(b * C4, C4)],
                                  w4e.at[4 * a + b], sems.at[SEM_W4])
            for a in range(4) for b in range(4)]
        for cp in w4_copies:
            cp.start()
        done = TOK * NSEG
        first = 4 * TOK * (NSEG // 4 - 1)

        def later(rows, n):
            return pl.ds(pl.multiple_of(rows + 8 * zero, 8), n)

        def run(dots, ties, *jobs, hold=(), lag=1):
            side = _Side(zero, len(dots) * len(ties), *jobs)
            prods = []
            for load in dots:
                lhs, rhs = load()
                for ref in hold if len(prods) >= lag else ():
                    side.after(ref, prods[-lag])
                for r0, c0 in ties:
                    lhs = side.tie(lhs, r0, c0)
                prods.append(_dot(_unpack(lhs), _unpack(rhs)))
            return prods

        hk, hn, hm = H * DH // 4, D // 2, P0 // 2

        def wo_op(p, j):
            if p == 3:
                return pool[j], 0, 0
            if p in (1, 4):
                return wo_b, hk * (p // 4), hn * (p // 4) + C4 * j
            return woe[{0: 0, 2: 1, 5: 2, 6: 0}[p]], 0, C4 * j

        def encode_wo(ps):
            for i0 in range(0, hk, 8):
                for j in range(2):
                    get = functools.cache(lambda k, a, b: _unzip(wo_b[
                        later(hk * a + i0 + 8 * ps[0] * zero, 8), pl.ds(hn * b + C4 * j, C4)], k))
                    ops = [_zip(*[_combine(functools.partial(get, k), SB[p]) for k in range(2)])
                           for p in ps]
                    for p, w in zip(ps, ops):
                        ref, r0, c0 = wo_op(p, j)
                        ref[pl.ds(r0 + i0, 8), pl.ds(c0, C4)] = w
                    yield [(wo_op(p, j)[0], (0,)) for p in ps]

        def encode_o(n):
            for kt in range(H // 2):
                for s in range(hm // 16):
                    pool[n][pl.ds(hm // 2 * (kt // 2) + 8 * s, 8), pl.ds(kt % 2 * 128, 128)] = (
                        _zip(*[_combine(
                            lambda a, b: q_r[H // 2 * b + kt][pl.ds(
                                (done + hm * a + 16 * s) % RING + k + n * zero, 8, stride=2), :],
                            SA[ORDER_B[n]]) for k in range(2)]))
                    if s % 4 == 3:
                        yield [(pool[n], (0,))]

        def wo_dots(n):
            def load(j, i):
                ref, r0, c0 = wo_op(ORDER_B[n], j)
                lhs = [pool[n][later(hm // 2 * c + hm // 4 * i + 8 * j * zero, hm // 4), :]
                       for c in range(8)]
                return (jnp.concatenate(lhs, axis=1),
                        ref[later(r0 + 8 * i * zero, hk), pl.ds(c0, C4)])
            return [functools.partial(load, j, i) for j, i in QUAD]

        def decode_wo(n, prods):
            for (j, i), v in zip(QUAD, prods):
                for r in range(0, hm // 2, 16):
                    for (a, b), sign in SC[ORDER_B[n]]:
                        fresh = all(key != (a, b) for q in ORDER_B[:n] for key, _ in SC[q])
                        row = done + hm * a + hm // 2 * i + r
                        for k in range(2):
                            c = 4 * b + 2 * j + k
                            old = (xs[pl.ds(row, 16), pl.ds(128 * c, 128)].astype(f32) if fresh
                                   else hbuf[c, later(row + 8 * n * zero, 16), :])
                            new = v[r:r + 16, 128 * k:128 * (k + 1)]
                            hbuf[c, pl.ds(row, 16), :] = old + new if sign > 0 else old - new
                    yield [(hbuf, (0, 0))]

        hsb = wo_b

        def norm_in():
            for r in range(done, S, 32):
                hsb[pl.ds(r, 32), :] = pltpu.bitcast(
                    _ln(_rows(hbuf, later(r + 56 * zero, 32))), u32)
                yield [(hsb, (r,))]
            for r in range(done, S, 32):
                ue[pl.ds((r - done) // 2, 16), :] = _pack(
                    _ln(pltpu.bitcast(hsb[later(r, 32), :], f32)))
                yield [(ue, (0,))]

        def in_dots(lhs, cols, n=0):
            return [lambda c=c: (lhs(c), w1b[c // 2, later(8 * n * zero, D // 2),
                                             pl.ds(128 * (c % 2), 128)]) for c in cols]

        def gelu_in(r0, cols, prods):
            for c, v in zip(cols, prods):
                for r in range(0, v.shape[0], 32):
                    xg[c, pl.ds(HALO + r0 + r, 32), :] = _gelu(v[r:r + 32])
                    yield [(xg, (c, HALO + r0))]

        def encode_g(i):
            for s in range(R4 // 16):
                for kt in range(2):
                    get = functools.cache(lambda k, a, b: xg[2 * b + kt, pl.ds(
                        HALO + i * RB + R4 * a + 16 * s + k + SHIFT[b], 8, stride=2), :])
                    for p in ORDER_A:
                        for r, w in enumerate(_encode7(SA, p, get)):
                            pool[i - 1][pl.ds(R4 // 2 * (7 * p + r) + 8 * s, 8),
                                        pl.ds(128 * kt, 128)] = w
                        yield [(pool[i - 1], (0,))]

        def out_dots(i, j):
            return [lambda p=p: (pool[i - 1][later(R4 // 2 * p + 8 * j * zero, R4 // 2), :],
                                 we[NC + j, later(128 * p + 8 * i * zero, 128), :])
                    for p in range(NP)]

        def decode_out(i, j, prods):
            for r0 in range(0, R4, 8):
                out = _decode(prods, r0)
                for ii, jj in QUAD:
                    for a, b in QUAD:
                        hsb[pl.ds(i * RB + R4 * (2 * a + ii) + r0, 8),
                            pl.ds(C4 * (2 * b + jj) + 128 * j, 128)] = pltpu.bitcast(
                                out[2 * a + ii, 2 * b + jj], u32)
                    yield [(hsb, (i * RB,))]

        def encode_w4():
            for c in range(NC):
                for i0 in range(0, 64, 8):
                    for j in range(2):
                        at = (c, pl.ds(i0, 8), pl.ds(128 * j, 128))
                        raw = {(a, b): w4e[(4 * a + b,) + at]
                               for a in range(4) for b in range(4)}
                        get = functools.cache(lambda k, a, b: _unzip(raw[a, b], k))
                        for p in ORDER_B:
                            for r, w in enumerate(_encode7(SB, p, get)):
                                w4e[(7 * p + r,) + at] = w
                            yield [(w4e, (0, c, i0))]

        def mixer_post(r0, zero):
            for r in range(0, RB, POST_ROWS):
                rows = pl.ds(_mult(r0 + r, 8), POST_ROWS)
                hv = _rows(hbuf, rows)
                x1 = _ln(hv) + pltpu.bitcast(hsb[rows, :], f32)
                _set_rows(xg, rows, hv + x1)
                _set_rows(ybuf, pl.ds(r, POST_ROWS), x1)
                yield [(ybuf, (0, 0)), (xg, (0, r0))]
            for r in range(0, RB, POST_ROWS):
                rows = pl.ds(pl.multiple_of(r + 8 * zero, 8), POST_ROWS)
                _set_rows(hbuf, pl.ds(_mult(r0 + r, 8), POST_ROWS), _ln(_rows(ybuf, rows)))
                yield [(hbuf, (0, r0))]
            for s in range(4):
                for kt in range(2):
                    get = functools.cache(lambda k, a, b: hbuf[2 * b + kt, pl.ds(
                        r0 + R4 * a + 4 * k + s, 8, stride=8), :])
                    for p in ORDER_A:
                        for r, w in enumerate(_encode7(SA, p, get)):
                            ye[7 * p + r, pl.ds(8 * s, 8), pl.ds(128 * kt, 128)] = w
                        if p in POST_P:
                            yield [(ye, (0, 8 * s))]

        def out_copies(i):
            rows = pl.ds(_mult(i * (RB // 2), RB // 2), RB // 2)
            return [pltpu.make_async_copy(
                woe[b].at[rows], out_hbm.bitcast(u32).at[rows, pl.ds(hn * b, hn)],
                sems.at[SEM_OUT + 2 * i + b]) for b in range(2)]

        n_g, n_out, n_o = 7 * R4 // 8, R4 // 2, H // 2 * hm // 64
        n_post = 2 * RB // POST_ROWS + 8 * len(POST_P)
        out_ties = ((0, 0), (16, 0))
        wo_ties = [(r0, c0) for c0 in range(0, 2 * D, 512) for r0 in range(0, 64, 8)]
        in_ties = [(r0, c0) for c0 in (0, 512) for r0 in range(0, 64, 8)]
        w4_job = encode_w4()
        wo_jobs = [encode_wo(ps) for ps in ((0,), (2, 5), (3, 6))]

        def mixer_out(i, pending, *jobs):
            for j in range(2):
                prods = run(out_dots(i, j), out_ties, pending,
                            *[(job, count // 2) for job, count in jobs],
                            hold=(w4e,), lag=6)
                pending = (decode_out(i, j, prods), n_out)
            return pending

        u = _pack(_ln(_ln(_rows(hbuf, pl.ds(first, done - first)))))
        pending = (encode_o(0), n_o)
        list(pending[0])
        for n in range(7):
            jobs = [(encode_o(n + 1), n_o) if n < 6 else (encode_g(0), n_g)]
            if n:
                jobs.append(pending)
            if n < 5:
                jobs.append((wo_jobs[(n + 1) // 2], hk // 8 if n else hk // 4))
            if n == W4_AT:
                for cp in w4_copies:
                    cp.wait()
            if n >= W4_AT:
                jobs.append((w4_job, 7 * W4_SPLIT[8]))
            prods = run(wo_dots(n), wo_ties, *jobs, hold=(w4e,) if n >= W4_AT else ())
            pending = (decode_wo(n, prods), hm // 8)
        prods = run(in_dots(lambda c: u, range(8)), in_ties[:6], pending)
        pending = (gelu_in(first, range(8), prods), 24)
        norm = norm_in()
        for i in range(5):
            jobs = [(w4_job, 7 * W4_SPLIT[i])]
            if i < 4:
                jobs.append((encode_g(i + 1), n_g))
            if i > 0:
                jobs.append((norm, P0 // 64))
            pending = mixer_out(i, pending, *jobs)
        post, g5 = mixer_post(0, zero), encode_g(5)
        for n in range(8):
            r0, cols = done + n // 2 * 128, range(n % 2 * 4, n % 2 * 4 + 4)
            jobs = [pending, (w4_job, 7 * W4_SPLIT[9])]
            jobs.append((post, n_post // 8))
            if n >= 6:
                jobs.append((g5, n_g // 2))
            prods = run(in_dots(
                lambda c: ue[later((r0 - done) // 2 + 8 * c * zero, 64), :], cols, n + 1),
                in_ties, *jobs, hold=(w4e,))
            pending = (gelu_in(r0, cols, prods), RB // 16)
        for i in range(5, 8):
            jobs = [(w4_job, 7 * W4_SPLIT[i])]
            if i < 7:
                jobs.append((encode_g(i + 1), n_g))
            pending = mixer_out(i, pending, *jobs)
        list(pending[0])
        list(w4_job)

        def mlp_block(i, carry):
            te = []
            for c in range(NC):
                prods = [_dot(_unpack(ye[p]), _unpack(we[c, pl.ds(128 * p, 128), :]))
                         for p in range(NP)]
                ops = []
                for s in range(R4 // 16):
                    act = [{key: _gelu(v) for key, v in _decode(
                        prods, 32 * k + 8 * s).items()}
                        for k in range(2)]
                    ops.append(_encode(SA, lambda k, a, b: act[k][a, b]))
                te.append([jnp.concatenate([o[p] for o in ops], axis=0) for p in range(NP)])

            def down(p, lo, hi, tie=lambda w: w):
                lhs = jnp.concatenate([tie(te[c][p]) if c in POST_C else te[c][p]
                                       for c in range(lo, hi)], axis=1)
                return _dot(_unpack(lhs), _unpack(w4e[p, lo:hi].reshape((hi - lo) * 64, C4)))

            prods = [down(p, 0, KSPLIT) for p in range(NSPLIT)]
            prods = [m + down(p, KSPLIT, NC) for p, m in enumerate(prods)]
            out = {}

            def finish(qa, qb):
                for a, b in ((2 * qa + n // 2, 2 * qb + n % 2) for n in range(4)):
                    for r in range(0, R4, 16):
                        row = i * RB + R4 * a + r
                        for j in range(2):
                            woe[qb][pl.ds(pl.multiple_of(row // 2, 8), 8),
                                    pl.ds(C4 * (b % 2) + 128 * j, 128)] = _zip(*[
                                        out[a, b][32 * k + r // 2:32 * k + r // 2 + 8,
                                                  128 * j:128 * (j + 1)]
                                        + xg[2 * b + j, pl.ds(row + k, 8, stride=2), :]
                                        for k in range(2)])
                        yield [(woe[qb], (i * (RB // 2),))]

            side = _Side(i >> 3, POST_N * len(POST_C),
                         (mixer_post(((i + 1) & 7) * RB, i >> 3), n_post))
            for p in range(7):
                done_quad = {4: (1, 0), 5: (0, 1), 6: (1, 1)}.get(p)
                store = _Side(i >> 3, 16, *([(finish(*done_quad), 16)] if done_quad else []))
                for q in range(len(prods), 7 * p + 7):
                    side.after(hbuf, prods[q - POST_LAG])
                    prods.append(down(q, 0, NC, side.tie if q % 7 == 0 else
                                      lambda w: store.tie(side.tie(w))))
                _decode7(p, prods[7 * p:7 * p + 7], out)
            list(finish(0, 0))
            for cp in out_copies(i):
                cp.start()
            return carry

        lax.fori_loop(0, S // RB, mlp_block, 0)
        for i in range(S // RB):
            for cp in out_copies(i):
                cp.wait()

    pl.run_scoped(
        tail,
        pltpu.VMEM((NP + 1, NC, 64, C4), u32),
        pltpu.VMEM((NP, R4 // 2, C4), u32),
        pltpu.VMEM((D // 128, RB, 128), f32),
        pltpu.VMEM((P0 // 2, D), u32),
        *[pltpu.VMEM((H * DH // 4, D // 2), u32)] * 3,
        *[pltpu.VMEM((NP * R4 // 2, C4), u32)] * 8,
    )


@jax.jit
def pallas_sequential_preLN__memory_aug_recurrent_mem_tr__mixer_s_mlp__prompt_kernel(
    A_x: jax.Array,
    A_mem0: jax.Array,
    A_Wq: jax.Array,
    A_Wk: jax.Array,
    A_Wv: jax.Array,
    A_Wo: jax.Array,
    A_seg_len: jax.Array,
    B_x: jax.Array,
    B_w1: jax.Array,
    B_w2: jax.Array,
    B_w3: jax.Array,
    B_w4: jax.Array,
):
    del A_seg_len, B_x
    hbm = pl.BlockSpec(memory_space=pl.ANY)
    vmem = pl.BlockSpec(memory_space=pltpu.VMEM)
    scratch = [
        pltpu.VMEM((H * DH // 2, D), u32),
        pltpu.VMEM((S, D), bf16),
        pltpu.VMEM((D // 128, S + 8, 128), f32),
        pltpu.VMEM((D // 128, S + 2 * HALO, 128), f32),
        pltpu.VMEM((4, D // 2, C4), u32),
        pltpu.VMEM((NC + 3, NP * 128, 128), u32),
        pltpu.SemaphoreType.DMA((NSEM,)),
    ] + [pltpu.VMEM((H // 8, RING, DH), f32)] * 8
    out = pl.pallas_call(
        _kernel,
        out_shape=jax.ShapeDtypeStruct((S, D), A_x.dtype),
        in_specs=[hbm, vmem] + [hbm] * 8,
        out_specs=hbm,
        scratch_shapes=scratch,
        compiler_params=pltpu.CompilerParams(vmem_limit_bytes=VMEM_LIMIT),
    )(A_x.reshape(S, D), A_mem0.reshape(MEM, D),
      A_Wq.reshape(D // 2, 2 * H, DH), A_Wk.reshape(D // 2, 2 * H, DH),
      A_Wv.reshape(D // 2, 2 * H, DH),
      A_Wo.reshape(H * DH, D), B_w1, B_w2, B_w3, B_w4.reshape(NC, 4, 128, D))
    return out.reshape(A_x.shape)
```

```python
import functools

import jax
import jax.numpy as jnp
from jax import lax
import jax.experimental.pallas as pl
import jax.experimental.pallas.tpu as pltpu

S = 2048
D = 1024
H = 32
DH = 128
MEM = 8
SEG = 32
F = 3584
NSEG = S // SEG
L = MEM + SEG
TOK = 24
P0 = S - TOK * NSEG
RING = 576
X0 = P0 + 128
C4 = D // 4
SHIFT = (-1, 1, -2, 2)
HALO = 8
RB = 256
R4 = RB // 4
NC = F // 512
NP = 49
EPS = 1e-5
NEG = -1000000000.0

LAG_QK, LAG_PV, LAG_WO = 2, 4, 6
FILL_AT = 20
UNROLL = 2
ENC = 4
VMEM_LIMIT = 127 * 1024 * 1024 + 896 * 1024
SIDE_R = (0,)
SIDE_AT = 6
SIDE_N = 48
LN_ROWS = 16
NSPLIT = 7
KSPLIT = 4
POST_C = (0, 2, 4)
PRO_AT = 1
PRO_K = 8
PRO_BAR = 0
FENCE = (0, 0, 0)
NORM_ROWS = 32
FENCE_J = (0,)
POST_N = 40
POST_LAG = 7
POST_P = (5,)
W4_SPLIT = (12, 4, 4, 4, 4, 12, 12, 12, 16, 0)
W4_AT = 5

bf16 = jnp.bfloat16
f32 = jnp.float32
u32 = jnp.uint32

SEM_X0, SEM_X, SEM_W1, SEM_W3, SEM_W4, SEM_WO, SEM_OUT, SEM_W = 0, 1, 2, 3, 4, 5, 9, 25
NSEM = SEM_W + 12

SA = (((0, 0), 1, (1, 1)), ((1, 0), 1, (1, 1)), ((0, 0),), ((1, 1),),
      ((0, 0), 1, (0, 1)), ((1, 0), -1, (0, 0)), ((0, 1), -1, (1, 1)))
SB = (((0, 0), 1, (1, 1)), ((0, 0),), ((0, 1), -1, (1, 1)), ((1, 0), -1, (0, 0)),
      ((1, 1),), ((0, 0), 1, (0, 1)), ((1, 0), 1, (1, 1)))
SC = ((((0, 0), 1), ((1, 1), 1)), (((1, 0), 1), ((1, 1), -1)),
      (((0, 1), 1), ((1, 1), 1)), (((0, 0), 1), ((1, 0), 1)),
      (((0, 0), -1), ((0, 1), 1)), (((1, 1), 1),), (((0, 0), 1),))
ORDER_A = (2, 3, 0, 4, 6, 1, 5)
ORDER_B = (1, 4, 0, 2, 5, 3, 6)
QUAD = ((0, 0), (0, 1), (1, 0), (1, 1))


def _mult(i, n):
    return i if isinstance(i, int) else pl.multiple_of(i, n)


def _ln(x):
    m = jnp.mean(x, axis=-1, keepdims=True)
    d = x - m
    v = jnp.mean(d * d, axis=-1, keepdims=True)
    return d * lax.rsqrt(v + EPS)


def _gelu(x):
    c = 0.7978845608028654
    half = 0.5 * x
    return half * jnp.tanh(x * (c + c * 0.044715 * (x * x))) + half


def _pack(x):
    return pltpu.bitcast(x.astype(bf16), u32)


def _unpack(x):
    return pltpu.bitcast(x, bf16)


def _dot(a, b):
    return jnp.dot(a, b, preferred_element_type=f32)


def _zip(even, odd):
    return pltpu.bitcast(pltpu.pack_elementwise([even, odd], packed_dtype=bf16), u32)


def _unzip(w, k):
    return pltpu.unpack_elementwise(w, index=k, packed_dtype=bf16, unpacked_dtype=f32)


def _combine(get, term):
    if len(term) == 1:
        return get(*term[0])
    a, b = get(*term[0]), get(*term[2])
    return a + b if term[1] > 0 else a - b


def _encode7(tab, p, get):
    outer = [{(i, j): _combine(lambda a, b: get(k, 2 * a + i, 2 * b + j), tab[p])
              for i, j in QUAD} for k in range(2)]
    return [_zip(*[_combine(lambda a, b: o[a, b], tab[r]) for o in outer])
            for r in range(7)]


def _encode(tab, get):
    get = functools.cache(get)
    ops = {p: _encode7(tab, p, get) for p in (ORDER_A if tab is SA else ORDER_B)}
    return [w for p in range(7) for w in ops[p]]


def _accumulate(acc, key, sign, v):
    if key not in acc:
        acc[key] = v
    else:
        acc[key] = acc[key] + v if sign > 0 else acc[key] - v


def _decode7(p, prods, out):
    inner = {}
    for r in range(7):
        for key, sign in SC[r]:
            _accumulate(inner, key, sign, prods[r])
    for (a, b), sign in SC[p]:
        for (i, j), v in inner.items():
            _accumulate(out, (2 * a + i, 2 * b + j), sign, v)


def _decode(prods, r0):
    out = {}
    for p in range(7):
        _decode7(p, [pltpu.bitcast(m[r0:r0 + 8, :], f32) for m in prods[7 * p:7 * p + 7]],
                 out)
    return out


def _rows(ref, rows):
    return jnp.concatenate([ref[c, rows, :] for c in range(ref.shape[0])], axis=1)


def _set_rows(ref, rows, v):
    for c in range(ref.shape[0]):
        ref[c, rows, :] = v[:, c * 128:(c + 1) * 128]


class _Side:
    def __init__(self, zero, slots, *jobs):
        self.zero = zero
        self.slots = slots
        self.jobs = [[job, count, 0] for job, count in jobs]
        self.at = 0

    def tie(self, w, r0=0, c0=0):
        self.at += 1
        head = old = w[r0:r0 + 8, c0:c0 + 128]
        for job in self.jobs:
            while job[2] * self.slots < min(self.at, self.slots) * job[1]:
                job[2] += 1
                for ref, idx in next(job[0]):
                    row = pl.ds(pl.multiple_of(idx[-1] + 8 * self.zero, 8), 8)
                    seen = ref[idx[:-1] + (row, pl.ds(0, 128))]
                    head = jnp.where(self.zero == 0, head, pltpu.bitcast(seen, u32))
        if head is old:
            return w
        row = [v for v in (w[r0:r0 + 8, :c0] if c0 else None, head,
                           w[r0:r0 + 8, c0 + 128:] if c0 + 128 < w.shape[1] else None)
               if v is not None]
        rows = (w[:r0] if r0 else None, jnp.concatenate(row, axis=1),
                w[r0 + 8:] if r0 + 8 < w.shape[0] else None)
        return jnp.concatenate([v for v in rows if v is not None], axis=0)

    def after(self, ref, r):
        spare = pl.multiple_of(ref.shape[-2] - 8 - 8 * self.zero, 8)
        lead = tuple(n - 1 - self.zero for n in ref.shape[:-2])
        ref[lead + (pl.ds(spare, 8), pl.ds(0, 128))] = pltpu.bitcast(r[:8, :128], ref.dtype)

    def finish(self):
        for job in self.jobs:
            for _ in job[0]:
                pass


def _ln_job(load, store, rows, group, mean_ref, rstd_ref, zero):
    wide = lambda ref, r, n, k: jnp.concatenate(
        [ref[pl.ds(pl.multiple_of(r + 8 * k * zero, 8), n), :]] * (D // 128), axis=1)
    if not group:
        for r in range(0, rows, 16):
            x = load(r, 16, 0)
            yield store(r, x, _ln(x))
        return
    for r in range(0, rows, group):
        m = jnp.mean(load(r, group, 0), axis=-1, keepdims=True)
        mean_ref[pl.ds(r, group), :] = jnp.broadcast_to(m, (group, 128))
        yield [(mean_ref, (r,))]
    for r in range(0, rows, group):
        d = load(r, group, 1) - wide(mean_ref, r, group, 1)
        v = jnp.mean(d * d, axis=-1, keepdims=True)
        rstd_ref[pl.ds(r, group), :] = jnp.broadcast_to(lax.rsqrt(v + EPS), (group, 128))
        yield [(rstd_ref, (r,))]
    for r in range(0, rows, 16):
        x = load(r, 16, 2)
        yield store(r, x, (x - wide(mean_ref, r, 16, 2)) * wide(rstd_ref, r, 16, 2))


def _kernel(x_hbm, mem0_ref, wq_hbm, wk_hbm, wv_hbm, wo_hbm, w1_hbm, w2_hbm,
            w3_hbm, w4_hbm, out_hbm,
            wo_b, xs, hbuf, xg, w1b, we, sems, fence_sem, *q_rings):
    w_hbm = (wq_hbm, wk_hbm, wv_hbm)
    q_r = [q_rings[h % 8].at[h // 8] for h in range(H)]

    x0_copy = pltpu.make_async_copy(x_hbm.at[pl.ds(0, X0)], xs.at[pl.ds(0, X0)],
                                    sems.at[SEM_X0])
    x_copy = pltpu.make_async_copy(x_hbm.at[pl.ds(X0, S - X0)], xs.at[pl.ds(X0, S - X0)],
                                   sems.at[SEM_X])

    def wo_copy(i):
        rows = pl.ds(_mult(i * 512, 512), 512)
        return pltpu.make_async_copy(wo_hbm.bitcast(u32).at[rows], wo_b.at[rows],
                                     sems.at[SEM_WO + i])

    def w1_copy(i):
        cols = pl.ds(_mult(i * C4, C4), C4)
        return pltpu.make_async_copy(w1_hbm.bitcast(u32).at[:, cols], w1b.at[i],
                                     sems.at[SEM_W1])

    w3_copies = [pltpu.make_async_copy(
        w3_hbm.bitcast(u32).at[:, pl.ds((4 * c + b) * 128, 128)],
        we.at[c, pl.ds(b * 512, 512)], sems.at[SEM_W3]) for c in range(NC) for b in range(4)]

    def w2_slot(p, j, r0=0, n=D // 4):
        return NC + p // 6, pl.ds(_mult(D * (p % 6) + D // 4 * j + r0, 8), n)

    def early_copies(j):
        return [pltpu.make_async_copy(
            w2_hbm.bitcast(u32).at[pl.ds(D // 4 * a, D // 4),
                                   pl.ds(_mult(D // 2 * b + 128 * j, 128), 128)],
            we.at[w2_slot(2 * a + b, j)], sems.at[SEM_W1]) for a, b in QUAD] + [
            pltpu.make_async_copy(
                w4_hbm.bitcast(u32).at[0, a, :, pl.ds(_mult(C4 * j + 128 * k, 128), 128)],
                we.at[NC + 2, pl.ds(_mult(128 * (4 * j + a) + 64 * k, 64), 64)],
                sems.at[SEM_W1]) for a in range(4) for k in range(2)]

    def fence():
        pl.semaphore_signal(fence_sem, 1)
        pl.semaphore_wait(fence_sem, 1)

    def block_a(wq_s, wk_s, wv_s, ubuf, tokbuf, lnbuf, *kv_rings):
        w_s = (wq_s, wk_s, wv_s)
        rings = tuple(q_rings) + tuple(kv_rings)
        ring = [[rings[m * 8 + h % 8].at[h // 8] for h in range(H)] for m in range(3)]
        k_r, v_r = ring[1:]

        stg = [we.at[m, pl.ds(0, 4 * D)] for m in range(3)]
        xe = [we.at[3, pl.ds(128 * p, 128)] for p in range(NP)]
        w_op = (hbuf, xg)

        def start_chunk(g, m):
            src = w_hbm[m].bitcast(u32)
            dst = stg[m].reshape(D // 2, 8, DH)
            for par in range(2):
                pltpu.make_async_copy(
                    src.at[:, pl.ds(_mult(16 * par + 4 * g, 4), 4), :],
                    dst.at[:, pl.ds(4 * par, 4), :],
                    sems.at[SEM_W + 3 * g + m]).start()

        def wait_chunk(g, m):
            pltpu.make_async_copy(stg[m], stg[m], sems.at[SEM_W + 3 * g + m]).wait()

        def encode_unit(g, m, half, slices):
            h0 = 8 * g + 4 * half
            for i0 in slices:
                blk = {}

                def get(k, a, b):
                    if (k, a, b) not in blk:
                        for par in range(2):
                            w = stg[m][pl.ds(8 * (128 * a + i0) + 4 * par + 2 * half + b // 2,
                                             8, stride=8), :]
                            for j in range(2):
                                blk[par, a, b - b % 2 + j] = _unzip(w, j)
                        for j in (b - b % 2, b - b % 2 + 1):
                            w_s[m][h0 + j, pl.ds(128 * a + i0, 8), :] = _zip(
                                blk[0, a, j], blk[1, a, j])
                    return blk[k, a, b]

                for p in ORDER_B:
                    known = len(blk)
                    for r, w in enumerate(_encode7(SB, p, get)):
                        q = 7 * p + r
                        if len(SB[p]) + len(SB[r]) > 2:
                            w_op[half][1 + q // 16, pl.ds(128 * (q % 16) + i0, 8), :] = (
                                pltpu.bitcast(w, f32))
                    yield [(w_op[half], (1, i0))] + [(w_s[m], (h0, i0))] * (len(blk) > known)

        def operand(g, m, half, q, zero):
            tp, tr = SB[q // 7], SB[q % 7]
            if len(tp) + len(tr) == 2:
                a, b = (2 * tp[0][n] + tr[0][n] for n in range(2))
                return w_s[m][8 * g + 4 * half + b, pl.ds(128 * a, 128), :]
            return w_op[half][1 + q // 16, pl.ds(
                pl.multiple_of(128 * (q % 16) + 8 * zero, 8), 128), :]

        def decode_unit(g, m, half, prods):
            for r0 in range(0, P0 // 4, 8):
                out = _decode(prods, r0)
                for i, j in QUAD:
                    for a, b in QUAD:
                        rings[8 * m + 4 * half + 2 * b + j][
                            g, pl.ds(P0 // 4 * (2 * a + i) + r0, 8), :] = out[2 * a + i, 2 * b + j]
                    yield [(rings[8 * m + 4 * half + 2 * b + j], (g, r0)) for b in range(2)]

        x0_copy.start()
        for m in range(3):
            start_chunk(0, m)
        x0_copy.wait()

        @pl.loop(0, P0 // 64)
        def _(s):
            for a in range(4):
                rows = pl.ds(pl.multiple_of(P0 // 4 * a + 16 * s, 16), 16)
                _set_rows(xg, rows, _ln(xs[rows, :].astype(f32)))
            for kt in range(2):
                ops = _encode(SA, lambda k, a, b: xg[
                    2 * b + kt, pl.ds(P0 // 4 * a + 16 * s + k, 8, stride=2), :])
                for p, w in enumerate(ops):
                    xe[p][pl.ds(pl.multiple_of(64 * kt + 8 * s, 8), 8), :] = w

        tokbuf[...] = _ln(xs[pl.ds(P0, UNROLL * TOK), :].astype(f32))
        wait_chunk(0, 0)

        @pl.loop(0, 16)
        def _(i):
            list(encode_unit(0, 0, 0, [pl.multiple_of(8 * i, 8)]))

        last = [we.at[4, pl.ds(128 * p, 128)] for p in range(NP)]

        @pl.loop(0, 4)
        def _(g):
            g1 = jnp.minimum(g + 1, 3)
            zero = g >> 2
            jobs = [(decode_unit((g + 3) & 3, 2, 1, last), 64)]
            for m in range(3):
                for half in range(2):
                    nxt = (g1, 0, 0) if (m, half) == (2, 1) else (g, m + half, 1 - half)
                    side = _Side(zero, (NP - PRO_AT - 1) * PRO_K,
                                 (encode_unit(*nxt, range(0, 128, 8)), 16 * 7), *jobs)
                    prods = []
                    for p in range(NP):
                        lhs = jnp.concatenate(
                            [xe[p][pl.ds(64 * kt, 64), :] for kt in range(2)], axis=1)
                        rhs = operand(g, m, half, p, zero)
                        if p > PRO_AT:
                            for k in range(PRO_K):
                                lhs = side.tie(lhs, 64 // PRO_K * k)
                        prods.append(_dot(_unpack(lhs), _unpack(rhs)))
                        if half == 0 and m > 0 and p == PRO_BAR:
                            fence()
                            if m == 1:
                                w1_copy(g).start()
                                for cp in early_copies(g):
                                    cp.start()
                            else:
                                wo_copy(g).start()
                        if half == 1 and p == PRO_BAR:
                            if m < 2:
                                wait_chunk(g, m + 1)
                            else:
                                pl.when(g < 3)(functools.partial(wait_chunk, g1, 0))
                            pl.when(g < 3)(functools.partial(start_chunk, g1, m))
                    jobs = [(decode_unit(g, m, half, prods), 64)]
            for p in range(NP):
                we[4, pl.ds(128 * p, 128), :] = pltpu.bitcast(prods[p], u32)

        list(decode_unit(3, 2, 1, last))

        x_copy.start()
        _set_rows(xg, pl.ds(0, HALO), jnp.zeros((HALO, D), f32))
        _set_rows(xg, pl.ds(HALO + S, HALO), jnp.zeros((HALO, D), f32))
        _set_rows(hbuf, pl.ds(0, UNROLL * TOK), jnp.zeros((UNROLL * TOK, D), f32))
        ubuf[...] = jnp.zeros(ubuf.shape, u32)
        for cp in w3_copies:
            cp.start()
        for i in range(4):
            for cp in [w1_copy(i)] + early_copies(i):
                cp.wait()
        for i in range(4):
            wo_copy(i).wait()

        def wrap(r):
            return jnp.where(r >= RING, r - RING, r)

        def step(s, carry, tok, side):
            mem, rp, ra, rw = carry
            ri = lax.broadcasted_iota(jnp.int32, (2 * MEM + SEG, 2 * L), 0)
            ci = lax.broadcasted_iota(jnp.int32, (2 * MEM + SEG, 2 * L), 1)
            key_b = ((ci >= MEM) & (ci < 2 * MEM)) | (ci >= 2 * MEM + SEG)
            same = key_b == ((ri >= MEM) & (ri < 2 * MEM))
            mask = same & ((ri < 2 * MEM) | (ri >= ci))
            fill = jnp.where(same, NEG, -jnp.inf)

            lhs = jnp.concatenate([mem, tok], axis=0).astype(bf16)
            rps = [pl.multiple_of(wrap(rp + 8 * i), 8) for i in range(3)]
            ra_ = pl.multiple_of(ra, SEG)
            rw_ = pl.multiple_of(rw, 8)

            col = s & 3
            group = jnp.maximum((s >> 2) - 1, 0)
            rb = pl.multiple_of(group * (4 * TOK), 8)

            def filler(j):
                u = ubuf[pl.ds(pl.multiple_of((group & 1) * (2 * TOK), 8), 2 * TOK), :]
                r = _dot(_unpack(u), _unpack(w1b[col, :, pl.ds(j * 128, 128)]))
                xg[2 * col + j, pl.ds(HALO + rb, 4 * TOK), :] = _gelu(r)

            mem_qkv = {}
            scores = {}
            o_mem = {}
            total = [None]

            def qkv(h):
                for m in range(3):
                    w = w_s[m][h]
                    for r0 in SIDE_R if h >= SIDE_AT else ():
                        w = side.tie(w, r0)
                    r = _dot(lhs, _unpack(w))
                    for i in range(3):
                        ring[m][h][pl.ds(rps[i], 8), :] = r[8 + 8 * i:16 + 8 * i]
                    mem_qkv[m, h] = r[:MEM]

            def segment(m, pair):
                a, b = 2 * pair, 2 * pair + 1
                ma, mb = mem_qkv.pop((m, a)), mem_qkv.pop((m, b))
                xa, xb = (ring[m][h][pl.ds(ra_, SEG), :] for h in (a, b))
                if m == 0:
                    parts = ((ma, mb, xa), (xb,))
                else:
                    parts = ((ma, mb, xa, xb), (mb, ma, xb))
                return [jnp.concatenate(v, axis=0).astype(bf16) for v in parts]

            def qk(pair):
                q, k = segment(0, pair), segment(1, pair)
                for n in (pair % 2, 1 - pair % 2):
                    scores[pair, n] = lax.dot_general(
                        q[n], k[n], (((1,), (1,)), ((), ())), preferred_element_type=f32)

            def pv(pair):
                v = segment(2, pair)
                for n in (pair % 2, 1 - pair % 2):
                    sc = scores.pop((pair, n)) * (DH ** -0.5)
                    if n == 0:
                        sc = jnp.where(mask, sc, fill)
                    else:
                        sc = jnp.where(mask[2 * MEM:, :2 * MEM + SEG], sc,
                                       fill[2 * MEM:, :2 * MEM + SEG])
                    mx = jnp.max(sc, axis=1, keepdims=True)
                    e = jnp.exp(sc - mx)
                    den = jnp.sum(e, axis=1, keepdims=True)
                    inv = pl.reciprocal(den, approx=True)
                    inv = inv * (2.0 - den * inv)
                    o = _dot(e.astype(bf16), v[n]) * inv
                    q_r[2 * pair + n][pl.ds(ra_, SEG), :] = o[-SEG:]
                    if n == 0:
                        o_mem[2 * pair], o_mem[2 * pair + 1] = o[:MEM], o[MEM:2 * MEM]

            def wo(h):
                lo = jnp.concatenate([o_mem.pop(h), q_r[h][pl.ds(rw_, TOK), :]],
                                     axis=0).astype(bf16)
                r = _dot(lo, _unpack(wo_b[pl.ds(h * DH // 2, DH // 2), :]))
                total[0] = r if total[0] is None else total[0] + r

            npair = H // 2
            for t in range(npair + LAG_WO):
                if 0 <= t - LAG_QK < npair:
                    qk(t - LAG_QK)
                if 0 <= t - LAG_PV < npair:
                    pv(t - LAG_PV)
                if t < npair:
                    qkv(2 * t)
                    qkv(2 * t + 1)
                if t == FILL_AT:
                    filler(0)
                if 0 <= t - LAG_WO < npair:
                    wo(2 * (t - LAG_WO))
                    wo(2 * (t - LAG_WO) + 1)
            filler(1)

            a = total[0]
            return (a[:MEM], wrap(rp + TOK), wrap(ra + SEG), wrap(rw + TOK)), a[MEM:]

        def steps(i, carry):
            n = UNROLL * TOK
            pl.when(i == 1)(x_copy.wait)

            @pl.when(i == 16 // ENC)
            def _():
                for cp in w3_copies:
                    cp.wait()

            zero = i >> 5

            def norm_filler():
                prev = jnp.maximum(i - 1, 0)
                for r in range(0, n, LN_ROWS):
                    rows = pl.ds(pl.multiple_of(n * prev + r, 8), LN_ROWS)
                    lnbuf[pl.ds(r, LN_ROWS), :] = _ln(_rows(hbuf, rows))
                    yield [(lnbuf, (r,))]
                for r in range(0, n, LN_ROWS):
                    rows = pl.ds(pl.multiple_of(r + 16 * zero, 8), LN_ROWS)
                    dst = pl.multiple_of((n * (prev & 3) + r) // 2, 8)
                    ubuf[pl.ds(dst, LN_ROWS // 2), :] = _pack(_ln(lnbuf[rows, :]))
                    yield [(ubuf, (dst,))]

            def norm_tokens():
                nxt = jnp.minimum(P0 + n * (i + 1), S - n)
                for r in range(0, n, 16):
                    rows = pl.ds(pl.multiple_of(nxt + r, 16), 16)
                    tokbuf[pl.ds(r, 16), :] = _ln(xs[rows, :].astype(f32))
                    yield [(tokbuf, (r,))]

            def encode_w23():
                for j in range(4):
                    raw = {(a, b): we[w2_slot(2 * a + b, j, 8 * i, 8)] for a, b in QUAD}
                    get = functools.cache(lambda k, a, b: _unzip(raw[a, b], k))
                    for p in range(7):
                        we[w2_slot(p, j, 8 * i, 8)] = _zip(
                            *[_combine(functools.partial(get, k), SB[p]) for k in range(2)])
                    yield [(we, (NC, 8 * i))]
                for k in range(ENC):
                    j = ENC * i + k
                    grp, i0 = jnp.where(j < 16, NC + 2, (j >> 4) - 1), 8 * (j & 15)
                    slot = lambda q: (grp, pl.ds(pl.multiple_of(128 * q + i0, 8), 8))
                    raw = {(a, b): we[slot(4 * b + a)] for a in range(4) for b in range(4)}
                    get = functools.cache(lambda k, a, b: _unzip(raw[a, b], k))
                    for p in ORDER_B:
                        for r, w in enumerate(_encode7(SB, p, get)):
                            we[slot(7 * p + r)] = w
                        yield [(we, (grp, i0))]

            jobs = [[(norm_filler(), 2 * n // LN_ROWS)],
                    [(encode_w23(), 4 + 7 * ENC), (norm_tokens(), n // 16)]]
            for k in range(UNROLL):
                s = i * UNROLL + k
                carry, o = step(s, carry, tokbuf[pl.ds(k * TOK, TOK), :],
                                _Side(zero, SIDE_N * len(SIDE_R), *jobs[k]))
                lo = k * TOK // 16 * 16
                xv = xs[pl.ds(pl.multiple_of(n * i + lo, 16), 32), :].astype(f32)
                _set_rows(hbuf, pl.ds(pl.multiple_of(TOK * s, 8), TOK),
                          xv[k * TOK - lo:(k + 1) * TOK - lo] + o)
            return carry

        carry = (mem0_ref[...].astype(f32), jnp.int32(P0), jnp.int32(0), jnp.int32(0))
        carry = lax.fori_loop(0, NSEG // UNROLL, steps, carry)
        return carry[1] >> 16

    zero = pl.run_scoped(
        block_a,
        *[pltpu.VMEM((H, D // 2, DH), u32)] * 3,
        pltpu.VMEM((4 * TOK, D), u32),
        pltpu.VMEM((UNROLL * TOK, D), f32),
        pltpu.VMEM((UNROLL * TOK, D), f32),
        *[pltpu.VMEM((H // 8, RING, DH), f32)] * 16,
    )

    def tail(w4e, ye, ybuf, ue, *bufs):
        woe, pool, stats = bufs[:3], bufs[3:11], bufs[11:]
        w4_copies = [
            pltpu.make_async_copy(w4_hbm.bitcast(u32).at[pl.ds(1, NC - 1), a, :, pl.ds(b * C4, C4)],
                                  w4e.at[4 * a + b], sems.at[SEM_W4])
            for a in range(4) for b in range(4)]
        for cp in w4_copies:
            cp.start()
        done = TOK * NSEG
        first = 4 * TOK * (NSEG // 4 - 1)

        def later(rows, n):
            return pl.ds(pl.multiple_of(rows + 8 * zero, 8), n)

        def run(dots, ties, start, *jobs):
            side = _Side(zero, (len(dots) - max(start, 0)) * len(ties), *jobs)
            prods = []
            for load in dots:
                if len(prods) == start:
                    fence()
                lhs, rhs = load()
                for r0, c0 in ties if len(prods) >= start else ():
                    lhs = side.tie(lhs, r0, c0)
                prods.append(_dot(_unpack(lhs), _unpack(rhs)))
            return prods

        hk, hn, hm = H * DH // 4, D // 2, P0 // 2

        def wo_op(p, j):
            if p == 3:
                return pool[j], 0, 0
            if p in (1, 4):
                return wo_b, hk * (p // 4), hn * (p // 4) + C4 * j
            return woe[{0: 0, 2: 1, 5: 2, 6: 0}[p]], 0, C4 * j

        def encode_wo(ps):
            for i0 in range(0, hk, 8):
                for j in range(2):
                    get = functools.cache(lambda k, a, b: _unzip(wo_b[
                        later(hk * a + i0 + 8 * ps[0] * zero, 8), pl.ds(hn * b + C4 * j, C4)], k))
                    ops = [_zip(*[_combine(functools.partial(get, k), SB[p]) for k in range(2)])
                           for p in ps]
                    for p, w in zip(ps, ops):
                        ref, r0, c0 = wo_op(p, j)
                        ref[pl.ds(r0 + i0, 8), pl.ds(c0, C4)] = w
                    yield [(wo_op(p, j)[0], (0,)) for p in ps]

        def encode_o(n):
            for kt in range(H // 2):
                for s in range(hm // 16):
                    pool[n][pl.ds(hm // 2 * (kt // 2) + 8 * s, 8), pl.ds(kt % 2 * 128, 128)] = (
                        _zip(*[_combine(
                            lambda a, b: q_r[H // 2 * b + kt][pl.ds(
                                (done + hm * a + 16 * s) % RING + k + n * zero, 8, stride=2), :],
                            SA[ORDER_B[n]]) for k in range(2)]))
                    if s % 4 == 3:
                        yield [(pool[n], (0,))]

        def wo_dots(n):
            def load(j, i):
                ref, r0, c0 = wo_op(ORDER_B[n], j)
                lhs = [pool[n][later(hm // 2 * c + hm // 4 * i + 8 * j * zero, hm // 4), :]
                       for c in range(8)]
                return (jnp.concatenate(lhs, axis=1),
                        ref[later(r0 + 8 * i * zero, hk), pl.ds(c0, C4)])
            return [functools.partial(load, j, i) for j, i in QUAD]

        def decode_wo(n, prods):
            for (j, i), v in zip(QUAD, prods):
                for r in range(0, hm // 2, 16):
                    for (a, b), sign in SC[ORDER_B[n]]:
                        fresh = all(key != (a, b) for q in ORDER_B[:n] for key, _ in SC[q])
                        row = done + hm * a + hm // 2 * i + r
                        for k in range(2):
                            c = 4 * b + 2 * j + k
                            old = (xs[pl.ds(row, 16), pl.ds(128 * c, 128)].astype(f32) if fresh
                                   else hbuf[c, later(row + 8 * n * zero, 16), :])
                            new = v[r:r + 16, 128 * k:128 * (k + 1)]
                            hbuf[c, pl.ds(row, 16), :] = old + new if sign > 0 else old - new
                    yield [(hbuf, (0, 0))]

        hsb = wo_b

        def norm_in():
            def first_norm(r, x, y):
                woe[2][pl.ds(r, 16), :] = pltpu.bitcast(y[:, :hn], u32)
                woe[2][pl.ds(P0 + r, 16), :] = pltpu.bitcast(y[:, hn:], u32)
                return [(woe[2], (r,))]

            def second_norm(r, x, y):
                ue[pl.ds(r // 2, 8), :] = _pack(y)
                return [(ue, (0,))]

            yield from _ln_job(
                lambda r, n, k: _rows(hbuf, later(done + r + 8 * (7 + k) * zero, n)),
                first_norm, P0, NORM_ROWS, *stats[:2], zero)
            yield from _ln_job(
                lambda r, n, k: pltpu.bitcast(jnp.concatenate(
                    [woe[2][later(r0 + r + 8 * k * zero, n), :] for r0 in (0, P0)], axis=1), f32),
                second_norm, P0, NORM_ROWS, *stats[2:], zero)

        def in_dots(lhs, cols, n=0):
            return [lambda c=c: (lhs(c), w1b[c // 2, later(8 * n * zero, D // 2),
                                             pl.ds(128 * (c % 2), 128)]) for c in cols]

        def gelu_in(r0, cols, prods):
            for c, v in zip(cols, prods):
                for r in range(0, v.shape[0], 32):
                    xg[c, pl.ds(HALO + r0 + r, 32), :] = _gelu(v[r:r + 32])
                    yield [(xg, (c, HALO + r0))]

        def encode_g(i):
            for s in range(RB // 32):
                for kt in range(4):
                    get = functools.cache(lambda k, a, b: xg[4 * b + kt, pl.ds(
                        HALO + i * RB + RB // 2 * a + 16 * s + k + SHIFT[2 * b + kt // 2],
                        8, stride=2), :])
                    for p in range(7):
                        pool[i - 1][pl.ds(128 * p + 64 * (kt // 2) + 8 * s, 8),
                                    pl.ds(128 * (kt % 2), 128)] = _zip(
                            *[_combine(functools.partial(get, k), SA[p]) for k in range(2)])
                    yield [(pool[i - 1], (0,))]

        def out_dots(i, j):
            return [lambda p=p: (
                jnp.concatenate([pool[i - 1][later(128 * p + 64 * k + 8 * j * zero, 64), :]
                                 for k in range(2)], axis=1),
                we[w2_slot(p, j, 8 * (i + 1) * zero)]) for p in range(7)]

        def decode_out(i, j, prods):
            for r0 in range(0, RB // 2, 8):
                out = {}
                for p in range(7):
                    for key, sign in SC[p]:
                        _accumulate(out, key, sign, prods[p][r0:r0 + 8])
                for (a, b), v in out.items():
                    hsb[pl.ds(i * RB + RB // 2 * a + r0, 8),
                        pl.ds(hn * b + 128 * j, 128)] = pltpu.bitcast(v, u32)
                yield [(hsb, (i * RB,))]

        def encode_w4():
            for c in range(NC - 1):
                for i0 in range(0, 64, 8):
                    for j in range(2):
                        at = (c, pl.ds(i0, 8), pl.ds(128 * j, 128))
                        raw = {(a, b): w4e[(4 * a + b,) + at]
                               for a in range(4) for b in range(4)}
                        get = functools.cache(lambda k, a, b: _unzip(raw[a, b], k))
                        for p in ORDER_B:
                            for r, w in enumerate(_encode7(SB, p, get)):
                                w4e[(7 * p + r,) + at] = w
                            yield [(w4e, (0, c, i0))]

        def mixer_post(r0, zero, group):
            def first_norm(r, hv, y):
                rows = pl.ds(_mult(r0 + r, 8), 16)
                x1 = y + pltpu.bitcast(hsb[rows, :], f32)
                _set_rows(xg, rows, hv + x1)
                _set_rows(ybuf, pl.ds(r, 16), x1)
                return [(ybuf, (0, 0)), (xg, (0, r0))]

            def second_norm(r, x1, y):
                _set_rows(hbuf, pl.ds(_mult(r0 + r, 8), 16), y)
                return [(hbuf, (0, r0))]

            at = lambda r, n, k: pl.ds(pl.multiple_of(r + 8 * k * zero, 8), n)
            yield from _ln_job(lambda r, n, k: _rows(hbuf, at(r0 + r, n, k)),
                               first_norm, RB, group, *stats[:2], zero)
            yield from _ln_job(lambda r, n, k: _rows(ybuf, at(r, n, k + 1)),
                               second_norm, RB, group, *stats[2:], zero)
            for s in range(4):
                for kt in range(2):
                    get = functools.cache(lambda k, a, b: hbuf[2 * b + kt, pl.ds(
                        r0 + R4 * a + 4 * k + s, 8, stride=8), :])
                    for p in ORDER_A:
                        for r, w in enumerate(_encode7(SA, p, get)):
                            ye[7 * p + r, pl.ds(8 * s, 8), pl.ds(128 * kt, 128)] = w
                        if p in POST_P:
                            yield [(ye, (0, 8 * s))]

        def out_copies(i):
            rows = pl.ds(_mult(i * (RB // 2), RB // 2), RB // 2)
            return [pltpu.make_async_copy(
                woe[b].at[rows], out_hbm.bitcast(u32).at[rows, pl.ds(hn * b, hn)],
                sems.at[SEM_OUT + 2 * i + b]) for b in range(2)]

        n_g, n_out, n_o = RB // 8, RB // 16, H // 2 * hm // 64
        n_post = RB // 8 + 8 * len(POST_P)
        out_ties = [(r0, 0) for r0 in range(0, 64, 8)]
        wo_ties = [(r0, c0) for c0 in range(0, 2 * D, 512) for r0 in range(0, 64, 8)]
        in_ties = [(r0, c0) for c0 in (0, 512) for r0 in range(0, 64, 8)]
        w4_job = encode_w4()
        wo_jobs = [encode_wo(ps) for ps in ((0,), (2, 5), (3, 6))]

        def mixer_out(i, pending, *jobs):
            for j in range(4):
                prods = run(out_dots(i, j), out_ties, FENCE[1] if j in FENCE_J else -1, pending,
                            *[(job, count // 4) for job, count in jobs])
                pending = (decode_out(i, j, prods), n_out)
            return pending

        pending = (encode_o(0), n_o)
        list(pending[0])
        for n in range(7):
            jobs = [(encode_o(n + 1), n_o) if n < 6 else (encode_g(0), n_g)]
            if n:
                jobs.append(pending)
            if n < 5:
                jobs.append((wo_jobs[(n + 1) // 2], hk // 8 if n else hk // 4))
            if n == W4_AT:
                for cp in w4_copies:
                    cp.wait()
            if n >= W4_AT:
                jobs.append((w4_job, 7 * W4_SPLIT[8]))
            prods = run(wo_dots(n), wo_ties, FENCE[0] if n else -1, *jobs)
            pending = (decode_wo(n, prods), hm // 8)
        u = _pack(_ln(_ln(_rows(hbuf, pl.ds(first, done - first)))))
        prods = run(in_dots(lambda c: u, range(8)), in_ties[:6], FENCE[0], pending)
        pending = (gelu_in(first, range(8), prods), 24)
        norm = norm_in()
        for i in range(5):
            jobs = [(w4_job, 7 * W4_SPLIT[i])]
            if i < 4:
                jobs.append((encode_g(i + 1), n_g))
            if i > 0:
                jobs.append((norm, P0 // NORM_ROWS + P0 // 32))
            pending = mixer_out(i, pending, *jobs)
        post, g5 = mixer_post(0, zero, NORM_ROWS), encode_g(5)
        for n in range(8):
            r0, cols = done + n // 2 * 128, range(n % 2 * 4, n % 2 * 4 + 4)
            jobs = [pending, (w4_job, 7 * W4_SPLIT[9])]
            jobs.append((post, (n_post + 4 * RB // NORM_ROWS) // 8))
            if n >= 6:
                jobs.append((g5, n_g // 2))
            prods = run(in_dots(
                lambda c: ue[later((r0 - done) // 2 + 8 * c * zero, 64), :], cols, n + 1),
                in_ties, FENCE[2] if n % 2 == 0 else -1, *jobs)
            pending = (gelu_in(r0, cols, prods), RB // 16)
        for i in range(5, 8):
            jobs = [(w4_job, 7 * W4_SPLIT[i])]
            if i < 7:
                jobs.append((encode_g(i + 1), n_g))
            pending = mixer_out(i, pending, *jobs)
        list(pending[0])
        list(w4_job)

        def mlp_block(i, carry):
            te = []
            for c in range(NC):
                prods = [_dot(_unpack(ye[p]), _unpack(we[c, pl.ds(128 * p, 128), :]))
                         for p in range(NP)]
                ops = []
                for s in range(R4 // 16):
                    act = [{key: _gelu(v) for key, v in _decode(
                        prods, 32 * k + 8 * s).items()}
                        for k in range(2)]
                    ops.append(_encode(SA, lambda k, a, b: act[k][a, b]))
                te.append([jnp.concatenate([o[p] for o in ops], axis=0) for p in range(NP)])

            def down(p, lo, hi, tie=lambda w: w):
                lhs = jnp.concatenate([tie(te[c][p]) if c in POST_C else te[c][p]
                                       for c in range(lo, hi)], axis=1)
                rhs = [w4e[p, c - 1] if c else jnp.concatenate(
                    [we[NC + 2, pl.ds(128 * p + 64 * k, 64), :] for k in range(2)], axis=1)
                    for c in range(lo, hi)]
                return _dot(_unpack(lhs), _unpack(jnp.concatenate(rhs, axis=0)))

            prods = [down(p, 0, KSPLIT) for p in range(NSPLIT)]
            prods = [m + down(p, KSPLIT, NC) for p, m in enumerate(prods)]
            out = {}

            def finish(qa, qb):
                for a, b in ((2 * qa + n // 2, 2 * qb + n % 2) for n in range(4)):
                    for r in range(0, R4, 16):
                        row = i * RB + R4 * a + r
                        for j in range(2):
                            woe[qb][pl.ds(pl.multiple_of(row // 2, 8), 8),
                                    pl.ds(C4 * (b % 2) + 128 * j, 128)] = _zip(*[
                                        out[a, b][32 * k + r // 2:32 * k + r // 2 + 8,
                                                  128 * j:128 * (j + 1)]
                                        + xg[2 * b + j, pl.ds(row + k, 8, stride=2), :]
                                        for k in range(2)])
                        yield [(woe[qb], (i * (RB // 2),))]

            side = _Side(i >> 3, POST_N * len(POST_C),
                         (mixer_post(((i + 1) & 7) * RB, i >> 3, 0), n_post))
            for p in range(7):
                done_quad = {4: (1, 0), 5: (0, 1), 6: (1, 1)}.get(p)
                store = _Side(i >> 3, 16, *([(finish(*done_quad), 16)] if done_quad else []))
                for q in range(len(prods), 7 * p + 7):
                    side.after(hbuf, prods[q - POST_LAG])
                    prods.append(down(q, 0, NC, side.tie if q % 7 == 0 else
                                      lambda w: store.tie(side.tie(w))))
                _decode7(p, prods[7 * p:7 * p + 7], out)
            list(finish(0, 0))
            for cp in out_copies(i):
                cp.start()
            return carry

        lax.fori_loop(0, S // RB, mlp_block, 0)
        for i in range(S // RB):
            for cp in out_copies(i):
                cp.wait()

    pl.run_scoped(
        tail,
        pltpu.VMEM((NP, NC - 1, 64, C4), u32),
        pltpu.VMEM((NP, R4 // 2, C4), u32),
        pltpu.VMEM((D // 128, RB, 128), f32),
        pltpu.VMEM((P0 // 2, D), u32),
        *[pltpu.VMEM((H * DH // 4, D // 2), u32)] * 3,
        *[pltpu.VMEM((D, C4), u32)] * 8,
        *[pltpu.VMEM((P0, 128), f32)] * 4,
    )


@jax.jit
def pallas_sequential_preLN__memory_aug_recurrent_mem_tr__mixer_s_mlp__prompt_kernel(
    A_x: jax.Array,
    A_mem0: jax.Array,
    A_Wq: jax.Array,
    A_Wk: jax.Array,
    A_Wv: jax.Array,
    A_Wo: jax.Array,
    A_seg_len: jax.Array,
    B_x: jax.Array,
    B_w1: jax.Array,
    B_w2: jax.Array,
    B_w3: jax.Array,
    B_w4: jax.Array,
):
    del A_seg_len, B_x
    hbm = pl.BlockSpec(memory_space=pl.ANY)
    vmem = pl.BlockSpec(memory_space=pltpu.VMEM)
    scratch = [
        pltpu.VMEM((H * DH // 2, D), u32),
        pltpu.VMEM((S, D), bf16),
        pltpu.VMEM((D // 128, S + 8, 128), f32),
        pltpu.VMEM((D // 128, S + 2 * HALO, 128), f32),
        pltpu.VMEM((4, D // 2, C4), u32),
        pltpu.VMEM((NC + 3, NP * 128, 128), u32),
        pltpu.SemaphoreType.DMA((NSEM,)),
        pltpu.SemaphoreType.REGULAR,
    ] + [pltpu.VMEM((H // 8, RING, DH), f32)] * 8
    out = pl.pallas_call(
        _kernel,
        out_shape=jax.ShapeDtypeStruct((S, D), A_x.dtype),
        in_specs=[hbm, vmem] + [hbm] * 8,
        out_specs=hbm,
        scratch_shapes=scratch,
        compiler_params=pltpu.CompilerParams(vmem_limit_bytes=VMEM_LIMIT),
    )(A_x.reshape(S, D), A_mem0.reshape(MEM, D),
      A_Wq.reshape(D // 2, 2 * H, DH), A_Wk.reshape(D // 2, 2 * H, DH),
      A_Wv.reshape(D // 2, 2 * H, DH),
      A_Wo.reshape(H * DH, D), B_w1, B_w2, B_w3, B_w4.reshape(NC, 4, 128, D))
    return out.reshape(A_x.shape)
```

```python
import functools

import jax
import jax.numpy as jnp
from jax import lax
import jax.experimental.pallas as pl
import jax.experimental.pallas.tpu as pltpu

S = 2048
D = 1024
H = 32
DH = 128
MEM = 8
SEG = 32
F = 3584
NSEG = S // SEG
L = MEM + SEG
TOK = 24
P0 = S - TOK * NSEG
RING = 576
X0 = P0 + 128
C4 = D // 4
SHIFT = (-1, 1, -2, 2)
HALO = 8
RB = 256
R4 = RB // 4
NC = F // 512
NP = 49
EPS = 1e-5
NEG = -1000000000.0

LAG_QK, LAG_PV, LAG_WO = 2, 4, 6
FILL_AT = 20
UNROLL = 2
ENC = 4
VMEM_LIMIT = 127 * 1024 * 1024 + 896 * 1024
SIDE_R = (256,)
CH_GROUP = 0
LN_UNROLL = 2
W_UNROLL = 4
SIDE_AT = 6
SIDE_N = 48
NSPLIT = 5
KSPLIT = 5
POST_C = (1, 3, 5)
PRO_AT = 1
PRO_N = 384
PRO_C = 128
TIE_C = 384
FENCE_I = (0, 1, 2, 3, 4, 5, 6, 7)
FENCE = (0, 0, -1)
NORM_ROWS = 32
POST_N = 44
UP_ROWS = 32
POST_LAG = 5
POST_P = (0, 6, 5)
W4_SPLIT = (12, 4, 4, 4, 4, 12, 12, 16, 14, 0)
W4_AT = 5

bf16 = jnp.bfloat16
f32 = jnp.float32
u32 = jnp.uint32

SEM_X0, SEM_X, SEM_W1, SEM_W3, SEM_W4, SEM_WO, SEM_OUT, SEM_W = 0, 3, 4, 5, 6, 7, 11, 27
NSEM = SEM_W + 6

SA = (((0, 0), 1, (1, 1)), ((1, 0), 1, (1, 1)), ((0, 0),), ((1, 1),),
      ((0, 0), 1, (0, 1)), ((1, 0), -1, (0, 0)), ((0, 1), -1, (1, 1)))
SB = (((0, 0), 1, (1, 1)), ((0, 0),), ((0, 1), -1, (1, 1)), ((1, 0), -1, (0, 0)),
      ((1, 1),), ((0, 0), 1, (0, 1)), ((1, 0), 1, (1, 1)))
SC = ((((0, 0), 1), ((1, 1), 1)), (((1, 0), 1), ((1, 1), -1)),
      (((0, 1), 1), ((1, 1), 1)), (((0, 0), 1), ((1, 0), 1)),
      (((0, 0), -1), ((0, 1), 1)), (((1, 1), 1),), (((0, 0), 1),))
ORDER_A = (2, 3, 0, 4, 6, 1, 5)
ORDER_B = (1, 4, 0, 2, 5, 3, 6)
QUAD = ((0, 0), (0, 1), (1, 0), (1, 1))


def _mult(i, n):
    return i if isinstance(i, int) else pl.multiple_of(i, n)


def _ln(x):
    m = jnp.mean(x, axis=-1, keepdims=True)
    d = x - m
    v = jnp.mean(d * d, axis=-1, keepdims=True)
    return d * lax.rsqrt(v + EPS)


def _gelu2(x):
    c = 0.7978845608028654
    return x * jnp.tanh(x * (c + c * 0.044715 * (x * x))) + x


def _gelu(x):
    return 0.5 * _gelu2(x)


def _pack(x):
    return pltpu.bitcast(x.astype(bf16), u32)


def _unpack(x):
    return pltpu.bitcast(x, bf16)


def _dot(a, b):
    return jnp.dot(a, b, preferred_element_type=f32)


def _zip(even, odd):
    return pltpu.bitcast(pltpu.pack_elementwise([even, odd], packed_dtype=bf16), u32)


def _unzip(w, k):
    return pltpu.unpack_elementwise(w, index=k, packed_dtype=bf16, unpacked_dtype=f32)


def _combine(get, term):
    if len(term) == 1:
        return get(*term[0])
    a, b = get(*term[0]), get(*term[2])
    return a + b if term[1] > 0 else a - b


def _encode7(tab, p, get):
    outer = [{(i, j): _combine(lambda a, b: get(k, 2 * a + i, 2 * b + j), tab[p])
              for i, j in QUAD} for k in range(2)]
    return [_zip(*[_combine(lambda a, b: o[a, b], tab[r]) for o in outer])
            for r in range(7)]


def _encode(tab, get):
    get = functools.cache(get)
    ops = {p: _encode7(tab, p, get) for p in (ORDER_A if tab is SA else ORDER_B)}
    return [w for p in range(7) for w in ops[p]]


def _accumulate(acc, key, sign, v):
    if key not in acc:
        acc[key] = v
    else:
        acc[key] = acc[key] + v if sign > 0 else acc[key] - v


def _decode7(p, prods, out):
    inner = {}
    for r in range(7):
        for key, sign in SC[r]:
            _accumulate(inner, key, sign, prods[r])
    for (a, b), sign in SC[p]:
        for (i, j), v in inner.items():
            _accumulate(out, (2 * a + i, 2 * b + j), sign, v)


def _decode(prods, r0):
    out = {}
    for p in range(7):
        _decode7(p, [pltpu.bitcast(m[r0:r0 + 8, :], f32) for m in prods[7 * p:7 * p + 7]],
                 out)
    return out


def _rows(ref, rows):
    return jnp.concatenate([ref[c, rows, :] for c in range(ref.shape[0])], axis=1)


def _set_rows(ref, rows, v):
    for c in range(ref.shape[0]):
        ref[c, rows, :] = v[:, c * 128:(c + 1) * 128]


class _Side:
    def __init__(self, zero, slots, *jobs):
        self.zero = zero
        self.slots = slots
        self.jobs = [[job, count, 0] for job, count in jobs]
        self.at = 0

    def tie(self, w, r0=0, c0=0):
        self.at += 1
        head = old = w[r0:r0 + 8, c0:c0 + 128]
        for job in self.jobs:
            while job[2] * self.slots < min(self.at, self.slots) * job[1]:
                job[2] += 1
                for ref, idx in next(job[0]):
                    row = pl.ds(pl.multiple_of(idx[-1] + 8 * self.zero, 8), 8)
                    seen = ref[idx[:-1] + (row, pl.ds(0, 128))]
                    head = jnp.where(self.zero == 0, head, pltpu.bitcast(seen, u32))
        if head is old:
            return w
        row = [v for v in (w[r0:r0 + 8, :c0] if c0 else None, head,
                           w[r0:r0 + 8, c0 + 128:] if c0 + 128 < w.shape[1] else None)
               if v is not None]
        rows = (w[:r0] if r0 else None, jnp.concatenate(row, axis=1),
                w[r0 + 8:] if r0 + 8 < w.shape[0] else None)
        return jnp.concatenate([v for v in rows if v is not None], axis=0)

    def after(self, ref, r):
        spare = pl.multiple_of(ref.shape[-2] - 8 - 8 * self.zero, 8)
        lead = tuple(n - 1 - self.zero for n in ref.shape[:-2])
        ref[lead + (pl.ds(spare, 8), pl.ds(0, 128))] = pltpu.bitcast(r[:8, :128], ref.dtype)

    def finish(self):
        for job in self.jobs:
            for _ in job[0]:
                pass


def _ln_job(load, store, rows, group, mean_ref, rstd_ref, zero):
    wide = lambda ref, r, n, k: jnp.concatenate(
        [ref[pl.ds(pl.multiple_of(r + 8 * k * zero, 8), n), :]] * (D // 128), axis=1)
    if not group:
        for r in range(0, rows, 16):
            x = load(r, 16, 0)
            yield store(r, x, _ln(x))
        return
    for r in range(0, rows, group):
        m = jnp.mean(load(r, group, 0), axis=-1, keepdims=True)
        mean_ref[pl.ds(r, group), :] = jnp.broadcast_to(m, (group, 128))
        yield [(mean_ref, (r,))]
    for r in range(0, rows, group):
        d = load(r, group, 1) - wide(mean_ref, r, group, 1)
        v = jnp.mean(d * d, axis=-1, keepdims=True)
        rstd_ref[pl.ds(r, group), :] = jnp.broadcast_to(lax.rsqrt(v + EPS), (group, 128))
        yield [(rstd_ref, (r,))]
    for r in range(0, rows, 16):
        x = load(r, 16, 2)
        yield store(r, x, (x - wide(mean_ref, r, 16, 2)) * wide(rstd_ref, r, 16, 2))


def _kernel(x_hbm, mem0_ref, wq_hbm, wk_hbm, wv_hbm, wo_hbm, w1_hbm, w2_hbm,
            w3_hbm, w4_hbm, out_hbm,
            wo_b, xs, hbuf, xg, w1b, we, sems, fence_sem, *bufs):
    stats, q_rings = bufs[:4], bufs[4:]
    w_hbm = (wq_hbm, wk_hbm, wv_hbm)
    q_r = [q_rings[h % 8].at[h // 8] for h in range(H)]

    def x0_copies(k):
        rows = ([pl.ds(P0 // 4 * a + P0 // 8 * k, P0 // 8) for a in range(4)] if k < 2
                else [pl.ds(P0, X0 - P0)])
        return [pltpu.make_async_copy(x_hbm.at[r], xs.at[r], sems.at[SEM_X0 + k])
                for r in rows]

    x_copy = pltpu.make_async_copy(x_hbm.at[pl.ds(X0, S - X0)], xs.at[pl.ds(X0, S - X0)],
                                   sems.at[SEM_X])

    def wo_copy(i):
        rows = pl.ds(_mult(i * 512, 512), 512)
        return pltpu.make_async_copy(wo_hbm.bitcast(u32).at[rows], wo_b.at[rows],
                                     sems.at[SEM_WO + i])

    def w1_copy(i):
        cols = pl.ds(_mult(i * C4, C4), C4)
        return pltpu.make_async_copy(w1_hbm.bitcast(u32).at[:, cols], w1b.at[i],
                                     sems.at[SEM_W1])

    w3_copies = [pltpu.make_async_copy(
        w3_hbm.bitcast(u32).at[:, pl.ds((4 * c + b) * 128, 128)],
        we.at[c, pl.ds(b * 512, 512)], sems.at[SEM_W3]) for c in range(NC) for b in range(4)]

    def w2_slot(p, j, r0=0, n=D // 4):
        return NC + p // 6, pl.ds(_mult(D * (p % 6) + D // 4 * j + r0, 8), n)

    def early_copies(j):
        return [pltpu.make_async_copy(
            w2_hbm.bitcast(u32).at[pl.ds(D // 4 * a, D // 4),
                                   pl.ds(_mult(D // 2 * b + 128 * j, 128), 128)],
            we.at[w2_slot(2 * a + b, j)], sems.at[SEM_W1]) for a, b in QUAD] + [
            pltpu.make_async_copy(
                w4_hbm.bitcast(u32).at[0, a, :, pl.ds(_mult(C4 * j + 128 * k, 128), 128)],
                we.at[NC + 2, pl.ds(_mult(128 * (4 * j + a) + 64 * k, 64), 64)],
                sems.at[SEM_W1]) for a in range(4) for k in range(2)]

    def fence():
        pl.semaphore_signal(fence_sem, 1)
        pl.semaphore_wait(fence_sem, 1)

    def block_a(wq_s, wk_s, wv_s, ubuf, tokbuf, lnbuf, *kv_rings):
        w_s = (wq_s, wk_s, wv_s)
        rings = tuple(q_rings) + tuple(kv_rings)
        ring = [[rings[m * 8 + h % 8].at[h // 8] for h in range(H)] for m in range(3)]
        k_r, v_r = ring[1:]

        xe = [we.at[3, pl.ds(128 * p, 128)] for p in range(NP)]
        w_op = (hbuf, xg)

        def start_chunk(g, m):
            for k in range(8):
                pltpu.make_async_copy(
                    w_hbm[m].bitcast(u32).at[:, 16 * (k % 2) + 4 * g + k // 2, :],
                    we.at[m, pl.ds(D // 2 * k, D // 2)],
                    sems.at[SEM_W + 2 * m + k // 4]).start()

        def wait_chunk(m, halves=(0, 1)):
            for half in halves:
                part = we.at[m, pl.ds(2 * D * half, 2 * D)]
                pltpu.make_async_copy(part, part, sems.at[SEM_W + 2 * m + half]).wait()

        def encode_unit(g, m, half, slices):
            h0 = 8 * g + 4 * half
            for i0 in slices:
                blk = {}

                def get(k, a, b):
                    if (k, a, b) not in blk:
                        for par in range(2):
                            w = we[m, pl.ds(_mult(D // 2 * (
                                4 * half + b - b % 2 + par) + 128 * a + i0, 8), 8), :]
                            for j in range(2):
                                blk[par, a, b - b % 2 + j] = _unzip(w, j)
                        for j in (b - b % 2, b - b % 2 + 1):
                            w_s[m][h0 + j, pl.ds(128 * a + i0, 8), :] = _zip(
                                blk[0, a, j], blk[1, a, j])
                    return blk[k, a, b]

                for p in ORDER_B:
                    known = len(blk)
                    for r, w in enumerate(_encode7(SB, p, get)):
                        q = 7 * p + r
                        if len(SB[p]) + len(SB[r]) > 2:
                            w_op[half][1 + q // 16, pl.ds(128 * (q % 16) + i0, 8), :] = (
                                pltpu.bitcast(w, f32))
                    yield [(w_op[half], (0, HALO))] + [(w_s[m], (h0, 0))] * (len(blk) > known)

        def operand(g, m, half, q, zero):
            tp, tr = SB[q // 7], SB[q % 7]
            if len(tp) + len(tr) == 2:
                a, b = (2 * tp[0][n] + tr[0][n] for n in range(2))
                return w_s[m][8 * g + 4 * half + b, pl.ds(128 * a, 128), :]
            return w_op[half][1 + q // 16, pl.ds(
                pl.multiple_of(128 * (q % 16) + 8 * zero, 8), 128), :]

        def decode_unit(g, m, half, prods):
            for r0 in range(0, P0 // 4, 8):
                out = _decode(prods, r0)
                for i, j in QUAD:
                    for a, b in QUAD:
                        rings[8 * m + 4 * half + 2 * b + j][
                            g, pl.ds(P0 // 4 * (2 * a + i) + r0, 8), :] = out[2 * a + i, 2 * b + j]
                    yield [(rings[8 * m + 4 * half + 2 * b + j], (g, 0)) for b in range(2)]

        for cp in x0_copies(0) + x0_copies(1):
            cp.start()
        for m in range(3):
            start_chunk(0, m)
        x0_copies(2)[0].start()

        @pl.loop(0, P0 // 64 // LN_UNROLL)
        def _(i):
            for k in range(2):
                @pl.when(i == k * P0 // 128 // LN_UNROLL)
                def _():
                    for cp in x0_copies(k):
                        cp.wait()
            n = 16 * LN_UNROLL
            for a in range(4):
                rows = pl.ds(pl.multiple_of(P0 // 4 * a + n * i, 16), n)
                _set_rows(xg, rows, _ln(xs[rows, :].astype(f32)))
            for s in range(LN_UNROLL):
                for kt in range(2):
                    ops = _encode(SA, lambda k, a, b: xg[2 * b + kt, pl.ds(
                        P0 // 4 * a + n * i + 16 * s + k, 8, stride=2), :])
                    for p, w in enumerate(ops):
                        xe[p][pl.ds(pl.multiple_of(64 * kt + n // 2 * i + 8 * s, 8), 8), :] = w

        wait_chunk(0, (0,))

        @pl.loop(0, 16 // W_UNROLL)
        def _(i):
            list(encode_unit(0, 0, 0, [pl.multiple_of(8 * (W_UNROLL * i + k), 8)
                                       for k in range(W_UNROLL)]))

        wait_chunk(0, (1,))

        def transfers(g, g1, m, half):
            if half == 1:
                if m < 2:
                    wait_chunk(m + 1)
                else:
                    pl.when(g < 3)(functools.partial(wait_chunk, 0))
                pl.when(g < 3)(functools.partial(start_chunk, g1, m))
            elif m > 0:
                fence()
                for cp in [w1_copy(g)] + early_copies(g) if m == 1 else [wo_copy(g)]:
                    cp.start()

        last = [we.at[4, pl.ds(128 * p, 128)] for p in range(NP)]

        @pl.loop(0, 4)
        def _(g):
            g1 = jnp.minimum(g + 1, 3)
            zero = g >> 2
            pending = decode_unit((g + 3) & 3, 2, 1, last)
            for m in range(3):
                for half in range(2):
                    nxt = (g1, 0, 0) if (m, half) == (2, 1) else (g, m + half, 1 - half)
                    side = _Side(zero, PRO_N,
                                 (encode_unit(*nxt, range(0, 128, 8)), 7 * 16), (pending, 64))
                    prods = []
                    for p in range(NP):
                        if p == PRO_AT:
                            transfers(g, g1, m, half)
                        lhs = jnp.concatenate(
                            [xe[p][pl.ds(64 * kt, 64), :] for kt in range(2)], axis=1)
                        rhs = operand(g, m, half, p, zero)
                        for k in range(0, 64, 8) if p >= PRO_AT else ():
                            lhs = side.tie(lhs, k, PRO_C)
                        prods.append(_dot(_unpack(lhs), _unpack(rhs)))
                    pending = decode_unit(g, m, half, prods)
            for p in range(NP):
                last[p][...] = pltpu.bitcast(prods[p], u32)

        list(decode_unit(3, 2, 1, last))

        x_copy.start()
        x0_copies(2)[0].wait()
        tokbuf[...] = _ln(xs[pl.ds(P0, UNROLL * TOK), :].astype(f32))
        _set_rows(xg, pl.ds(0, HALO), jnp.zeros((HALO, D), f32))
        _set_rows(xg, pl.ds(HALO + S, HALO), jnp.zeros((HALO, D), f32))
        _set_rows(hbuf, pl.ds(0, UNROLL * TOK), jnp.zeros((UNROLL * TOK, D), f32))
        ubuf[...] = jnp.zeros(ubuf.shape, u32)
        for cp in w3_copies:
            cp.start()
        for i in range(4):
            for cp in [w1_copy(i)] + early_copies(i):
                cp.wait()
        for i in range(4):
            wo_copy(i).wait()

        def wrap(r):
            return jnp.where(r >= RING, r - RING, r)

        def step(s, carry, tok, side, last):
            mem, rp, ra, rw = carry
            ri = lax.broadcasted_iota(jnp.int32, (2 * MEM + SEG, 2 * L), 0)
            ci = lax.broadcasted_iota(jnp.int32, (2 * MEM + SEG, 2 * L), 1)
            key_b = ((ci >= MEM) & (ci < 2 * MEM)) | (ci >= 2 * MEM + SEG)
            same = key_b == ((ri >= MEM) & (ri < 2 * MEM))
            mask = same & ((ri < 2 * MEM) | (ri >= ci))
            fill = jnp.where(same, NEG, -jnp.inf)

            lhs = jnp.concatenate([mem, tok], axis=0).astype(bf16)
            rps = [pl.multiple_of(wrap(rp + 8 * i), 8) for i in range(3)]
            ra_ = pl.multiple_of(ra, SEG)
            rw_ = pl.multiple_of(rw, 8)

            col = s & 3
            group = jnp.maximum((s >> 2) - 1, 0)
            rb = pl.multiple_of(group * (4 * TOK), 8)

            def filler(j):
                u = ubuf[pl.ds(pl.multiple_of((group & 1) * (2 * TOK), 8), 2 * TOK), :]
                r = _dot(_unpack(u), _unpack(w1b[col, :, pl.ds(j * 128, 128)]))
                xg[2 * col + j, pl.ds(HALO + rb, 4 * TOK), :] = r if last and j else _gelu(r)

            mem_qkv = {}
            scores = {}
            o_mem = {}
            total = [None]

            def qkv(h):
                for m in range(3):
                    w = w_s[m][h]
                    for r0 in SIDE_R if h >= SIDE_AT else ():
                        w = side.tie(w, r0)
                    r = _dot(lhs, _unpack(w))
                    for i in range(3):
                        ring[m][h][pl.ds(rps[i], 8), :] = r[8 + 8 * i:16 + 8 * i]
                    mem_qkv[m, h] = r[:MEM]

            def segment(m, pair):
                a, b = 2 * pair, 2 * pair + 1
                ma, mb = mem_qkv.pop((m, a)), mem_qkv.pop((m, b))
                xa, xb = (ring[m][h][pl.ds(ra_, SEG), :] for h in (a, b))
                if m == 0:
                    parts = ((ma, mb, xa), (xb,))
                else:
                    parts = ((ma, mb, xa, xb), (mb, ma, xb))
                return [jnp.concatenate(v, axis=0).astype(bf16) for v in parts]

            def qk(pair):
                q, k = segment(0, pair), segment(1, pair)
                for n in (pair % 2, 1 - pair % 2):
                    scores[pair, n] = lax.dot_general(
                        q[n], k[n], (((1,), (1,)), ((), ())), preferred_element_type=f32)

            def pv(pair):
                v = segment(2, pair)
                for n in (pair % 2, 1 - pair % 2):
                    sc = scores.pop((pair, n)) * (DH ** -0.5)
                    if n == 0:
                        sc = jnp.where(mask, sc, fill)
                    else:
                        sc = jnp.where(mask[2 * MEM:, :2 * MEM + SEG], sc,
                                       fill[2 * MEM:, :2 * MEM + SEG])
                    mx = jnp.max(sc, axis=1, keepdims=True)
                    e = jnp.exp(sc - mx)
                    den = jnp.sum(e, axis=1, keepdims=True)
                    inv = pl.reciprocal(den, approx=True)
                    inv = inv * (2.0 - den * inv)
                    o = _dot(e.astype(bf16), v[n]) * inv
                    q_r[2 * pair + n][pl.ds(ra_, SEG), :] = o[-SEG:]
                    if n == 0:
                        o_mem[2 * pair], o_mem[2 * pair + 1] = o[:MEM], o[MEM:2 * MEM]

            def wo(h):
                lo = jnp.concatenate([o_mem.pop(h), q_r[h][pl.ds(rw_, TOK), :]],
                                     axis=0).astype(bf16)
                r = _dot(lo, _unpack(wo_b[pl.ds(h * DH // 2, DH // 2), :]))
                total[0] = r if total[0] is None else total[0] + r

            npair = H // 2
            for t in range(npair + LAG_WO):
                if 0 <= t - LAG_QK < npair:
                    qk(t - LAG_QK)
                if 0 <= t - LAG_PV < npair:
                    pv(t - LAG_PV)
                if t < npair:
                    qkv(2 * t)
                    qkv(2 * t + 1)
                if t == FILL_AT:
                    filler(0)
                if 0 <= t - LAG_WO < npair:
                    wo(2 * (t - LAG_WO))
                    wo(2 * (t - LAG_WO) + 1)
            filler(1)

            a = total[0]
            return (a[:MEM], wrap(rp + TOK), wrap(ra + SEG), wrap(rw + TOK)), a[MEM:]

        def late_gelu(s):
            rb = jnp.maximum((s >> 2) - 1, 0) * (4 * TOK)
            at = (2 * (s & 3) + 1, pl.ds(pl.multiple_of(HALO + rb, 8), 4 * TOK))
            xg[at] = _gelu(xg[at])
            yield [(xg, (at[0], HALO + rb))]

        def steps(i, carry):
            n = UNROLL * TOK
            pl.when(i == 1)(x_copy.wait)

            @pl.when(i == 16 // ENC)
            def _():
                raw = we.at[pl.ds(0, NC), pl.ds(0, 4 * 512)]
                pltpu.make_async_copy(raw, raw, sems.at[SEM_W3]).wait()

            zero = i >> 5
            at = lambda r, m, k: pl.ds(pl.multiple_of(r + 16 * k * zero, 16), m)
            n_ln = n // 16 + (CH_GROUP and 2 * n // CH_GROUP)

            def norm_filler():
                prev = jnp.maximum(i - 1, 0)

                def first_norm(r, x, y):
                    lnbuf[pl.ds(r, 16), :] = y
                    return [(lnbuf, (r,))]

                def second_norm(r, x, y):
                    dst = pl.multiple_of((n * (prev & 3) + r) // 2, 8)
                    ubuf[pl.ds(dst, 8), :] = _pack(y)
                    return [(ubuf, (dst,))]

                yield from _ln_job(lambda r, m, k: _rows(hbuf, at(n * prev + r, m, k)),
                                   first_norm, n, CH_GROUP, *stats[:2], zero)
                yield from _ln_job(lambda r, m, k: lnbuf[at(r, m, k + 2), :],
                                   second_norm, n, CH_GROUP, *stats[2:], zero)

            def norm_tokens():
                def keep(r, x, y):
                    tokbuf[pl.ds(r, 16), :] = y
                    return [(tokbuf, (r,))]

                nxt = jnp.minimum(P0 + n * (i + 1), S - n)
                return _ln_job(lambda r, m, k: xs[at(nxt + r, m, k), :].astype(f32),
                               keep, n, CH_GROUP, *stats[:2], zero)

            def encode_w23():
                for j in range(4):
                    raw = {(a, b): we[w2_slot(2 * a + b, j, 8 * i, 8)] for a, b in QUAD}
                    get = functools.cache(lambda k, a, b: _unzip(raw[a, b], k))
                    for p in range(7):
                        we[w2_slot(p, j, 8 * i, 8)] = _zip(
                            *[_combine(functools.partial(get, k), SB[p]) for k in range(2)])
                    yield [(we, (NC, 8 * i))]
                for k in range(ENC):
                    j = ENC * i + k
                    grp, i0 = jnp.where(j < 16, NC + 2, (j >> 4) - 1), 8 * (j & 15)
                    slot = lambda q: (grp, pl.ds(pl.multiple_of(128 * q + i0, 8), 8))
                    raw = {(a, b): we[slot(4 * b + a)] for a in range(4) for b in range(4)}
                    get = functools.cache(lambda k, a, b: _unzip(raw[a, b], k))
                    for p in ORDER_B:
                        for r, w in enumerate(_encode7(SB, p, get)):
                            we[slot(7 * p + r)] = w
                        yield [(we, (grp, i0))]

            jobs = [[(norm_filler(), 2 * n_ln), (late_gelu(jnp.maximum(UNROLL * i - 1, 0)), 1)],
                    [(encode_w23(), 4 + 7 * ENC), (norm_tokens(), n_ln)]]
            for k in range(UNROLL):
                s = i * UNROLL + k
                carry, o = step(s, carry, tokbuf[pl.ds(k * TOK, TOK), :],
                                _Side(zero, SIDE_N * len(SIDE_R), *jobs[k]), k == UNROLL - 1)
                lo = k * TOK // 16 * 16
                xv = xs[pl.ds(pl.multiple_of(n * i + lo, 16), 32), :].astype(f32)
                _set_rows(hbuf, pl.ds(pl.multiple_of(TOK * s, 8), TOK),
                          xv[k * TOK - lo:(k + 1) * TOK - lo] + o)
            return carry

        carry = (mem0_ref[...].astype(f32), jnp.int32(P0), jnp.int32(0), jnp.int32(0))
        carry = lax.fori_loop(0, NSEG // UNROLL, steps, carry)
        list(late_gelu(jnp.int32(NSEG - 1)))
        return carry[1] >> 16

    zero = pl.run_scoped(
        block_a,
        *[pltpu.VMEM((H, D // 2, DH), u32)] * 3,
        pltpu.VMEM((4 * TOK, D), u32),
        pltpu.VMEM((UNROLL * TOK, D), f32),
        pltpu.VMEM((UNROLL * TOK, D), f32),
        *[pltpu.VMEM((H // 8, RING, DH), f32)] * 16,
    )

    def tail(w4e, ye, ybuf, ue, *bufs):
        woe, pool = bufs[:3], bufs[3:]
        w4_copies = [
            pltpu.make_async_copy(w4_hbm.bitcast(u32).at[pl.ds(1, NC - 1), a, :, pl.ds(b * C4, C4)],
                                  w4e.at[4 * a + b], sems.at[SEM_W4])
            for a in range(4) for b in range(4)]
        for cp in w4_copies:
            cp.start()
        done = TOK * NSEG
        first = 4 * TOK * (NSEG // 4 - 1)

        def later(rows, n):
            return pl.ds(pl.multiple_of(rows + 8 * zero, 8), n)

        def run(dots, ties, start, *jobs):
            side = _Side(zero, (len(dots) - max(start, 0)) * len(ties), *jobs)
            prods = []
            for load in dots:
                if len(prods) == start:
                    fence()
                lhs, rhs = load()
                for r0, c0 in ties if len(prods) >= start else ():
                    lhs = side.tie(lhs, r0, c0)
                prods.append(_dot(_unpack(lhs), _unpack(rhs)))
            return prods

        hk, hn, hm = H * DH // 4, D // 2, P0 // 2

        def wo_op(p, j):
            if p == 3:
                return pool[j], 0, 0
            if p in (1, 4):
                return wo_b, hk * (p // 4), hn * (p // 4) + C4 * j
            return woe[{0: 0, 2: 1, 5: 2, 6: 0}[p]], 0, C4 * j

        def encode_wo(ps):
            for i0 in range(0, hk, 8):
                for j in range(2):
                    get = functools.cache(lambda k, a, b: _unzip(wo_b[
                        later(hk * a + i0 + 8 * ps[0] * zero, 8), pl.ds(hn * b + C4 * j, C4)], k))
                    ops = [_zip(*[_combine(functools.partial(get, k), SB[p]) for k in range(2)])
                           for p in ps]
                    for p, w in zip(ps, ops):
                        ref, r0, c0 = wo_op(p, j)
                        ref[pl.ds(r0 + i0, 8), pl.ds(c0, C4)] = w
                    yield [(wo_op(p, j)[0], (0,)) for p in ps]

        def encode_o(n):
            for kt in range(H // 2):
                for s in range(hm // 16):
                    pool[n][pl.ds(hm // 2 * (kt // 2) + 8 * s, 8), pl.ds(kt % 2 * 128, 128)] = (
                        _zip(*[_combine(
                            lambda a, b: q_r[H // 2 * b + kt][pl.ds(
                                (done + hm * a + 16 * s) % RING + k + n * zero, 8, stride=2), :],
                            SA[ORDER_B[n]]) for k in range(2)]))
                    if s % 4 == 3:
                        yield [(pool[n], (0,))]

        def wo_dots(n):
            def load(j, i):
                ref, r0, c0 = wo_op(ORDER_B[n], j)
                lhs = [pool[n][later(hm // 2 * c + hm // 4 * i + 8 * j * zero, hm // 4), :]
                       for c in range(8)]
                return (jnp.concatenate(lhs, axis=1),
                        ref[later(r0 + 8 * i * zero, hk), pl.ds(c0, C4)])
            return [functools.partial(load, j, i) for j, i in QUAD]

        def decode_wo(n, prods):
            for (j, i), v in zip(QUAD, prods):
                for r in range(0, hm // 2, 16):
                    for (a, b), sign in SC[ORDER_B[n]]:
                        fresh = all(key != (a, b) for q in ORDER_B[:n] for key, _ in SC[q])
                        row = done + hm * a + hm // 2 * i + r
                        for k in range(2):
                            c = 4 * b + 2 * j + k
                            old = (xs[pl.ds(row, 16), pl.ds(128 * c, 128)].astype(f32) if fresh
                                   else hbuf[c, later(row + 8 * n * zero, 16), :])
                            new = v[r:r + 16, 128 * k:128 * (k + 1)]
                            hbuf[c, pl.ds(row, 16), :] = old + new if sign > 0 else old - new
                    yield [(hbuf, (0, 0))]

        hsb = wo_b

        def norm_in():
            def first_norm(r, x, y):
                woe[2][pl.ds(r, 16), :] = pltpu.bitcast(y[:, :hn], u32)
                woe[2][pl.ds(P0 + r, 16), :] = pltpu.bitcast(y[:, hn:], u32)
                return [(woe[2], (r,))]

            def second_norm(r, x, y):
                ue[pl.ds(r // 2, 8), :] = _pack(y)
                return [(ue, (0,))]

            yield from _ln_job(
                lambda r, n, k: _rows(hbuf, later(done + r + 8 * (7 + k) * zero, n)),
                first_norm, P0, NORM_ROWS, *stats[:2], zero)
            yield from _ln_job(
                lambda r, n, k: pltpu.bitcast(jnp.concatenate(
                    [woe[2][later(r0 + r + 8 * k * zero, n), :] for r0 in (0, P0)], axis=1), f32),
                second_norm, P0, NORM_ROWS, *stats[2:], zero)

        def in_dots(lhs, cols, n=0):
            return [lambda c=c: (lhs(c), w1b[c // 2, later(8 * n * zero, D // 2),
                                             pl.ds(128 * (c % 2), 128)]) for c in cols]

        def gelu_in(r0, cols, prods):
            for c, v in zip(cols, prods):
                for r in range(0, v.shape[0], 32):
                    xg[c, pl.ds(HALO + r0 + r, 32), :] = _gelu(v[r:r + 32])
                    yield [(xg, (c, HALO + r0))]

        def encode_g(i):
            for s in range(RB // 32):
                for kt in range(4):
                    get = functools.cache(lambda k, a, b: xg[4 * b + kt, pl.ds(
                        HALO + i * RB + RB // 2 * a + 16 * s + k + SHIFT[2 * b + kt // 2],
                        8, stride=2), :])
                    for p in range(7):
                        pool[i - 1][pl.ds(128 * p + 64 * (kt // 2) + 8 * s, 8),
                                    pl.ds(128 * (kt % 2), 128)] = _zip(
                            *[_combine(functools.partial(get, k), SA[p]) for k in range(2)])
                    yield [(pool[i - 1], (0,))]

        def out_dots(i, j):
            return [lambda p=p: (
                jnp.concatenate([pool[i - 1][later(128 * p + 64 * k + 8 * j * zero, 64), :]
                                 for k in range(2)], axis=1),
                we[w2_slot(p, j, 8 * (i + 1) * zero)]) for p in range(7)]

        def decode_out(i, j, prods):
            for r0 in range(0, RB // 2, 8):
                out = {}
                for p in range(7):
                    for key, sign in SC[p]:
                        _accumulate(out, key, sign, prods[p][r0:r0 + 8])
                for (a, b), v in out.items():
                    hsb[pl.ds(i * RB + RB // 2 * a + r0, 8),
                        pl.ds(hn * b + 128 * j, 128)] = pltpu.bitcast(v, u32)
                yield [(hsb, (i * RB,))]

        def encode_w4():
            for c in range(NC - 1):
                for i0 in range(0, 64, 8):
                    for j in range(2):
                        at = (c, pl.ds(i0, 8), pl.ds(128 * j, 128))
                        raw = {(a, b): w4e[(4 * a + b,) + at]
                               for a in range(4) for b in range(4)}
                        get = functools.cache(lambda k, a, b: _unzip(raw[a, b], k))
                        for p in ORDER_B:
                            for r, w in enumerate(_encode7(SB, p, get)):
                                w4e[(7 * p + r,) + at] = w
                            yield [(w4e, (0, c, i0))]

        def mixer_post(r0, zero, group):
            def first_norm(r, hv, y):
                rows = pl.ds(_mult(r0 + r, 8), 16)
                x1 = y + pltpu.bitcast(hsb[rows, :], f32)
                _set_rows(xg, rows, hv + x1)
                _set_rows(ybuf, pl.ds(r, 16), x1)
                return [(ybuf, (0, 0)), (xg, (0, r0))]

            def second_norm(r, x1, y):
                _set_rows(hbuf, pl.ds(_mult(r0 + r, 8), 16), y)
                return [(hbuf, (0, r0))]

            at = lambda r, n, k: pl.ds(pl.multiple_of(r + 8 * k * zero, 8), n)
            yield from _ln_job(lambda r, n, k: _rows(hbuf, at(r0 + r, n, k)),
                               first_norm, RB, group, *stats[:2], zero)
            yield from _ln_job(lambda r, n, k: _rows(ybuf, at(r, n, k + 1)),
                               second_norm, RB, group, *stats[2:], zero)
            for s in range(4):
                for kt in range(2):
                    get = functools.cache(lambda k, a, b: hbuf[2 * b + kt, pl.ds(
                        r0 + R4 * a + 4 * k + 2 * (s % 2) + s // 2, 8, stride=8), :])
                    for p in ORDER_A:
                        for r, w in enumerate(_encode7(SA, p, get)):
                            ye[7 * p + r, pl.ds(8 * s, 8), pl.ds(128 * kt, 128)] = w
                        if p in POST_P:
                            yield [(ye, (0, 8 * s))]

        def out_copies(i):
            rows = pl.ds(_mult(i * (RB // 2), RB // 2), RB // 2)
            return [pltpu.make_async_copy(
                woe[b].at[rows], out_hbm.bitcast(u32).at[rows, pl.ds(hn * b, hn)],
                sems.at[SEM_OUT + 2 * i + b]) for b in range(2)]

        n_g, n_out, n_o = RB // 8, RB // 16, H // 2 * hm // 64
        n_post = RB // 8 + 8 * len(POST_P)
        out_ties = [(r0, TIE_C) for r0 in range(0, 64, 8)]
        wo_ties = [(r0, c0) for c0 in range(TIE_C, 2 * D, 512) for r0 in range(0, 64, 8)]
        in_ties = [(r0, c0) for c0 in (TIE_C, 512 + TIE_C) for r0 in range(0, 64, 8)]
        w4_job = encode_w4()
        wo_jobs = [encode_wo(ps) for ps in ((0,), (2, 5), (3, 6))]

        def mixer_out(i, pending, *jobs):
            for j in range(4):
                prods = run(out_dots(i, j), out_ties, FENCE[1] if j == 0 and i in FENCE_I else -1, pending,
                            *[(job, count // 4) for job, count in jobs])
                pending = (decode_out(i, j, prods), n_out)
            return pending

        pending = (encode_o(0), n_o)
        list(pending[0])
        for n in range(7):
            jobs = [(encode_o(n + 1), n_o) if n < 6 else (encode_g(0), n_g)]
            if n:
                jobs.append(pending)
            if n < 5:
                jobs.append((wo_jobs[(n + 1) // 2], hk // 8 if n else hk // 4))
            if n == W4_AT:
                for cp in w4_copies:
                    cp.wait()
            if n >= W4_AT:
                jobs.append((w4_job, 7 * W4_SPLIT[8]))
            prods = run(wo_dots(n), wo_ties, FENCE[0] if n else -1, *jobs)
            pending = (decode_wo(n, prods), hm // 8)
        u = _pack(_ln(_ln(_rows(hbuf, pl.ds(first, done - first)))))
        prods = run(in_dots(lambda c: u, range(8)), in_ties[:6], FENCE[0], pending)
        pending = (gelu_in(first, range(8), prods), 24)
        norm = norm_in()
        for i in range(5):
            jobs = [(w4_job, 7 * W4_SPLIT[i])]
            if i < 4:
                jobs.append((encode_g(i + 1), n_g))
            if i > 0:
                jobs.append((norm, P0 // NORM_ROWS + P0 // 32))
            pending = mixer_out(i, pending, *jobs)
        post, g5 = mixer_post(0, zero, NORM_ROWS), encode_g(5)
        for n in range(8):
            r0, cols = done + n // 2 * 128, range(n % 2 * 4, n % 2 * 4 + 4)
            jobs = [pending, (w4_job, 7 * W4_SPLIT[9])]
            jobs.append((post, (n_post + 4 * RB // NORM_ROWS) // 8))
            if n >= 6:
                jobs.append((g5, n_g // 2))
            prods = run(in_dots(
                lambda c: ue[later((r0 - done) // 2 + 8 * c * zero, 64), :], cols, n + 1),
                in_ties, FENCE[2] if n % 2 == 0 else -1, *jobs)
            pending = (gelu_in(r0, cols, prods), RB // 16)
        for i in range(5, 8):
            jobs = [(w4_job, 7 * W4_SPLIT[i])]
            if i < 7:
                jobs.append((encode_g(i + 1), n_g))
            pending = mixer_out(i, pending, *jobs)
        list(pending[0])
        list(w4_job)

        def mlp_block(i, carry):
            te = []
            for c in range(NC):
                ops = []
                for r0 in range(0, R4, UP_ROWS):
                    prods = [_dot(_unpack(ye[p, pl.ds(r0 // 2, UP_ROWS // 2), :]), _unpack(
                        we[c, pl.ds(pl.multiple_of(128 * p + r0 * (i >> 3), 8), 128), :]))
                        for p in range(NP)]
                    for s in range(UP_ROWS // 16):
                        act = [{key: _gelu2(v) for key, v in _decode(
                            prods, 32 * (s // 2) + 16 * k + 8 * (s % 2)).items()}
                            for k in range(2)]
                        ops.append(_encode(SA, lambda k, a, b: act[k][a, b]))
                te.append([jnp.concatenate([o[p] for o in ops], axis=0) for p in range(NP)])

            def down(p, lo, hi, tie=lambda w: w):
                lhs = jnp.concatenate([tie(te[c][p]) if c in POST_C else te[c][p]
                                       for c in range(lo, hi)], axis=1)
                rhs = [w4e[p, c - 1] if c else jnp.concatenate(
                    [we[NC + 2, pl.ds(128 * p + 64 * k, 64), :] for k in range(2)], axis=1)
                    for c in range(lo, hi)]
                return _dot(_unpack(lhs), _unpack(jnp.concatenate(rhs, axis=0)))

            prods = [down(p, 0, KSPLIT) for p in range(NSPLIT)]
            prods = [m + down(p, KSPLIT, NC) for p, m in enumerate(prods)]
            out = {}

            def finish(qa, qb):
                for a, b in ((2 * qa + n // 2, 2 * qb + n % 2) for n in range(4)):
                    for r in range(0, R4, 16):
                        row = i * RB + R4 * a + r
                        for j in range(2):
                            woe[qb][pl.ds(pl.multiple_of(row // 2, 8), 8),
                                    pl.ds(C4 * (b % 2) + 128 * j, 128)] = _zip(*[
                                        0.5 * out[a, b][32 * k + r // 2:32 * k + r // 2 + 8,
                                                  128 * j:128 * (j + 1)]
                                        + xg[2 * b + j, pl.ds(row + k, 8, stride=2), :]
                                        for k in range(2)])
                        yield [(woe[qb], (i * (RB // 2),))]

            side = _Side(i >> 3, POST_N * len(POST_C),
                         (mixer_post(((i + 1) & 7) * RB, i >> 3, 0), n_post))
            for p in range(7):
                done_quad = {4: (1, 0), 5: (0, 1), 6: (1, 1)}.get(p)
                store = _Side(i >> 3, 16, *([(finish(*done_quad), 16)] if done_quad else []))
                for q in range(len(prods), 7 * p + 7):
                    side.after(hbuf, prods[q - POST_LAG])
                    prods.append(down(q, 0, NC, side.tie if q % 7 == 0 else
                                      lambda w: store.tie(side.tie(w))))
                _decode7(p, prods[7 * p:7 * p + 7], out)
            list(finish(0, 0))
            for cp in out_copies(i):
                cp.start()
            return carry

        lax.fori_loop(0, S // RB, mlp_block, 0)
        for i in range(S // RB):
            for cp in out_copies(i):
                cp.wait()

    pl.run_scoped(
        tail,
        pltpu.VMEM((NP, NC - 1, 64, C4), u32),
        pltpu.VMEM((NP, R4 // 2, C4), u32),
        pltpu.VMEM((D // 128, RB, 128), f32),
        pltpu.VMEM((P0 // 2, D), u32),
        *[pltpu.VMEM((H * DH // 4, D // 2), u32)] * 3,
        *[pltpu.VMEM((D, C4), u32)] * 8,
    )


@jax.jit
def pallas_sequential_preLN__memory_aug_recurrent_mem_tr__mixer_s_mlp__prompt_kernel(
    A_x: jax.Array,
    A_mem0: jax.Array,
    A_Wq: jax.Array,
    A_Wk: jax.Array,
    A_Wv: jax.Array,
    A_Wo: jax.Array,
    A_seg_len: jax.Array,
    B_x: jax.Array,
    B_w1: jax.Array,
    B_w2: jax.Array,
    B_w3: jax.Array,
    B_w4: jax.Array,
):
    del A_seg_len, B_x
    hbm = pl.BlockSpec(memory_space=pl.ANY)
    vmem = pl.BlockSpec(memory_space=pltpu.VMEM)
    scratch = [
        pltpu.VMEM((H * DH // 2, D), u32),
        pltpu.VMEM((S, D), bf16),
        pltpu.VMEM((D // 128, S + 8, 128), f32),
        pltpu.VMEM((D // 128, S + 2 * HALO, 128), f32),
        pltpu.VMEM((4, D // 2, C4), u32),
        pltpu.VMEM((NC + 3, NP * 128, 128), u32),
        pltpu.SemaphoreType.DMA((NSEM,)),
        pltpu.SemaphoreType.REGULAR,
    ] + [pltpu.VMEM((P0, 128), f32)] * 4 + [pltpu.VMEM((H // 8, RING, DH), f32)] * 8
    out = pl.pallas_call(
        _kernel,
        out_shape=jax.ShapeDtypeStruct((S, D), A_x.dtype),
        in_specs=[hbm, vmem] + [hbm] * 8,
        out_specs=hbm,
        scratch_shapes=scratch,
        compiler_params=pltpu.CompilerParams(vmem_limit_bytes=VMEM_LIMIT),
    )(A_x.reshape(S, D), A_mem0.reshape(MEM, D),
      A_Wq.reshape(D // 2, 2 * H, DH), A_Wk.reshape(D // 2, 2 * H, DH),
      A_Wv.reshape(D // 2, 2 * H, DH),
      A_Wo.reshape(H * DH, D), B_w1, B_w2, B_w3, B_w4.reshape(NC, 4, 128, D))
    return out.reshape(A_x.shape)
```

```python
import functools

import jax
import jax.numpy as jnp
from jax import lax
import jax.experimental.pallas as pl
import jax.experimental.pallas.tpu as pltpu

S = 2048
D = 1024
H = 32
DH = 128
MEM = 8
SEG = 32
F = 3584
NSEG = S // SEG
L = MEM + SEG
TOK = 24
P0 = S - TOK * NSEG
RING = 576
X0 = P0 + 128
C4 = D // 4
SHIFT = (-1, 1, -2, 2)
HALO = 8
RB = 256
R4 = RB // 4
NC = F // 512
NP = 49
EPS = 1e-5
NEG = -1000000000.0

VMEM_LIMIT = 127 * 1024 * 1024 + 896 * 1024

LAG_QK = 2
LAG_PV = 4
LAG_WO = 6
FILL_AT = 20
UNROLL = 2
ENC = 4
SIDE_AT = 6
SIDE_N = 50
LN_UNROLL = 2
W_UNROLL = 4
TIE_C = 384
NORM_ROWS = 16
W4_AT = 5
W4_WO = 14
W4_SPLIT = (12, 4, 4, 4, 4, 12, 12, 16)
UP_ROWS = 32
NSPLIT = 5
KSPLIT = 5
POST_C = (1, 3, 5)
POST_N = 44
POST_LAG = 5
POST_P = (0, 6, 5)
assert (7 - W4_AT) * W4_WO + sum(W4_SPLIT) == 16 * (NC - 1)

bf16 = jnp.bfloat16
f32 = jnp.float32
u32 = jnp.uint32

SEM_X0, SEM_X, SEM_W1, SEM_W3, SEM_W4, SEM_WO, SEM_OUT, SEM_W = 0, 3, 4, 5, 6, 7, 11, 27
NSEM = SEM_W + 6

SA = (((0, 0), 1, (1, 1)), ((1, 0), 1, (1, 1)), ((0, 0),), ((1, 1),),
      ((0, 0), 1, (0, 1)), ((1, 0), -1, (0, 0)), ((0, 1), -1, (1, 1)))
SB = (((0, 0), 1, (1, 1)), ((0, 0),), ((0, 1), -1, (1, 1)), ((1, 0), -1, (0, 0)),
      ((1, 1),), ((0, 0), 1, (0, 1)), ((1, 0), 1, (1, 1)))
SC = ((((0, 0), 1), ((1, 1), 1)), (((1, 0), 1), ((1, 1), -1)),
      (((0, 1), 1), ((1, 1), 1)), (((0, 0), 1), ((1, 0), 1)),
      (((0, 0), -1), ((0, 1), 1)), (((1, 1), 1),), (((0, 0), 1),))
ORDER_A = (2, 3, 0, 4, 6, 1, 5)
ORDER_B = (1, 4, 0, 2, 5, 3, 6)
QUAD = ((0, 0), (0, 1), (1, 0), (1, 1))


def _mult(i, n):
    return i if isinstance(i, int) else pl.multiple_of(i, n)


def _ln(x):
    m = jnp.mean(x, axis=-1, keepdims=True)
    d = x - m
    v = jnp.mean(d * d, axis=-1, keepdims=True)
    return d * lax.rsqrt(v + EPS)


def _gelu2(x):
    c = 0.7978845608028654
    return x * jnp.tanh(x * (c + c * 0.044715 * (x * x))) + x


def _gelu(x):
    return 0.5 * _gelu2(x)


def _pack(x):
    return pltpu.bitcast(x.astype(bf16), u32)


def _unpack(x):
    return pltpu.bitcast(x, bf16)


def _dot(a, b):
    return jnp.dot(a, b, preferred_element_type=f32)


def _zip(even, odd):
    return pltpu.bitcast(pltpu.pack_elementwise([even, odd], packed_dtype=bf16), u32)


def _unzip(w, k):
    return pltpu.unpack_elementwise(w, index=k, packed_dtype=bf16, unpacked_dtype=f32)


def _combine(get, term):
    if len(term) == 1:
        return get(*term[0])
    a, b = get(*term[0]), get(*term[2])
    return a + b if term[1] > 0 else a - b


def _encode7(tab, p, get):
    outer = [{(i, j): _combine(lambda a, b: get(k, 2 * a + i, 2 * b + j), tab[p])
              for i, j in QUAD} for k in range(2)]
    return [_zip(*[_combine(lambda a, b: o[a, b], tab[r]) for o in outer])
            for r in range(7)]


def _encode(tab, get):
    get = functools.cache(get)
    ops = {p: _encode7(tab, p, get) for p in (ORDER_A if tab is SA else ORDER_B)}
    return [w for p in range(7) for w in ops[p]]


def _accumulate(acc, key, sign, v):
    if key not in acc:
        acc[key] = v
    else:
        acc[key] = acc[key] + v if sign > 0 else acc[key] - v


def _decode7(p, prods, out):
    inner = {}
    for r in range(7):
        for key, sign in SC[r]:
            _accumulate(inner, key, sign, prods[r])
    for (a, b), sign in SC[p]:
        for (i, j), v in inner.items():
            _accumulate(out, (2 * a + i, 2 * b + j), sign, v)


def _decode(prods, r0):
    out = {}
    for p in range(7):
        _decode7(p, [pltpu.bitcast(m[r0:r0 + 8, :], f32) for m in prods[7 * p:7 * p + 7]],
                 out)
    return out


def _rows(ref, rows):
    return jnp.concatenate([ref[c, rows, :] for c in range(ref.shape[0])], axis=1)


def _set_rows(ref, rows, v):
    for c in range(ref.shape[0]):
        ref[c, rows, :] = v[:, c * 128:(c + 1) * 128]


class _Side:
    def __init__(self, zero, slots, *jobs):
        self.zero = zero
        self.slots = slots
        self.jobs = [[job, count, 0] for job, count in jobs]
        self.at = 0

    def tie(self, w, r0=0, c0=0):
        self.at += 1
        head = old = w[r0:r0 + 8, c0:c0 + 128]
        for job in self.jobs:
            while job[2] * self.slots < min(self.at, self.slots) * job[1]:
                job[2] += 1
                for ref, idx in next(job[0]):
                    row = pl.ds(pl.multiple_of(idx[-1] + 8 * self.zero, 8), 8)
                    seen = ref[idx[:-1] + (row, pl.ds(0, 128))]
                    head = jnp.where(self.zero == 0, head, pltpu.bitcast(seen, u32))
        if head is old:
            return w
        row = [v for v in (w[r0:r0 + 8, :c0] if c0 else None, head,
                           w[r0:r0 + 8, c0 + 128:] if c0 + 128 < w.shape[1] else None)
               if v is not None]
        rows = (w[:r0] if r0 else None, jnp.concatenate(row, axis=1),
                w[r0 + 8:] if r0 + 8 < w.shape[0] else None)
        return jnp.concatenate([v for v in rows if v is not None], axis=0)

    def after(self, ref, r):
        spare = pl.multiple_of(ref.shape[-2] - 8 - 8 * self.zero, 8)
        lead = tuple(n - 1 - self.zero for n in ref.shape[:-2])
        ref[lead + (pl.ds(spare, 8), pl.ds(0, 128))] = pltpu.bitcast(r[:8, :128], ref.dtype)


def _ln_job(load, store, rows, group=0, mean_ref=None, rstd_ref=None, zero=None):
    wide = lambda ref, r, n, k: jnp.concatenate(
        [ref[pl.ds(pl.multiple_of(r + 8 * k * zero, 8), n), :]] * (D // 128), axis=1)
    if not group:
        for r in range(0, rows, 16):
            x = load(r, 16, 0)
            yield store(r, x, _ln(x))
        return
    for r in range(0, rows + 2 * group, group):
        if r < rows:
            m = jnp.mean(load(r, group, 0), axis=-1, keepdims=True)
            mean_ref[pl.ds(r, group), :] = jnp.broadcast_to(m, (group, 128))
            yield [(mean_ref, (r,))]
        if 0 <= r - group < rows:
            d = load(r - group, group, 1) - wide(mean_ref, r - group, group, 1)
            v = jnp.mean(d * d, axis=-1, keepdims=True)
            rstd_ref[pl.ds(r - group, group), :] = jnp.broadcast_to(
                lax.rsqrt(v + EPS), (group, 128))
            yield [(rstd_ref, (r - group,))]
        for q in range(r - 2 * group, r - group, 16) if r >= 2 * group else ():
            x = load(q, 16, 2)
            yield store(q, x, (x - wide(mean_ref, q, 16, 2)) * wide(rstd_ref, q, 16, 2))


def _kernel(x_hbm, mem0_ref, wq_hbm, wk_hbm, wv_hbm, wo_hbm, w1_hbm, w2_hbm,
            w3_hbm, w4_hbm, out_hbm,
            wo_b, xs, hbuf, xg, w1b, we, sems, fence_sem, *bufs):
    stats, q_rings = bufs[:4], bufs[4:]
    w_hbm = (wq_hbm, wk_hbm, wv_hbm)
    q_r = [q_rings[h % 8].at[h // 8] for h in range(H)]

    def x0_copies(k):
        rows = ([pl.ds(P0 // 4 * a + P0 // 8 * k, P0 // 8) for a in range(4)] if k < 2
                else [pl.ds(P0, X0 - P0)])
        return [pltpu.make_async_copy(x_hbm.at[r], xs.at[r], sems.at[SEM_X0 + k])
                for r in rows]

    x_copy = pltpu.make_async_copy(x_hbm.at[pl.ds(X0, S - X0)], xs.at[pl.ds(X0, S - X0)],
                                   sems.at[SEM_X])

    def wo_copy(i):
        rows = pl.ds(_mult(i * 512, 512), 512)
        return pltpu.make_async_copy(wo_hbm.bitcast(u32).at[rows], wo_b.at[rows],
                                     sems.at[SEM_WO + i])

    def w1_copy(i):
        cols = pl.ds(_mult(i * C4, C4), C4)
        return pltpu.make_async_copy(w1_hbm.bitcast(u32).at[:, cols], w1b.at[i],
                                     sems.at[SEM_W1])

    w3_copies = [pltpu.make_async_copy(
        w3_hbm.bitcast(u32).at[:, pl.ds((4 * c + b) * 128, 128)],
        we.at[c, pl.ds(b * 512, 512)], sems.at[SEM_W3]) for c in range(NC) for b in range(4)]

    def w2_slot(p, j, r0=0, n=D // 4):
        return NC + p // 6, pl.ds(_mult(D * (p % 6) + D // 4 * j + r0, 8), n)

    def early_copies(j):
        return [pltpu.make_async_copy(
            w2_hbm.bitcast(u32).at[pl.ds(D // 4 * a, D // 4),
                                   pl.ds(_mult(D // 2 * b + 128 * j, 128), 128)],
            we.at[w2_slot(2 * a + b, j)], sems.at[SEM_W1]) for a, b in QUAD] + [
            pltpu.make_async_copy(
                w4_hbm.bitcast(u32).at[0, a, :, pl.ds(_mult(C4 * j + 128 * k, 128), 128)],
                we.at[NC + 2, pl.ds(_mult(128 * (4 * j + a) + 64 * k, 64), 64)],
                sems.at[SEM_W1]) for a in range(4) for k in range(2)]

    def fence():
        pl.semaphore_signal(fence_sem, 1)
        pl.semaphore_wait(fence_sem, 1)

    def block_a(wq_s, wk_s, wv_s, ubuf, tokbuf, lnbuf, *kv_rings):
        w_s = (wq_s, wk_s, wv_s)
        rings = tuple(q_rings) + tuple(kv_rings)
        ring = [[rings[m * 8 + h % 8].at[h // 8] for h in range(H)] for m in range(3)]
        k_r, v_r = ring[1:]

        xe = [we.at[3, pl.ds(128 * p, 128)] for p in range(NP)]
        w_op = (hbuf, xg)

        def start_chunk(g, m):
            for k in range(8):
                pltpu.make_async_copy(
                    w_hbm[m].bitcast(u32).at[:, 16 * (k % 2) + 4 * g + k // 2, :],
                    we.at[m, pl.ds(D // 2 * k, D // 2)],
                    sems.at[SEM_W + 2 * m + k // 4]).start()

        def wait_chunk(m, halves=(0, 1)):
            for half in halves:
                part = we.at[m, pl.ds(2 * D * half, 2 * D)]
                pltpu.make_async_copy(part, part, sems.at[SEM_W + 2 * m + half]).wait()

        def encode_unit(g, m, half, slices):
            h0 = 8 * g + 4 * half
            for i0 in slices:
                blk = {}

                def get(k, a, b):
                    if (k, a, b) not in blk:
                        for par in range(2):
                            w = we[m, pl.ds(_mult(D // 2 * (
                                4 * half + b - b % 2 + par) + 128 * a + i0, 8), 8), :]
                            for j in range(2):
                                blk[par, a, b - b % 2 + j] = _unzip(w, j)
                        for j in (b - b % 2, b - b % 2 + 1):
                            w_s[m][h0 + j, pl.ds(128 * a + i0, 8), :] = _zip(
                                blk[0, a, j], blk[1, a, j])
                    return blk[k, a, b]

                for p in ORDER_B:
                    known = len(blk)
                    for r, w in enumerate(_encode7(SB, p, get)):
                        q = 7 * p + r
                        if len(SB[p]) + len(SB[r]) > 2:
                            w_op[half][1 + q // 16, pl.ds(128 * (q % 16) + i0, 8), :] = (
                                pltpu.bitcast(w, f32))
                    yield [(w_op[half], (0, HALO))] + [(w_s[m], (h0, 0))] * (len(blk) > known)

        def operand(g, m, half, q, zero):
            tp, tr = SB[q // 7], SB[q % 7]
            if len(tp) + len(tr) == 2:
                a, b = (2 * tp[0][n] + tr[0][n] for n in range(2))
                return w_s[m][8 * g + 4 * half + b, pl.ds(128 * a, 128), :]
            return w_op[half][1 + q // 16, pl.ds(
                pl.multiple_of(128 * (q % 16) + 8 * zero, 8), 128), :]

        def decode_unit(g, m, half, prods):
            for r0 in range(0, P0 // 4, 8):
                out = _decode(prods, r0)
                for i, j in QUAD:
                    for a, b in QUAD:
                        rings[8 * m + 4 * half + 2 * b + j][
                            g, pl.ds(P0 // 4 * (2 * a + i) + r0, 8), :] = out[2 * a + i, 2 * b + j]
                    yield [(rings[8 * m + 4 * half + 2 * b + j], (g, 0)) for b in range(2)]

        for cp in x0_copies(0) + x0_copies(1):
            cp.start()
        for m in range(3):
            start_chunk(0, m)
        x0_copies(2)[0].start()

        @pl.loop(0, P0 // 64 // LN_UNROLL)
        def _(i):
            for k in range(2):
                @pl.when(i == k * P0 // 128 // LN_UNROLL)
                def _():
                    for cp in x0_copies(k):
                        cp.wait()
            n = 16 * LN_UNROLL
            for a in range(4):
                rows = pl.ds(pl.multiple_of(P0 // 4 * a + n * i, 16), n)
                _set_rows(xg, rows, _ln(xs[rows, :].astype(f32)))
            for s in range(LN_UNROLL):
                for kt in range(2):
                    ops = _encode(SA, lambda k, a, b: xg[2 * b + kt, pl.ds(
                        P0 // 4 * a + n * i + 16 * s + k, 8, stride=2), :])
                    for p, w in enumerate(ops):
                        xe[p][pl.ds(pl.multiple_of(64 * kt + n // 2 * i + 8 * s, 8), 8), :] = w

        wait_chunk(0, (0,))

        @pl.loop(0, 16 // W_UNROLL)
        def _(i):
            list(encode_unit(0, 0, 0, [pl.multiple_of(8 * (W_UNROLL * i + k), 8)
                                       for k in range(W_UNROLL)]))

        wait_chunk(0, (1,))

        def transfers(g, g1, m, half):
            if half == 1:
                if m < 2:
                    wait_chunk(m + 1)
                else:
                    pl.when(g < 3)(functools.partial(wait_chunk, 0))
                pl.when(g < 3)(functools.partial(start_chunk, g1, m))
            elif m > 0:
                fence()
                for cp in [w1_copy(g)] + early_copies(g) if m == 1 else [wo_copy(g)]:
                    cp.start()

        last = [we.at[4, pl.ds(128 * p, 128)] for p in range(NP)]

        @pl.loop(0, 4)
        def _(g):
            g1 = jnp.minimum(g + 1, 3)
            zero = g >> 2
            pending = decode_unit((g + 3) & 3, 2, 1, last)
            for m in range(3):
                for half in range(2):
                    nxt = (g1, 0, 0) if (m, half) == (2, 1) else (g, m + half, 1 - half)
                    side = _Side(zero, 8 * (NP - 1),
                                 (encode_unit(*nxt, range(0, 128, 8)), 7 * 16), (pending, 64))
                    prods = []
                    for p in range(NP):
                        if p == 1:
                            transfers(g, g1, m, half)
                        lhs = jnp.concatenate(
                            [xe[p][pl.ds(64 * kt, 64), :] for kt in range(2)], axis=1)
                        rhs = operand(g, m, half, p, zero)
                        for k in range(0, 64, 8) if p else ():
                            lhs = side.tie(lhs, k, 128)
                        prods.append(_dot(_unpack(lhs), _unpack(rhs)))
                    pending = decode_unit(g, m, half, prods)
            for p in range(NP):
                last[p][...] = pltpu.bitcast(prods[p], u32)

        list(decode_unit(3, 2, 1, last))

        x_copy.start()
        x0_copies(2)[0].wait()
        tokbuf[...] = _ln(xs[pl.ds(P0, UNROLL * TOK), :].astype(f32))
        _set_rows(xg, pl.ds(0, HALO), jnp.zeros((HALO, D), f32))
        _set_rows(xg, pl.ds(HALO + S, HALO), jnp.zeros((HALO, D), f32))
        _set_rows(hbuf, pl.ds(0, UNROLL * TOK), jnp.zeros((UNROLL * TOK, D), f32))
        ubuf[...] = jnp.zeros(ubuf.shape, u32)
        for cp in w3_copies:
            cp.start()
        for i in range(4):
            for cp in [w1_copy(i)] + early_copies(i):
                cp.wait()
        for i in range(4):
            wo_copy(i).wait()

        def wrap(r):
            return jnp.where(r >= RING, r - RING, r)

        def step(s, carry, tok, side, last):
            mem, rp, ra, rw = carry
            ri = lax.broadcasted_iota(jnp.int32, (2 * MEM + SEG, 2 * L), 0)
            ci = lax.broadcasted_iota(jnp.int32, (2 * MEM + SEG, 2 * L), 1)
            key_b = ((ci >= MEM) & (ci < 2 * MEM)) | (ci >= 2 * MEM + SEG)
            same = key_b == ((ri >= MEM) & (ri < 2 * MEM))
            mask = same & ((ri < 2 * MEM) | (ri >= ci))
            fill = jnp.where(same, NEG, -jnp.inf)

            lhs = jnp.concatenate([mem, tok], axis=0).astype(bf16)
            rps = [pl.multiple_of(wrap(rp + 8 * i), 8) for i in range(3)]
            ra_ = pl.multiple_of(ra, SEG)
            rw_ = pl.multiple_of(rw, 8)

            col = s & 3
            group = jnp.maximum((s >> 2) - 1, 0)
            rb = pl.multiple_of(group * (4 * TOK), 8)

            def filler(j):
                u = ubuf[pl.ds(pl.multiple_of((group & 1) * (2 * TOK), 8), 2 * TOK), :]
                r = _dot(_unpack(u), _unpack(w1b[col, :, pl.ds(j * 128, 128)]))
                xg[2 * col + j, pl.ds(HALO + rb, 4 * TOK), :] = r if last and j else _gelu(r)

            mem_qkv = {}
            scores = {}
            o_mem = {}
            total = [None]

            def qkv(h):
                for m in range(3):
                    w = w_s[m][h]
                    r = _dot(lhs, _unpack(side.tie(w, D // 4) if h >= SIDE_AT else w))
                    for i in range(3):
                        ring[m][h][pl.ds(rps[i], 8), :] = r[8 + 8 * i:16 + 8 * i]
                    mem_qkv[m, h] = r[:MEM]

            def segment(m, pair):
                a, b = 2 * pair, 2 * pair + 1
                ma, mb = mem_qkv.pop((m, a)), mem_qkv.pop((m, b))
                xa, xb = (ring[m][h][pl.ds(ra_, SEG), :] for h in (a, b))
                if m == 0:
                    parts = ((ma, mb, xa), (xb,))
                else:
                    parts = ((ma, mb, xa, xb), (mb, ma, xb))
                return [jnp.concatenate(v, axis=0).astype(bf16) for v in parts]

            def qk(pair):
                q, k = segment(0, pair), segment(1, pair)
                for n in range(2):
                    scores[pair, n] = lax.dot_general(
                        q[n], k[n], (((1,), (1,)), ((), ())), preferred_element_type=f32)

            def pv(pair):
                v = segment(2, pair)
                for n in range(2):
                    sc = scores.pop((pair, n)) * (DH ** -0.5)
                    if n == 0:
                        sc = jnp.where(mask, sc, fill)
                    else:
                        sc = jnp.where(mask[2 * MEM:, :2 * MEM + SEG], sc,
                                       fill[2 * MEM:, :2 * MEM + SEG])
                    mx = jnp.max(sc, axis=1, keepdims=True)
                    e = jnp.exp(sc - mx)
                    den = jnp.sum(e, axis=1, keepdims=True)
                    inv = pl.reciprocal(den, approx=True)
                    inv = inv * (2.0 - den * inv)
                    o = _dot(e.astype(bf16), v[n]) * inv
                    q_r[2 * pair + n][pl.ds(ra_, SEG), :] = o[-SEG:]
                    if n == 0:
                        o_mem[2 * pair], o_mem[2 * pair + 1] = o[:MEM], o[MEM:2 * MEM]

            def wo(h):
                lo = jnp.concatenate([o_mem.pop(h), q_r[h][pl.ds(rw_, TOK), :]],
                                     axis=0).astype(bf16)
                r = _dot(lo, _unpack(wo_b[pl.ds(h * DH // 2, DH // 2), :]))
                total[0] = r if total[0] is None else total[0] + r

            npair = H // 2
            for t in range(npair + LAG_WO):
                if 0 <= t - LAG_QK < npair:
                    qk(t - LAG_QK)
                if 0 <= t - LAG_PV < npair:
                    pv(t - LAG_PV)
                if t < npair:
                    qkv(2 * t)
                    qkv(2 * t + 1)
                if t == FILL_AT:
                    filler(0)
                if 0 <= t - LAG_WO < npair:
                    wo(2 * (t - LAG_WO))
                    wo(2 * (t - LAG_WO) + 1)
            filler(1)

            a = total[0]
            return (a[:MEM], wrap(rp + TOK), wrap(ra + SEG), wrap(rw + TOK)), a[MEM:]

        def late_gelu(s):
            rb = jnp.maximum((s >> 2) - 1, 0) * (4 * TOK)
            at = (2 * (s & 3) + 1, pl.ds(pl.multiple_of(HALO + rb, 8), 4 * TOK))
            xg[at] = _gelu(xg[at])
            yield [(xg, (at[0], HALO + rb))]

        def steps(i, carry):
            n = UNROLL * TOK
            pl.when(i == 1)(x_copy.wait)

            @pl.when(i == 16 // ENC)
            def _():
                raw = we.at[pl.ds(0, NC), pl.ds(0, 4 * 512)]
                pltpu.make_async_copy(raw, raw, sems.at[SEM_W3]).wait()

            zero = i >> 5
            at = lambda r, m, k: pl.ds(pl.multiple_of(r + 16 * k * zero, 16), m)

            def norm_filler():
                prev = jnp.maximum(i - 1, 0)

                def first_norm(r, x, y):
                    lnbuf[pl.ds(r, 16), :] = y
                    return [(lnbuf, (r,))]

                def second_norm(r, x, y):
                    dst = pl.multiple_of((n * (prev & 3) + r) // 2, 8)
                    ubuf[pl.ds(dst, 8), :] = _pack(y)
                    return [(ubuf, (dst,))]

                yield from _ln_job(lambda r, m, k: _rows(hbuf, at(n * prev + r, m, k)),
                                   first_norm, n)
                yield from _ln_job(lambda r, m, k: lnbuf[at(r, m, k + 2), :],
                                   second_norm, n)

            def norm_tokens():
                def keep(r, x, y):
                    tokbuf[pl.ds(r, 16), :] = y
                    return [(tokbuf, (r,))]

                nxt = jnp.minimum(P0 + n * (i + 1), S - n)
                return _ln_job(lambda r, m, k: xs[at(nxt + r, m, k), :].astype(f32),
                               keep, n)

            def encode_b():
                for j in range(4):
                    raw = {(a, b): we[w2_slot(2 * a + b, j, 8 * i, 8)] for a, b in QUAD}
                    get = functools.cache(lambda k, a, b: _unzip(raw[a, b], k))
                    for p in range(7):
                        we[w2_slot(p, j, 8 * i, 8)] = _zip(
                            *[_combine(functools.partial(get, k), SB[p]) for k in range(2)])
                    yield [(we, (NC, 8 * i))]
                for k in range(ENC):
                    j = ENC * i + k
                    grp, i0 = jnp.where(j < 16, NC + 2, (j >> 4) - 1), 8 * (j & 15)
                    slot = lambda q: (grp, pl.ds(pl.multiple_of(128 * q + i0, 8), 8))
                    raw = {(a, b): we[slot(4 * b + a)] for a in range(4) for b in range(4)}
                    get = functools.cache(lambda k, a, b: _unzip(raw[a, b], k))
                    for p in ORDER_B:
                        for r, w in enumerate(_encode7(SB, p, get)):
                            we[slot(7 * p + r)] = w
                        yield [(we, (grp, i0))]

            jobs = [[(norm_filler(), 2 * n // 16), (late_gelu(jnp.maximum(UNROLL * i - 1, 0)), 1)],
                    [(encode_b(), 4 + 7 * ENC), (norm_tokens(), n // 16)]]
            for k in range(UNROLL):
                s = i * UNROLL + k
                carry, o = step(s, carry, tokbuf[pl.ds(k * TOK, TOK), :],
                                _Side(zero, SIDE_N, *jobs[k]), k == UNROLL - 1)
                lo = k * TOK // 16 * 16
                xv = xs[pl.ds(pl.multiple_of(n * i + lo, 16), 32), :].astype(f32)
                _set_rows(hbuf, pl.ds(pl.multiple_of(TOK * s, 8), TOK),
                          xv[k * TOK - lo:(k + 1) * TOK - lo] + o)
            return carry

        carry = (mem0_ref[...].astype(f32), jnp.int32(P0), jnp.int32(0), jnp.int32(0))
        carry = lax.fori_loop(0, NSEG // UNROLL, steps, carry)
        list(late_gelu(jnp.int32(NSEG - 1)))
        return carry[1] >> 16

    zero = pl.run_scoped(
        block_a,
        *[pltpu.VMEM((H, D // 2, DH), u32)] * 3,
        pltpu.VMEM((4 * TOK, D), u32),
        pltpu.VMEM((UNROLL * TOK, D), f32),
        pltpu.VMEM((UNROLL * TOK, D), f32),
        *[pltpu.VMEM((H // 8, RING, DH), f32)] * 16,
    )

    def tail(w4e, ye, ybuf, ue, *bufs):
        woe, pool = bufs[:3], bufs[3:]
        w4_copies = [
            pltpu.make_async_copy(w4_hbm.bitcast(u32).at[pl.ds(1, NC - 1), a, :, pl.ds(b * C4, C4)],
                                  w4e.at[4 * a + b], sems.at[SEM_W4])
            for a in range(4) for b in range(4)]
        for cp in w4_copies:
            cp.start()
        done = TOK * NSEG
        first = 4 * TOK * (NSEG // 4 - 1)

        def later(rows, n):
            return pl.ds(pl.multiple_of(rows + 8 * zero, 8), n)

        def run(dots, ties, start, *jobs):
            side = _Side(zero, (len(dots) - max(start, 0)) * len(ties), *jobs)
            prods = []
            for load in dots:
                if len(prods) == start:
                    fence()
                lhs, rhs = load()
                for r0, c0 in ties if len(prods) >= start else ():
                    lhs = side.tie(lhs, r0, c0)
                prods.append(_dot(_unpack(lhs), _unpack(rhs)))
            return prods

        hk, hn, hm = H * DH // 4, D // 2, P0 // 2

        def wo_op(p, j):
            if p == 3:
                return pool[j], 0, 0
            if p in (1, 4):
                return wo_b, hk * (p // 4), hn * (p // 4) + C4 * j
            return woe[{0: 0, 2: 1, 5: 2, 6: 0}[p]], 0, C4 * j

        def encode_wo(ps):
            for i0 in range(0, hk, 8):
                for j in range(2):
                    get = functools.cache(lambda k, a, b: _unzip(wo_b[
                        later(hk * a + i0 + 8 * ps[0] * zero, 8), pl.ds(hn * b + C4 * j, C4)], k))
                    ops = [_zip(*[_combine(functools.partial(get, k), SB[p]) for k in range(2)])
                           for p in ps]
                    for p, w in zip(ps, ops):
                        ref, r0, c0 = wo_op(p, j)
                        ref[pl.ds(r0 + i0, 8), pl.ds(c0, C4)] = w
                    yield [(wo_op(p, j)[0], (0,)) for p in ps]

        def encode_o(n):
            for kt in range(H // 2):
                for s in range(hm // 16):
                    pool[n][pl.ds(hm // 2 * (kt // 2) + 8 * s, 8), pl.ds(kt % 2 * 128, 128)] = (
                        _zip(*[_combine(
                            lambda a, b: q_r[H // 2 * b + kt][pl.ds(
                                (done + hm * a + 16 * s) % RING + k + n * zero, 8, stride=2), :],
                            SA[ORDER_B[n]]) for k in range(2)]))
                    if s % 4 == 3:
                        yield [(pool[n], (0,))]

        def wo_dots(n):
            def load(j, i):
                ref, r0, c0 = wo_op(ORDER_B[n], j)
                lhs = [pool[n][later(hm // 2 * c + hm // 4 * i + 8 * j * zero, hm // 4), :]
                       for c in range(8)]
                return (jnp.concatenate(lhs, axis=1),
                        ref[later(r0 + 8 * i * zero, hk), pl.ds(c0, C4)])
            return [functools.partial(load, j, i) for j, i in QUAD]

        def decode_wo(n, prods):
            for (j, i), v in zip(QUAD, prods):
                for r in range(0, hm // 2, 16):
                    for (a, b), sign in SC[ORDER_B[n]]:
                        fresh = all(key != (a, b) for q in ORDER_B[:n] for key, _ in SC[q])
                        row = done + hm * a + hm // 2 * i + r
                        for k in range(2):
                            c = 4 * b + 2 * j + k
                            old = (xs[pl.ds(row, 16), pl.ds(128 * c, 128)].astype(f32) if fresh
                                   else hbuf[c, later(row + 8 * n * zero, 16), :])
                            new = v[r:r + 16, 128 * k:128 * (k + 1)]
                            hbuf[c, pl.ds(row, 16), :] = old + new if sign > 0 else old - new
                    yield [(hbuf, (0, 0))]

        hsb = wo_b

        def norm_in():
            def first_norm(r, x, y):
                woe[2][pl.ds(r, 16), :] = pltpu.bitcast(y[:, :hn], u32)
                woe[2][pl.ds(P0 + r, 16), :] = pltpu.bitcast(y[:, hn:], u32)
                return [(woe[2], (r,))]

            def second_norm(r, x, y):
                ue[pl.ds(r // 2, 8), :] = _pack(y)
                return [(ue, (0,))]

            yield from _ln_job(
                lambda r, n, k: _rows(hbuf, later(done + r + 8 * (7 + k) * zero, n)),
                first_norm, P0, NORM_ROWS, *stats[:2], zero)
            yield from _ln_job(
                lambda r, n, k: pltpu.bitcast(jnp.concatenate(
                    [woe[2][later(r0 + r + 8 * k * zero, n), :] for r0 in (0, P0)], axis=1), f32),
                second_norm, P0, NORM_ROWS, *stats[2:], zero)

        def in_dots(lhs, cols, n=0):
            return [lambda c=c: (lhs(c), w1b[c // 2, later(8 * n * zero, D // 2),
                                             pl.ds(128 * (c % 2), 128)]) for c in cols]

        def gelu_in(r0, cols, prods):
            for c, v in zip(cols, prods):
                for r in range(0, v.shape[0], 32):
                    xg[c, pl.ds(HALO + r0 + r, 32), :] = _gelu(v[r:r + 32])
                    yield [(xg, (c, HALO + r0))]

        def encode_g(i):
            for s in range(RB // 32):
                for kt in range(4):
                    get = functools.cache(lambda k, a, b: xg[4 * b + kt, pl.ds(
                        HALO + i * RB + RB // 2 * a + 16 * s + k + SHIFT[2 * b + kt // 2],
                        8, stride=2), :])
                    for p in range(7):
                        pool[i - 1][pl.ds(128 * p + 64 * (kt // 2) + 8 * s, 8),
                                    pl.ds(128 * (kt % 2), 128)] = _zip(
                            *[_combine(functools.partial(get, k), SA[p]) for k in range(2)])
                    yield [(pool[i - 1], (0,))]

        def out_dots(i, j):
            return [lambda p=p: (
                jnp.concatenate([pool[i - 1][later(128 * p + 64 * k + 8 * j * zero, 64), :]
                                 for k in range(2)], axis=1),
                we[w2_slot(p, j, 8 * (i + 1) * zero)]) for p in range(7)]

        def decode_out(i, j, prods):
            for r0 in range(0, RB // 2, 8):
                out = {}
                for p in range(7):
                    for key, sign in SC[p]:
                        _accumulate(out, key, sign, prods[p][r0:r0 + 8])
                for (a, b), v in out.items():
                    hsb[pl.ds(i * RB + RB // 2 * a + r0, 8),
                        pl.ds(hn * b + 128 * j, 128)] = pltpu.bitcast(v, u32)
                yield [(hsb, (i * RB,))]

        def encode_w4():
            for c in range(NC - 1):
                for i0 in range(0, 64, 8):
                    for j in range(2):
                        at = (c, pl.ds(i0, 8), pl.ds(128 * j, 128))
                        raw = {(a, b): w4e[(4 * a + b,) + at]
                               for a in range(4) for b in range(4)}
                        get = functools.cache(lambda k, a, b: _unzip(raw[a, b], k))
                        for p in ORDER_B:
                            for r, w in enumerate(_encode7(SB, p, get)):
                                w4e[(7 * p + r,) + at] = w
                            yield [(w4e, (0, c, i0))]

        def mixer_post(r0, zero, group):
            def first_norm(r, hv, y):
                rows = pl.ds(_mult(r0 + r, 8), 16)
                x1 = y + pltpu.bitcast(hsb[rows, :], f32)
                _set_rows(xg, rows, hv + x1)
                _set_rows(ybuf, pl.ds(r, 16), x1)
                return [(ybuf, (0, 0)), (xg, (0, r0))]

            def second_norm(r, x1, y):
                _set_rows(hbuf, pl.ds(_mult(r0 + r, 8), 16), y)
                return [(hbuf, (0, r0))]

            at = lambda r, n, k: pl.ds(pl.multiple_of(r + 8 * k * zero, 8), n)
            yield from _ln_job(lambda r, n, k: _rows(hbuf, at(r0 + r, n, k)),
                               first_norm, RB, group, *stats[:2], zero)
            yield from _ln_job(lambda r, n, k: _rows(ybuf, at(r, n, k + 1)),
                               second_norm, RB, group, *stats[2:], zero)
            for s in range(4):
                for kt in range(2):
                    get = functools.cache(lambda k, a, b: hbuf[2 * b + kt, pl.ds(
                        r0 + R4 * a + 4 * k + 2 * (s % 2) + s // 2, 8, stride=8), :])
                    for p in ORDER_A:
                        for r, w in enumerate(_encode7(SA, p, get)):
                            ye[7 * p + r, pl.ds(8 * s, 8), pl.ds(128 * kt, 128)] = w
                        if p in POST_P:
                            yield [(ye, (0, 8 * s))]

        def out_copies(i):
            rows = pl.ds(_mult(i * (RB // 2), RB // 2), RB // 2)
            return [pltpu.make_async_copy(
                woe[b].at[rows], out_hbm.bitcast(u32).at[rows, pl.ds(hn * b, hn)],
                sems.at[SEM_OUT + 2 * i + b]) for b in range(2)]

        n_g, n_out, n_o = RB // 8, RB // 16, H // 2 * hm // 64
        n_post = RB // 8 + 8 * len(POST_P)
        out_ties = [(r0, TIE_C) for r0 in range(0, 64, 8)]
        wo_ties = [(r0, c0) for c0 in range(TIE_C, 2 * D, 512) for r0 in range(0, 64, 8)]
        in_ties = [(r0, c0) for c0 in (TIE_C, 512 + TIE_C) for r0 in range(0, 64, 8)]
        w4_job = encode_w4()
        wo_jobs = [encode_wo(ps) for ps in ((0,), (2, 5), (3, 6))]

        def mixer_out(i, pending, *jobs):
            for j in range(4):
                prods = run(out_dots(i, j), out_ties, -1 if j else 0, pending,
                            *[(job, count // 4) for job, count in jobs])
                pending = (decode_out(i, j, prods), n_out)
            return pending

        u = _pack(_ln(_ln(_rows(hbuf, pl.ds(first, done - first)))))
        prods = run(in_dots(lambda c: u, range(8)), in_ties[:6], -1, (encode_o(0), n_o))
        pending = (gelu_in(first, range(8), prods), 24)
        for n in range(7):
            jobs = [(encode_o(n + 1), n_o) if n < 6 else (encode_g(0), n_g), pending]
            if n < 5:
                jobs.append((wo_jobs[(n + 1) // 2], hk // 8 if n else hk // 4))
            if n == W4_AT:
                for cp in w4_copies:
                    cp.wait()
            if n >= W4_AT:
                jobs.append((w4_job, 7 * W4_WO))
            prods = run(wo_dots(n), wo_ties, 0, *jobs)
            pending = (decode_wo(n, prods), hm // 8)
        norm = norm_in()
        for i in range(5):
            jobs = [(w4_job, 7 * W4_SPLIT[i])]
            if i < 4:
                jobs.append((encode_g(i + 1), n_g))
            if i > 0:
                jobs.append((norm, P0 // NORM_ROWS + P0 // 32))
            pending = mixer_out(i, pending, *jobs)
        post, g5 = mixer_post(0, zero, NORM_ROWS), encode_g(5)
        for n in range(8):
            r0, cols = done + n // 2 * 128, range(n % 2 * 4, n % 2 * 4 + 4)
            jobs = [pending]
            jobs.append((post, (n_post + 4 * RB // NORM_ROWS) // 8))
            if n >= 6:
                jobs.append((g5, n_g // 2))
            prods = run(in_dots(
                lambda c: ue[later((r0 - done) // 2 + 8 * c * zero, 64), :], cols, n + 1),
                in_ties, -1, *jobs)
            pending = (gelu_in(r0, cols, prods), RB // 16)
        for i in range(5, 8):
            jobs = [(w4_job, 7 * W4_SPLIT[i])]
            if i < 7:
                jobs.append((encode_g(i + 1), n_g))
            pending = mixer_out(i, pending, *jobs)
        list(pending[0])

        def mlp_block(i, carry):
            te = []
            for c in range(NC):
                ops = []
                for r0 in range(0, R4, UP_ROWS):
                    prods = [_dot(_unpack(ye[p, pl.ds(r0 // 2, UP_ROWS // 2), :]), _unpack(
                        we[c, pl.ds(pl.multiple_of(128 * p + r0 * (i >> 3), 8), 128), :]))
                        for p in range(NP)]
                    for s in range(UP_ROWS // 16):
                        act = [{key: _gelu2(v) for key, v in _decode(
                            prods, 32 * (s // 2) + 16 * k + 8 * (s % 2)).items()}
                            for k in range(2)]
                        ops.append(_encode(SA, lambda k, a, b: act[k][a, b]))
                te.append([jnp.concatenate([o[p] for o in ops], axis=0) for p in range(NP)])

            def down(p, lo, hi, tie=lambda w: w):
                lhs = jnp.concatenate([tie(te[c][p]) if c in POST_C else te[c][p]
                                       for c in range(lo, hi)], axis=1)
                rhs = [w4e[p, c - 1] if c else jnp.concatenate(
                    [we[NC + 2, pl.ds(128 * p + 64 * k, 64), :] for k in range(2)], axis=1)
                    for c in range(lo, hi)]
                return _dot(_unpack(lhs), _unpack(jnp.concatenate(rhs, axis=0)))

            prods = [down(p, 0, KSPLIT) for p in range(NSPLIT)]
            prods = [m + down(p, KSPLIT, NC) for p, m in enumerate(prods)]
            out = {}

            def finish(qa, qb):
                for a, b in ((2 * qa + n // 2, 2 * qb + n % 2) for n in range(4)):
                    for r in range(0, R4, 16):
                        row = i * RB + R4 * a + r
                        for j in range(2):
                            woe[qb][pl.ds(pl.multiple_of(row // 2, 8), 8),
                                    pl.ds(C4 * (b % 2) + 128 * j, 128)] = _zip(*[
                                        0.5 * out[a, b][32 * k + r // 2:32 * k + r // 2 + 8,
                                                  128 * j:128 * (j + 1)]
                                        + xg[2 * b + j, pl.ds(row + k, 8, stride=2), :]
                                        for k in range(2)])
                        yield [(woe[qb], (i * (RB // 2),))]

            side = _Side(i >> 3, POST_N * len(POST_C),
                         (mixer_post(((i + 1) & 7) * RB, i >> 3, 0), n_post))
            for p in range(7):
                done_quad = {4: (1, 0), 5: (0, 1), 6: (1, 1)}.get(p)
                store = _Side(i >> 3, 16, *([(finish(*done_quad), 16)] if done_quad else []))
                for q in range(len(prods), 7 * p + 7):
                    side.after(hbuf, prods[q - POST_LAG])
                    prods.append(down(q, 0, NC, side.tie if q % 7 == 0 else
                                      lambda w: store.tie(side.tie(w))))
                _decode7(p, prods[7 * p:7 * p + 7], out)
            list(finish(0, 0))
            for cp in out_copies(i):
                cp.start()
            return carry

        lax.fori_loop(0, S // RB, mlp_block, 0)
        for i in range(S // RB):
            for cp in out_copies(i):
                cp.wait()

    pl.run_scoped(
        tail,
        pltpu.VMEM((NP, NC - 1, 64, C4), u32),
        pltpu.VMEM((NP, R4 // 2, C4), u32),
        pltpu.VMEM((D // 128, RB, 128), f32),
        pltpu.VMEM((P0 // 2, D), u32),
        *[pltpu.VMEM((H * DH // 4, D // 2), u32)] * 3,
        *[pltpu.VMEM((D, C4), u32)] * 8,
    )


@jax.jit
def pallas_sequential_preLN__memory_aug_recurrent_mem_tr__mixer_s_mlp__prompt_kernel(
    A_x: jax.Array,
    A_mem0: jax.Array,
    A_Wq: jax.Array,
    A_Wk: jax.Array,
    A_Wv: jax.Array,
    A_Wo: jax.Array,
    A_seg_len: jax.Array,
    B_x: jax.Array,
    B_w1: jax.Array,
    B_w2: jax.Array,
    B_w3: jax.Array,
    B_w4: jax.Array,
):
    del A_seg_len, B_x
    hbm = pl.BlockSpec(memory_space=pl.ANY)
    vmem = pl.BlockSpec(memory_space=pltpu.VMEM)
    scratch = [
        pltpu.VMEM((H * DH // 2, D), u32),
        pltpu.VMEM((S, D), bf16),
        pltpu.VMEM((D // 128, S + 8, 128), f32),
        pltpu.VMEM((D // 128, S + 2 * HALO, 128), f32),
        pltpu.VMEM((4, D // 2, C4), u32),
        pltpu.VMEM((NC + 3, NP * 128, 128), u32),
        pltpu.SemaphoreType.DMA((NSEM,)),
        pltpu.SemaphoreType.REGULAR,
    ] + [pltpu.VMEM((P0, 128), f32)] * 4 + [pltpu.VMEM((H // 8, RING, DH), f32)] * 8
    out = pl.pallas_call(
        _kernel,
        out_shape=jax.ShapeDtypeStruct((S, D), A_x.dtype),
        in_specs=[hbm, vmem] + [hbm] * 8,
        out_specs=hbm,
        scratch_shapes=scratch,
        compiler_params=pltpu.CompilerParams(vmem_limit_bytes=VMEM_LIMIT),
    )(A_x.reshape(S, D), A_mem0.reshape(MEM, D),
      A_Wq.reshape(D // 2, 2 * H, DH), A_Wk.reshape(D // 2, 2 * H, DH),
      A_Wv.reshape(D // 2, 2 * H, DH),
      A_Wo.reshape(H * DH, D), B_w1, B_w2, B_w3, B_w4.reshape(NC, 4, 128, D))
    return out.reshape(A_x.shape)
```

```python
import functools

import jax
import jax.numpy as jnp
from jax import lax
import jax.experimental.pallas as pl
import jax.experimental.pallas.tpu as pltpu

S = 2048
D = 1024
H = 32
DH = 128
MEM = 8
SEG = 32
F = 3584
NSEG = S // SEG
L = MEM + SEG
TOK = 24
P0 = S - TOK * NSEG
RING = 576
X0 = P0 + 128
C4 = D // 4
SHIFT = (-1, 1, -2, 2)
HALO = 8
RB = 256
R4 = RB // 4
NC = F // 512
NP = 49
EPS = 1e-5
NEG = -1000000000.0

VMEM_LIMIT = 127 * 1024 * 1024 + 896 * 1024

LAG_QK = 2
LAG_PV = 4
LAG_WO = 6
UNROLL = 2
ENC = 4
SIDE_AT = 6
SIDE_N = 50
LN_UNROLL = 2
W_UNROLL = 4
TIE_C = 384
IN_FENCE = (0, -1)
NORM_ROWS = 16
W4_AT = 5
W4_WO = 14
W4_SPLIT = (12, 4, 4, 4, 4, 12, 12, 16)
UP_ROWS = 32
NSPLIT = 5
KSPLIT = 5
POST_C = (1, 3, 5)
POST_N = 44
POST_LAG = 5
POST_P = (0, 6, 5)
assert (7 - W4_AT) * W4_WO + sum(W4_SPLIT) == 16 * (NC - 1)

bf16 = jnp.bfloat16
f32 = jnp.float32
u32 = jnp.uint32

SEM_X0, SEM_X, SEM_W1, SEM_W3, SEM_W4, SEM_WO, SEM_OUT, SEM_W = 0, 3, 4, 5, 6, 7, 11, 27
NSEM = SEM_W + 6

SA = (((0, 0), 1, (1, 1)), ((1, 0), 1, (1, 1)), ((0, 0),), ((1, 1),),
      ((0, 0), 1, (0, 1)), ((1, 0), -1, (0, 0)), ((0, 1), -1, (1, 1)))
SB = (((0, 0), 1, (1, 1)), ((0, 0),), ((0, 1), -1, (1, 1)), ((1, 0), -1, (0, 0)),
      ((1, 1),), ((0, 0), 1, (0, 1)), ((1, 0), 1, (1, 1)))
SC = ((((0, 0), 1), ((1, 1), 1)), (((1, 0), 1), ((1, 1), -1)),
      (((0, 1), 1), ((1, 1), 1)), (((0, 0), 1), ((1, 0), 1)),
      (((0, 0), -1), ((0, 1), 1)), (((1, 1), 1),), (((0, 0), 1),))
ORDER_A = (2, 3, 0, 4, 6, 1, 5)
ORDER_B = (1, 4, 0, 2, 5, 3, 6)
QUAD = ((0, 0), (0, 1), (1, 0), (1, 1))


def _mult(i, n):
    return i if isinstance(i, int) else pl.multiple_of(i, n)


def _ln(x):
    m = jnp.mean(x, axis=-1, keepdims=True)
    d = x - m
    v = jnp.mean(d * d, axis=-1, keepdims=True)
    return d * lax.rsqrt(v + EPS)


def _gelu2(x):
    c = 0.7978845608028654
    return x * jnp.tanh(x * (c + c * 0.044715 * (x * x))) + x


def _gelu(x):
    return 0.5 * _gelu2(x)


def _unpack(x):
    return pltpu.bitcast(x, bf16)


def _dot(a, b):
    return jnp.dot(a, b, preferred_element_type=f32)


def _zip(even, odd):
    return pltpu.bitcast(pltpu.pack_elementwise([even, odd], packed_dtype=bf16), u32)


def _unzip(w, k):
    return pltpu.unpack_elementwise(w, index=k, packed_dtype=bf16, unpacked_dtype=f32)


def _combine(get, term):
    if len(term) == 1:
        return get(*term[0])
    a, b = get(*term[0]), get(*term[2])
    return a + b if term[1] > 0 else a - b


def _encode7(tab, p, get):
    outer = [{(i, j): _combine(lambda a, b: get(k, 2 * a + i, 2 * b + j), tab[p])
              for i, j in QUAD} for k in range(2)]
    return [_zip(*[_combine(lambda a, b: o[a, b], tab[r]) for o in outer])
            for r in range(7)]


def _encode(tab, get):
    get = functools.cache(get)
    ops = {p: _encode7(tab, p, get) for p in (ORDER_A if tab is SA else ORDER_B)}
    return [w for p in range(7) for w in ops[p]]


def _encode1(tab, get):
    get = functools.cache(get)
    return [_zip(*[_combine(functools.partial(get, k), t) for k in range(2)]) for t in tab]


def _decode1(prods):
    out = {}
    for p in range(7):
        for key, sign in SC[p]:
            _accumulate(out, key, sign, prods[p])
    return out


def _accumulate(acc, key, sign, v):
    if key not in acc:
        acc[key] = v
    else:
        acc[key] = acc[key] + v if sign > 0 else acc[key] - v


def _decode7(p, prods, out):
    inner = _decode1(prods)
    for (a, b), sign in SC[p]:
        for (i, j), v in inner.items():
            _accumulate(out, (2 * a + i, 2 * b + j), sign, v)


def _decode(prods, r0):
    out = {}
    for p in range(7):
        _decode7(p, [pltpu.bitcast(m[r0:r0 + 8, :], f32) for m in prods[7 * p:7 * p + 7]],
                 out)
    return out


def _rows(ref, rows):
    return jnp.concatenate([ref[c, rows, :] for c in range(ref.shape[0])], axis=1)


def _set_rows(ref, rows, v):
    for c in range(ref.shape[0]):
        ref[c, rows, :] = v[:, c * 128:(c + 1) * 128]


class _Side:
    def __init__(self, zero, slots, *jobs):
        self.zero = zero
        self.slots = slots
        self.jobs = [[job, count, 0] for job, count in jobs]
        self.at = 0

    def tie(self, w, r0=0, c0=0):
        self.at += 1
        head = old = w[r0:r0 + 8, c0:c0 + 128]
        for job in self.jobs:
            while job[2] * self.slots < min(self.at, self.slots) * job[1]:
                job[2] += 1
                for ref, idx in next(job[0]):
                    row = pl.ds(pl.multiple_of(idx[-1] + 8 * self.zero, 8), 8)
                    seen = ref[idx[:-1] + (row, pl.ds(0, 128))]
                    head = jnp.where(self.zero == 0, head, pltpu.bitcast(seen, u32))
        if head is old:
            return w
        row = [v for v in (w[r0:r0 + 8, :c0] if c0 else None, head,
                           w[r0:r0 + 8, c0 + 128:] if c0 + 128 < w.shape[1] else None)
               if v is not None]
        rows = (w[:r0] if r0 else None, jnp.concatenate(row, axis=1),
                w[r0 + 8:] if r0 + 8 < w.shape[0] else None)
        return jnp.concatenate([v for v in rows if v is not None], axis=0)

    def after(self, ref, r):
        spare = pl.multiple_of(ref.shape[-2] - 8 - 8 * self.zero, 8)
        lead = tuple(n - 1 - self.zero for n in ref.shape[:-2])
        ref[lead + (pl.ds(spare, 8), pl.ds(0, 128))] = pltpu.bitcast(r[:8, :128], ref.dtype)


def _ln_job(load, store, rows, group=0, mean_ref=None, rstd_ref=None, zero=None):
    wide = lambda ref, r, n, k: jnp.concatenate(
        [ref[pl.ds(pl.multiple_of(r + 8 * k * zero, 8), n), :]] * (D // 128), axis=1)
    if not group:
        for r in range(0, rows, 16):
            x = load(r, 16, 0)
            yield store(r, x, _ln(x))
        return
    for r in range(0, rows + 2 * group, group):
        if r < rows:
            m = jnp.mean(load(r, group, 0), axis=-1, keepdims=True)
            mean_ref[pl.ds(r, group), :] = jnp.broadcast_to(m, (group, 128))
            yield [(mean_ref, (r,))]
        if 0 <= r - group < rows:
            d = load(r - group, group, 1) - wide(mean_ref, r - group, group, 1)
            v = jnp.mean(d * d, axis=-1, keepdims=True)
            rstd_ref[pl.ds(r - group, group), :] = jnp.broadcast_to(
                lax.rsqrt(v + EPS), (group, 128))
            yield [(rstd_ref, (r - group,))]
        for q in range(r - 2 * group, r - group, 16) if r >= 2 * group else ():
            x = load(q, 16, 2)
            yield store(q, x, (x - wide(mean_ref, q, 16, 2)) * wide(rstd_ref, q, 16, 2))


def _kernel(x_hbm, mem0_ref, wq_hbm, wk_hbm, wv_hbm, wo_hbm, w1_hbm, w2_hbm,
            w3_hbm, w4_hbm, out_hbm,
            wo_b, xs, hbuf, xg, w1e, we, sems, fence_sem, *bufs):
    stats, q_rings = bufs[:4], bufs[4:]
    w_hbm = (wq_hbm, wk_hbm, wv_hbm)
    q_r = [q_rings[h % 8].at[h // 8] for h in range(H)]

    def x0_copies(k):
        rows = ([pl.ds(P0 // 4 * a + P0 // 8 * k, P0 // 8) for a in range(4)] if k < 2
                else [pl.ds(P0, X0 - P0)])
        return [pltpu.make_async_copy(x_hbm.at[r], xs.at[r], sems.at[SEM_X0 + k])
                for r in rows]

    x_copy = pltpu.make_async_copy(x_hbm.at[pl.ds(X0, S - X0)], xs.at[pl.ds(X0, S - X0)],
                                   sems.at[SEM_X])

    def wo_copy(i):
        rows = pl.ds(_mult(i * 512, 512), 512)
        return pltpu.make_async_copy(wo_hbm.bitcast(u32).at[rows], wo_b.at[rows],
                                     sems.at[SEM_WO + i])

    w3_copies = [pltpu.make_async_copy(
        w3_hbm.bitcast(u32).at[:, pl.ds((4 * c + b) * 128, 128)],
        we.at[c, pl.ds(b * 512, 512)], sems.at[SEM_W3]) for c in range(NC) for b in range(4)]

    def w2_slot(p, j, r0=0, n=D // 4):
        return NC + p // 6, pl.ds(_mult(D * (p % 6) + D // 4 * j + r0, 8), n)

    def early_copies(j):
        return [pltpu.make_async_copy(
            src.bitcast(u32).at[pl.ds(D // 4 * a, D // 4),
                                pl.ds(_mult(D // 2 * b + 128 * j, 128), 128)],
            dst, sems.at[SEM_W1]) for a, b in QUAD for src, dst in (
                (w1_hbm, w1e.at[j, (1, 2, 3, 4)[2 * a + b]]),
                (w2_hbm, we.at[w2_slot(2 * a + b, j)]))] + [
            pltpu.make_async_copy(
                w4_hbm.bitcast(u32).at[0, a, :, pl.ds(_mult(C4 * j + 128 * k, 128), 128)],
                we.at[NC + 2, pl.ds(_mult(128 * (4 * j + a) + 64 * k, 64), 64)],
                sems.at[SEM_W1]) for a in range(4) for k in range(2)]

    def fence():
        pl.semaphore_signal(fence_sem, 1)
        pl.semaphore_wait(fence_sem, 1)

    def block_a(wq_s, wk_s, wv_s, ubuf, useq, tokbuf, lnbuf, *kv_rings):
        w_s = (wq_s, wk_s, wv_s)
        rings = tuple(q_rings) + tuple(kv_rings)
        ring = [[rings[m * 8 + h % 8].at[h // 8] for h in range(H)] for m in range(3)]
        k_r, v_r = ring[1:]

        xe = [we.at[3, pl.ds(128 * p, 128)] for p in range(NP)]
        w_op = (hbuf, xg)

        def start_chunk(g, m):
            for k in range(8):
                pltpu.make_async_copy(
                    w_hbm[m].bitcast(u32).at[:, 16 * (k % 2) + 4 * g + k // 2, :],
                    we.at[m, pl.ds(D // 2 * k, D // 2)],
                    sems.at[SEM_W + 2 * m + k // 4]).start()

        def wait_chunk(m, halves=(0, 1)):
            for half in halves:
                part = we.at[m, pl.ds(2 * D * half, 2 * D)]
                pltpu.make_async_copy(part, part, sems.at[SEM_W + 2 * m + half]).wait()

        def encode_unit(g, m, half, slices):
            h0 = 8 * g + 4 * half
            for i0 in slices:
                blk = {}

                def get(k, a, b):
                    if (k, a, b) not in blk:
                        for par in range(2):
                            w = we[m, pl.ds(_mult(D // 2 * (
                                4 * half + b - b % 2 + par) + 128 * a + i0, 8), 8), :]
                            for j in range(2):
                                blk[par, a, b - b % 2 + j] = _unzip(w, j)
                        for j in (b - b % 2, b - b % 2 + 1):
                            w_s[m][h0 + j, pl.ds(128 * a + i0, 8), :] = _zip(
                                blk[0, a, j], blk[1, a, j])
                    return blk[k, a, b]

                for p in ORDER_B:
                    known = len(blk)
                    for r, w in enumerate(_encode7(SB, p, get)):
                        q = 7 * p + r
                        if len(SB[p]) + len(SB[r]) > 2:
                            w_op[half][1 + q // 16, pl.ds(128 * (q % 16) + i0, 8), :] = (
                                pltpu.bitcast(w, f32))
                    yield [(w_op[half], (1, 0))] + [(w_s[m], (h0, 0))] * (len(blk) > known)

        def operand(g, m, half, q, zero):
            tp, tr = SB[q // 7], SB[q % 7]
            if len(tp) + len(tr) == 2:
                a, b = (2 * tp[0][n] + tr[0][n] for n in range(2))
                return w_s[m][8 * g + 4 * half + b, pl.ds(128 * a, 128), :]
            return w_op[half][1 + q // 16, pl.ds(
                pl.multiple_of(128 * (q % 16) + 8 * zero, 8), 128), :]

        def decode_unit(g, m, half, prods):
            for r0 in range(0, P0 // 4, 8):
                out = _decode(prods, r0)
                for i, j in QUAD:
                    for a, b in QUAD:
                        rings[8 * m + 4 * half + 2 * b + j][
                            g, pl.ds(P0 // 4 * (2 * a + i) + r0, 8), :] = out[2 * a + i, 2 * b + j]
                    yield [(rings[8 * m + 4 * half + 2 * b + j], (g, 0)) for b in range(2)]

        for cp in x0_copies(0) + x0_copies(1):
            cp.start()
        for m in range(3):
            start_chunk(0, m)
        x0_copies(2)[0].start()

        @pl.loop(0, NP)
        def _(p):
            we[4, pl.ds(pl.multiple_of(128 * p, 128), 128), :] = jnp.zeros((128, 128), u32)

        @pl.loop(0, P0 // 64 // LN_UNROLL)
        def _(i):
            for k in range(2):
                @pl.when(i == k * P0 // 128 // LN_UNROLL)
                def _():
                    for cp in x0_copies(k):
                        cp.wait()
            n = 16 * LN_UNROLL
            for a in range(4):
                rows = pl.ds(pl.multiple_of(P0 // 4 * a + n * i, 16), n)
                _set_rows(xg, rows, _ln(xs[rows, :].astype(f32)))
            for s in range(LN_UNROLL):
                for kt in range(2):
                    ops = _encode(SA, lambda k, a, b: xg[2 * b + kt, pl.ds(
                        P0 // 4 * a + n * i + 16 * s + k, 8, stride=2), :])
                    for p, w in enumerate(ops):
                        xe[p][pl.ds(pl.multiple_of(64 * kt + n // 2 * i + 8 * s, 8), 8), :] = w

        wait_chunk(0, (0,))

        @pl.loop(0, 16 // W_UNROLL)
        def _(i):
            list(encode_unit(0, 0, 0, [pl.multiple_of(8 * (W_UNROLL * i + k), 8)
                                       for k in range(W_UNROLL)]))

        wait_chunk(0, (1,))

        def transfers(g, g1, m, half):
            if half == 1:
                if m < 2:
                    wait_chunk(m + 1)
                else:
                    pl.when(g < 3)(functools.partial(wait_chunk, 0))
                pl.when(g < 3)(functools.partial(start_chunk, g1, m))
            elif m > 0:
                fence()
                for cp in early_copies(g) if m == 1 else [wo_copy(g)]:
                    cp.start()

        last = [we.at[4, pl.ds(128 * p, 128)] for p in range(NP)]

        @pl.loop(0, 4)
        def _(g):
            g1 = jnp.minimum(g + 1, 3)
            zero = g >> 2
            pending = decode_unit((g + 3) & 3, 2, 1, last)
            for m in range(3):
                for half in range(2):
                    nxt = (g1, 0, 0) if (m, half) == (2, 1) else (g, m + half, 1 - half)
                    side = _Side(zero, 8 * (NP - 1),
                                 (encode_unit(*nxt, range(0, 128, 8)), 7 * 16), (pending, 64))
                    prods = []
                    for p in range(NP):
                        if p == 1:
                            transfers(g, g1, m, half)
                        lhs = jnp.concatenate(
                            [xe[p][pl.ds(64 * kt, 64), :] for kt in range(2)], axis=1)
                        rhs = operand(g, m, half, p, zero)
                        for k in range(0, 64, 8) if p else ():
                            lhs = side.tie(lhs, k, 128)
                        prods.append(_dot(_unpack(lhs), _unpack(rhs)))
                    pending = decode_unit(g, m, half, prods)
            for p in range(NP):
                last[p][...] = pltpu.bitcast(prods[p], u32)

        list(decode_unit(3, 2, 1, last))

        x_copy.start()
        x0_copies(2)[0].wait()
        tokbuf[...] = _ln(xs[pl.ds(P0, UNROLL * TOK), :].astype(f32))
        _set_rows(xg, pl.ds(0, HALO), jnp.zeros((HALO, D), f32))
        _set_rows(xg, pl.ds(HALO + S, HALO), jnp.zeros((HALO, D), f32))
        _set_rows(hbuf, pl.ds(0, UNROLL * TOK), jnp.zeros((UNROLL * TOK, D), f32))
        _set_rows(useq, pl.ds(2 * TOK, 2 * TOK), jnp.zeros((2 * TOK, D), f32))
        for cp in w3_copies:
            cp.start()
        for i in range(4):
            for cp in early_copies(i):
                cp.wait()

        @pl.loop(0, 4)
        def _(j):
            for r in range(0, D // 4, 16):
                raw = {key: w1e[j, 1 + n, pl.ds(r, 16), :] for n, key in enumerate(QUAD)}
                ops = _encode1(SB, lambda k, a, b: _unzip(raw[a, b], k))
                for p in (0, 2, 3, 5, 6):
                    w1e[j, p, pl.ds(r, 16), :] = ops[p]

        for i in range(4):
            wo_copy(i).wait()

        def wrap(r):
            return jnp.where(r >= RING, r - RING, r)

        def step(s, carry, tok, side, last):
            mem, rp, ra, rw = carry
            ri = lax.broadcasted_iota(jnp.int32, (2 * MEM + SEG, 2 * L), 0)
            ci = lax.broadcasted_iota(jnp.int32, (2 * MEM + SEG, 2 * L), 1)
            key_b = ((ci >= MEM) & (ci < 2 * MEM)) | (ci >= 2 * MEM + SEG)
            same = key_b == ((ri >= MEM) & (ri < 2 * MEM))
            mask = same & ((ri < 2 * MEM) | (ri >= ci))
            fill = jnp.where(same, NEG, -jnp.inf)

            lhs = jnp.concatenate([mem, tok], axis=0).astype(bf16)
            rps = [pl.multiple_of(wrap(rp + 8 * i), 8) for i in range(3)]
            ra_ = pl.multiple_of(ra, SEG)
            rw_ = pl.multiple_of(rw, 8)

            col = s & 3
            group = jnp.maximum((s >> 2) - 1, 0)
            rb = pl.multiple_of(group * (4 * TOK), 8)

            mem_qkv = {}
            scores = {}
            o_mem = {}
            total = [None]

            def qkv(h):
                for m in range(3):
                    w = w_s[m][h]
                    r = _dot(lhs, _unpack(side.tie(w, D // 4) if h >= SIDE_AT else w))
                    for i in range(3):
                        ring[m][h][pl.ds(rps[i], 8), :] = r[8 + 8 * i:16 + 8 * i]
                    mem_qkv[m, h] = r[:MEM]

            def segment(m, pair):
                a, b = 2 * pair, 2 * pair + 1
                ma, mb = mem_qkv.pop((m, a)), mem_qkv.pop((m, b))
                xa, xb = (ring[m][h][pl.ds(ra_, SEG), :] for h in (a, b))
                if m == 0:
                    parts = ((ma, mb, xa), (xb,))
                else:
                    parts = ((ma, mb, xa, xb), (mb, ma, xb))
                return [jnp.concatenate(v, axis=0).astype(bf16) for v in parts]

            def qk(pair):
                q, k = segment(0, pair), segment(1, pair)
                for n in range(2):
                    scores[pair, n] = lax.dot_general(
                        q[n], k[n], (((1,), (1,)), ((), ())), preferred_element_type=f32)

            def pv(pair):
                v = segment(2, pair)
                for n in range(2):
                    sc = scores.pop((pair, n)) * (DH ** -0.5)
                    if n == 0:
                        sc = jnp.where(mask, sc, fill)
                    else:
                        sc = jnp.where(mask[2 * MEM:, :2 * MEM + SEG], sc,
                                       fill[2 * MEM:, :2 * MEM + SEG])
                    mx = jnp.max(sc, axis=1, keepdims=True)
                    e = jnp.exp(sc - mx)
                    den = jnp.sum(e, axis=1, keepdims=True)
                    inv = pl.reciprocal(den, approx=True)
                    inv = inv * (2.0 - den * inv)
                    o = _dot(e.astype(bf16), v[n]) * inv
                    q_r[2 * pair + n][pl.ds(ra_, SEG), :] = o[-SEG:]
                    if n == 0:
                        o_mem[2 * pair], o_mem[2 * pair + 1] = o[:MEM], o[MEM:2 * MEM]

            def wo(h):
                lo = jnp.concatenate([o_mem.pop(h), q_r[h][pl.ds(rw_, TOK), :]],
                                     axis=0).astype(bf16)
                r = _dot(lo, _unpack(wo_b[pl.ds(h * DH // 2, DH // 2), :]))
                total[0] = r if total[0] is None else total[0] + r

            npair = H // 2
            for t in range(npair + LAG_WO):
                if 0 <= t - LAG_QK < npair:
                    qk(t - LAG_QK)
                if 0 <= t - LAG_PV < npair:
                    pv(t - LAG_PV)
                if t < npair:
                    qkv(2 * t)
                    qkv(2 * t + 1)
                if 0 <= t - LAG_WO < npair:
                    wo(2 * (t - LAG_WO))
                    wo(2 * (t - LAG_WO) + 1)
            fills = [_dot(_unpack(ubuf[p]), _unpack(w1e[col, p])) for p in range(7)]
            for (a, b), v in _decode1(fills).items():
                xg[4 * b + col, pl.ds(HALO + rb + 2 * TOK * a, 2 * TOK), :] = (
                    v if last and a == b else _gelu(v))

            a = total[0]
            return (a[:MEM], wrap(rp + TOK), wrap(ra + SEG), wrap(rw + TOK)), a[MEM:]

        def late_gelu(s):
            rb = jnp.maximum((s >> 2) - 1, 0) * (4 * TOK)
            for a in range(2):
                at = (4 * a + (s & 3),
                      pl.ds(pl.multiple_of(HALO + rb + 2 * TOK * a, 8), 2 * TOK))
                xg[at] = _gelu(xg[at])
            yield [(xg, (s & 3, HALO + rb))]

        def steps(i, carry):
            n = UNROLL * TOK
            pl.when(i == 1)(x_copy.wait)

            @pl.when(i == 16 // ENC)
            def _():
                raw = we.at[pl.ds(0, NC), pl.ds(0, 4 * 512)]
                pltpu.make_async_copy(raw, raw, sems.at[SEM_W3]).wait()

            zero = i >> 5
            at = lambda r, m, k: pl.ds(pl.multiple_of(r + 16 * k * zero, 16), m)

            def norm_filler():
                prev = jnp.maximum(i - 1, 0)

                def first_norm(r, x, y):
                    lnbuf[pl.ds(r, 16), :] = y
                    return [(lnbuf, (r,))]

                def second_norm(r, x, y):
                    dst = pl.multiple_of(n * (prev & 3) + r, 8)
                    _set_rows(useq, pl.ds(dst, 16), y)
                    return [(useq, (0, dst))]

                yield from _ln_job(lambda r, m, k: _rows(hbuf, at(n * prev + r, m, k)),
                                   first_norm, n)
                yield from _ln_job(lambda r, m, k: lnbuf[at(r, m, k + 2), :],
                                   second_norm, n)
                base = (jnp.maximum((UNROLL * i >> 2) - 1, 0) & 1) * (2 * n)
                for r in range(0, n, 16):
                    for kt in range(4):
                        ops = _encode1(SA, lambda k, a, b: useq[
                            4 * b + kt, pl.ds(base + n * a + r + k, 8, stride=2), :])
                        for p, w in enumerate(ops):
                            ubuf[p, pl.ds(r // 2, 8), pl.ds(128 * kt, 128)] = w
                        if kt % 2:
                            yield [(ubuf, (0, 0))]

            def norm_tokens():
                def keep(r, x, y):
                    tokbuf[pl.ds(r, 16), :] = y
                    return [(tokbuf, (r,))]

                nxt = jnp.minimum(P0 + n * (i + 1), S - n)
                return _ln_job(lambda r, m, k: xs[at(nxt + r, m, k), :].astype(f32),
                               keep, n)

            def encode_b():
                for j in range(4):
                    raw = {(a, b): we[w2_slot(2 * a + b, j, 8 * i, 8)] for a, b in QUAD}
                    for p, w in enumerate(_encode1(SB, lambda k, a, b: _unzip(raw[a, b], k))):
                        we[w2_slot(p, j, 8 * i, 8)] = w
                    yield [(we, (NC, 8 * i))]
                for k in range(ENC):
                    j = ENC * i + k
                    grp, i0 = jnp.where(j < 16, NC + 2, (j >> 4) - 1), 8 * (j & 15)
                    slot = lambda q: (grp, pl.ds(pl.multiple_of(128 * q + i0, 8), 8))
                    raw = {(a, b): we[slot(4 * b + a)] for a in range(4) for b in range(4)}
                    get = functools.cache(lambda k, a, b: _unzip(raw[a, b], k))
                    for p in ORDER_B:
                        for r, w in enumerate(_encode7(SB, p, get)):
                            we[slot(7 * p + r)] = w
                        yield [(we, (grp, i0))]

            jobs = [[(norm_filler(), 4 * n // 16), (late_gelu(jnp.maximum(UNROLL * i - 1, 0)), 1)],
                    [(encode_b(), 4 + 7 * ENC), (norm_tokens(), n // 16)]]
            for k in range(UNROLL):
                s = i * UNROLL + k
                carry, o = step(s, carry, tokbuf[pl.ds(k * TOK, TOK), :],
                                _Side(zero, SIDE_N, *jobs[k]), k == UNROLL - 1)
                lo = k * TOK // 16 * 16
                xv = xs[pl.ds(pl.multiple_of(n * i + lo, 16), 32), :].astype(f32)
                _set_rows(hbuf, pl.ds(pl.multiple_of(TOK * s, 8), TOK),
                          xv[k * TOK - lo:(k + 1) * TOK - lo] + o)
            return carry

        carry = (mem0_ref[...].astype(f32), jnp.int32(P0), jnp.int32(0), jnp.int32(0))
        carry = lax.fori_loop(0, NSEG // UNROLL, steps, carry)
        list(late_gelu(jnp.int32(NSEG - 1)))
        return carry[1] >> 16

    zero = pl.run_scoped(
        block_a,
        *[pltpu.VMEM((H, D // 2, DH), u32)] * 3,
        pltpu.VMEM((7, TOK, D // 2), u32),
        pltpu.VMEM((D // 128, 8 * TOK, 128), f32),
        pltpu.VMEM((UNROLL * TOK, D), f32),
        pltpu.VMEM((UNROLL * TOK, D), f32),
        *[pltpu.VMEM((H // 8, RING, DH), f32)] * 16,
    )

    def tail(w4e, ye, ybuf, *bufs):
        woe, pool = bufs[:3], bufs[3:]
        w4_copies = [
            pltpu.make_async_copy(w4_hbm.bitcast(u32).at[pl.ds(1, NC - 1), a, :, pl.ds(b * C4, C4)],
                                  w4e.at[4 * a + b], sems.at[SEM_W4])
            for a in range(4) for b in range(4)]
        for cp in w4_copies:
            cp.start()
        done = TOK * NSEG
        first = 4 * TOK * (NSEG // 4 - 1)

        def later(rows, n):
            return pl.ds(pl.multiple_of(rows + 8 * zero, 8), n)

        def run(dots, ties, start, *jobs):
            side = _Side(zero, (len(dots) - max(start, 0)) * len(ties), *jobs)
            prods = []
            for load in dots:
                if len(prods) == start:
                    fence()
                lhs, rhs = load()
                for r0, c0 in ties if len(prods) >= start else ():
                    lhs = side.tie(lhs, r0, c0)
                prods.append(_dot(_unpack(lhs), _unpack(rhs)))
            return prods

        hk, hn, hm = H * DH // 4, D // 2, P0 // 2

        def wo_op(p, j):
            if p == 3:
                return pool[j], 0, 0
            if p in (1, 4):
                return wo_b, hk * (p // 4), hn * (p // 4) + C4 * j
            return woe[{0: 0, 2: 1, 5: 2, 6: 0}[p]], 0, C4 * j

        def encode_wo(ps):
            for i0 in range(0, hk, 8):
                for j in range(2):
                    get = functools.cache(lambda k, a, b: _unzip(wo_b[
                        later(hk * a + i0 + 8 * ps[0] * zero, 8), pl.ds(hn * b + C4 * j, C4)], k))
                    ops = [_zip(*[_combine(functools.partial(get, k), SB[p]) for k in range(2)])
                           for p in ps]
                    for p, w in zip(ps, ops):
                        ref, r0, c0 = wo_op(p, j)
                        ref[pl.ds(r0 + i0, 8), pl.ds(c0, C4)] = w
                    yield [(wo_op(p, j)[0], (0,)) for p in ps]

        def encode_o(n):
            for kt in range(H // 2):
                for s in range(hm // 16):
                    pool[n][pl.ds(hm // 2 * (kt // 2) + 8 * s, 8), pl.ds(kt % 2 * 128, 128)] = (
                        _zip(*[_combine(
                            lambda a, b: q_r[H // 2 * b + kt][pl.ds(
                                (done + hm * a + 16 * s) % RING + k + n * zero, 8, stride=2), :],
                            SA[ORDER_B[n]]) for k in range(2)]))
                    if s % 4 == 3:
                        yield [(pool[n], (0,))]

        def wo_dots(n):
            def load(j, i):
                ref, r0, c0 = wo_op(ORDER_B[n], j)
                lhs = [pool[n][later(hm // 2 * c + hm // 4 * i + 8 * j * zero, hm // 4), :]
                       for c in range(8)]
                return (jnp.concatenate(lhs, axis=1),
                        ref[later(r0 + 8 * i * zero, hk), pl.ds(c0, C4)])
            return [functools.partial(load, j, i) for j, i in QUAD]

        def decode_wo(n, prods):
            for (j, i), v in zip(QUAD, prods):
                for r in range(0, hm // 2, 16):
                    for (a, b), sign in SC[ORDER_B[n]]:
                        fresh = all(key != (a, b) for q in ORDER_B[:n] for key, _ in SC[q])
                        row = done + hm * a + hm // 2 * i + r
                        for k in range(2):
                            c = 4 * b + 2 * j + k
                            old = (xs[pl.ds(row, 16), pl.ds(128 * c, 128)].astype(f32) if fresh
                                   else hbuf[c, later(row + 8 * n * zero, 16), :])
                            new = v[r:r + 16, 128 * k:128 * (k + 1)]
                            hbuf[c, pl.ds(row, 16), :] = old + new if sign > 0 else old - new
                    yield [(hbuf, (0, 0))]

        hsb = wo_b

        def norm_in():
            def first_norm(r, x, y):
                woe[2][pl.ds(r, 16), :] = pltpu.bitcast(y[:, :hn], u32)
                woe[2][pl.ds(P0 + r, 16), :] = pltpu.bitcast(y[:, hn:], u32)
                return [(woe[2], (r,))]

            def second_norm(r, x, y):
                _set_rows(xg, pl.ds(HALO + done + r, 16), y)
                return [(xg, (0, HALO + done))]

            yield from _ln_job(
                lambda r, n, k: _rows(hbuf, later(done + r + 8 * (7 + k) * zero, n)),
                first_norm, P0, NORM_ROWS, *stats[:2], zero)
            yield from _ln_job(
                lambda r, n, k: pltpu.bitcast(jnp.concatenate(
                    [woe[2][later(r0 + r + 8 * k * zero, n), :] for r0 in (0, P0)], axis=1), f32),
                second_norm, P0, NORM_ROWS, *stats[2:], zero)

        def encode_rows(buf, r0, n, shift=(0, 0, 0, 0)):
            for r in range(0, n // 2, 16):
                for kt in range(4):
                    ops = _encode1(SA, lambda k, a, b: xg[4 * b + kt, pl.ds(
                        HALO + r0 + n // 2 * a + r + k + shift[2 * b + kt // 2],
                        8, stride=2), :])
                    for p, w in enumerate(ops):
                        buf[pl.ds(128 * p + 64 * (kt // 2) + r // 2, 8),
                            pl.ds(128 * (kt % 2), 128)] = w
                    yield [(buf, (0,))]

        def encode_g(i):
            return encode_rows(pool[i - 1], i * RB, RB, SHIFT)

        def mixer(buf, n, weights, store, start, pending, *jobs):
            def decode(j, prods):
                for r in range(0, n // 2, 8):
                    for (a, b), v in _decode1([m[r:r + 8] for m in prods]).items():
                        seen = store(n // 2 * a + r, 4 * b + j, v)
                    yield seen

            for j in range(4):
                dots = [lambda p=p: (
                    jnp.concatenate([buf[later(128 * p + 64 * k + 8 * j * zero, n // 4), :]
                                     for k in range(2)], axis=1),
                    weights(p, j)) for p in range(7)]
                prods = run(dots, [(r, TIE_C) for r in range(0, n // 4, 8)],
                            -1 if j else start, pending,
                            *[(job, count // 4) for job, count in jobs])
                pending = (decode(j, prods), n // 16)
            return pending

        def mixer_in(buf, r0, n, *args):
            def store(r, c, v):
                xg[c, pl.ds(HALO + r0 + r, 8), :] = _gelu(v)
                return [(xg, (0, HALO + r0))]

            return mixer(buf, n, lambda p, j: w1e[j, p, later(r0 * zero, D // 4), :],
                         store, *args)

        def mixer_out(i, *args):
            def store(r, c, v):
                hsb[pl.ds(i * RB + r, 8), pl.ds(128 * c, 128)] = pltpu.bitcast(v, u32)
                return [(hsb, (i * RB,))]

            return mixer(pool[i - 1], RB, lambda p, j: we[w2_slot(p, j, 8 * (i + 1) * zero)],
                         store, 0, *args)

        def encode_w4():
            for c in range(NC - 1):
                for i0 in range(0, 64, 8):
                    for j in range(2):
                        at = (c, pl.ds(i0, 8), pl.ds(128 * j, 128))
                        raw = {(a, b): w4e[(4 * a + b,) + at]
                               for a in range(4) for b in range(4)}
                        get = functools.cache(lambda k, a, b: _unzip(raw[a, b], k))
                        for p in ORDER_B:
                            for r, w in enumerate(_encode7(SB, p, get)):
                                w4e[(7 * p + r,) + at] = w
                            yield [(w4e, (0, c, i0))]

        def mixer_post(r0, zero, group):
            def first_norm(r, hv, y):
                rows = pl.ds(_mult(r0 + r, 8), 16)
                x1 = y + pltpu.bitcast(hsb[rows, :], f32)
                _set_rows(xg, rows, hv + x1)
                _set_rows(ybuf, pl.ds(r, 16), x1)
                return [(ybuf, (0, 0)), (xg, (0, r0))]

            def second_norm(r, x1, y):
                _set_rows(hbuf, pl.ds(_mult(r0 + r, 8), 16), y)
                return [(hbuf, (0, r0))]

            at = lambda r, n, k: pl.ds(pl.multiple_of(r + 8 * k * zero, 8), n)
            yield from _ln_job(lambda r, n, k: _rows(hbuf, at(r0 + r, n, k)),
                               first_norm, RB, group, *stats[:2], zero)
            yield from _ln_job(lambda r, n, k: _rows(ybuf, at(r, n, k + 1)),
                               second_norm, RB, group, *stats[2:], zero)
            for s in range(4):
                for kt in range(2):
                    get = functools.cache(lambda k, a, b: hbuf[2 * b + kt, pl.ds(
                        r0 + R4 * a + 4 * k + 2 * (s % 2) + s // 2, 8, stride=8), :])
                    for p in ORDER_A:
                        for r, w in enumerate(_encode7(SA, p, get)):
                            ye[7 * p + r, pl.ds(8 * s, 8), pl.ds(128 * kt, 128)] = w
                        if p in POST_P:
                            yield [(ye, (0, 8 * s))]

        def out_copies(i):
            rows = pl.ds(_mult(i * RB, RB), RB)
            return [pltpu.make_async_copy(
                woe[b].bitcast(bf16).at[rows], out_hbm.at[rows, pl.ds(hn * b, hn)],
                sems.at[SEM_OUT + 2 * i + b]) for b in range(2)]

        n_g, n_o = RB // 8, H // 2 * hm // 64
        n_post = RB // 8 + 8 * len(POST_P)
        wo_ties = [(r0, c0) for c0 in range(TIE_C, 2 * D, 512) for r0 in range(0, 64, 8)]
        w4_job = encode_w4()
        wo_jobs = [encode_wo(ps) for ps in ((0,), (2, 5), (3, 6))]

        _set_rows(xg, pl.ds(HALO + first, done - first),
                  _ln(_ln(_rows(hbuf, pl.ds(first, done - first)))))
        list(encode_rows(pool[7], first, done - first))
        pending = mixer_in(pool[7], first, done - first, -1, (None, 0), (encode_o(0), n_o))
        for n in range(7):
            jobs = [(encode_o(n + 1), n_o) if n < 6 else (encode_g(0), n_g), pending]
            if n < 5:
                jobs.append((wo_jobs[(n + 1) // 2], hk // 8 if n else hk // 4))
            if n == W4_AT:
                for cp in w4_copies:
                    cp.wait()
            if n >= W4_AT:
                jobs.append((w4_job, 7 * W4_WO))
            prods = run(wo_dots(n), wo_ties, 0, *jobs)
            pending = (decode_wo(n, prods), hm // 8)
        norm = norm_in()
        for i in range(5):
            jobs = [(w4_job, 7 * W4_SPLIT[i])]
            jobs.append((encode_g(i + 1) if i < 4 else encode_rows(pool[7], done, RB), n_g))
            if i > 0:
                jobs.append((norm, P0 // NORM_ROWS + P0 // 32))
            pending = mixer_out(i, pending, *jobs)
        post = (mixer_post(0, zero, NORM_ROWS), (n_post + 4 * RB // NORM_ROWS) // 2)
        pending = mixer_in(pool[7], done, RB, IN_FENCE[0], pending, post,
                           (encode_rows(pool[0], done + RB, RB), n_g))
        pending = mixer_in(pool[0], done + RB, RB, IN_FENCE[1], pending, post,
                           (encode_g(5), n_g))
        for i in range(5, 8):
            jobs = [(w4_job, 7 * W4_SPLIT[i])]
            if i < 7:
                jobs.append((encode_g(i + 1), n_g))
            pending = mixer_out(i, pending, *jobs)
        list(pending[0])

        def mlp_block(i, carry):
            te = []
            for c in range(NC):
                ops = []
                for r0 in range(0, R4, UP_ROWS):
                    prods = [_dot(_unpack(ye[p, pl.ds(r0 // 2, UP_ROWS // 2), :]), _unpack(
                        we[c, pl.ds(pl.multiple_of(128 * p + r0 * (i >> 3), 8), 128), :]))
                        for p in range(NP)]
                    for s in range(UP_ROWS // 16):
                        act = [{key: _gelu2(v) for key, v in _decode(
                            prods, 32 * (s // 2) + 16 * k + 8 * (s % 2)).items()}
                            for k in range(2)]
                        ops.append(_encode(SA, lambda k, a, b: act[k][a, b]))
                te.append([jnp.concatenate([o[p] for o in ops], axis=0) for p in range(NP)])

            def down(p, lo, hi, tie=lambda w: w):
                lhs = jnp.concatenate([tie(te[c][p]) if c in POST_C else te[c][p]
                                       for c in range(lo, hi)], axis=1)
                rhs = [w4e[p, c - 1] if c else jnp.concatenate(
                    [we[NC + 2, pl.ds(128 * p + 64 * k, 64), :] for k in range(2)], axis=1)
                    for c in range(lo, hi)]
                return _dot(_unpack(lhs), _unpack(jnp.concatenate(rhs, axis=0)))

            prods = [down(p, 0, KSPLIT) for p in range(NSPLIT)]
            prods = [m + down(p, KSPLIT, NC) for p, m in enumerate(prods)]
            out = {}

            def finish(qa, qb):
                for a, b in ((2 * qa + n // 2, 2 * qb + n % 2) for n in range(4)):
                    for r in range(0, R4, 16):
                        row = i * RB + R4 * a + r
                        for j in range(2):
                            woe[qb][pl.ds(pl.multiple_of(row // 2, 8), 8),
                                    pl.ds(C4 * (b % 2) + 128 * j, 128)] = _zip(*[
                                        0.5 * out[a, b][32 * k + r // 2:32 * k + r // 2 + 8,
                                                  128 * j:128 * (j + 1)]
                                        + xg[2 * b + j, pl.ds(row + k, 8, stride=2), :]
                                        for k in range(2)])
                        yield [(woe[qb], (i * (RB // 2),))]

            side = _Side(i >> 3, POST_N * len(POST_C),
                         (mixer_post(((i + 1) & 7) * RB, i >> 3, 0), n_post))
            for p in range(7):
                done_quad = {4: (1, 0), 5: (0, 1), 6: (1, 1)}.get(p)
                store = _Side(i >> 3, 16, *([(finish(*done_quad), 16)] if done_quad else []))
                for q in range(len(prods), 7 * p + 7):
                    side.after(hbuf, prods[q - POST_LAG])
                    prods.append(down(q, 0, NC, side.tie if q % 7 == 0 else
                                      lambda w: store.tie(side.tie(w))))
                _decode7(p, prods[7 * p:7 * p + 7], out)
            list(finish(0, 0))
            for cp in out_copies(i):
                cp.start()
            return carry

        lax.fori_loop(0, S // RB, mlp_block, 0)
        for i in range(S // RB):
            for cp in out_copies(i):
                cp.wait()

    pl.run_scoped(
        tail,
        pltpu.VMEM((NP, NC - 1, 64, C4), u32),
        pltpu.VMEM((NP, R4 // 2, C4), u32),
        pltpu.VMEM((D // 128, RB, 128), f32),
        *[pltpu.VMEM((H * DH // 4, D // 2), u32)] * 3,
        *[pltpu.VMEM((D, C4), u32)] * 8,
    )


@jax.jit
def pallas_sequential_preLN__memory_aug_recurrent_mem_tr__mixer_s_mlp__prompt_kernel(
    A_x: jax.Array,
    A_mem0: jax.Array,
    A_Wq: jax.Array,
    A_Wk: jax.Array,
    A_Wv: jax.Array,
    A_Wo: jax.Array,
    A_seg_len: jax.Array,
    B_x: jax.Array,
    B_w1: jax.Array,
    B_w2: jax.Array,
    B_w3: jax.Array,
    B_w4: jax.Array,
):
    del A_seg_len, B_x
    hbm = pl.BlockSpec(memory_space=pl.ANY)
    vmem = pl.BlockSpec(memory_space=pltpu.VMEM)
    scratch = [
        pltpu.VMEM((H * DH // 2, D), u32),
        pltpu.VMEM((S, D), bf16),
        pltpu.VMEM((D // 128, S + 8, 128), f32),
        pltpu.VMEM((D // 128, S + 2 * HALO, 128), f32),
        pltpu.VMEM((4, 7, D // 4, 128), u32),
        pltpu.VMEM((NC + 3, NP * 128, 128), u32),
        pltpu.SemaphoreType.DMA((NSEM,)),
        pltpu.SemaphoreType.REGULAR,
    ] + [pltpu.VMEM((P0, 128), f32)] * 4 + [pltpu.VMEM((H // 8, RING, DH), f32)] * 8
    out = pl.pallas_call(
        _kernel,
        out_shape=jax.ShapeDtypeStruct((S, D), A_x.dtype),
        in_specs=[hbm, vmem] + [hbm] * 8,
        out_specs=hbm,
        scratch_shapes=scratch,
        compiler_params=pltpu.CompilerParams(vmem_limit_bytes=VMEM_LIMIT),
    )(A_x.reshape(S, D), A_mem0.reshape(MEM, D),
      A_Wq.reshape(D // 2, 2 * H, DH), A_Wk.reshape(D // 2, 2 * H, DH),
      A_Wv.reshape(D // 2, 2 * H, DH),
      A_Wo.reshape(H * DH, D), B_w1, B_w2, B_w3, B_w4.reshape(NC, 4, 128, D))
    return out.reshape(A_x.shape)
```

```python
import functools

import jax
import jax.numpy as jnp
from jax import lax
import jax.experimental.pallas as pl
import jax.experimental.pallas.tpu as pltpu

S = 2048
D = 1024
H = 32
DH = 128
MEM = 8
SEG = 32
F = 3584
NSEG = S // SEG
L = MEM + SEG
TOK = 24
P0 = S - TOK * NSEG
RING = 576
X0 = P0 + 128
C4 = D // 4
SHIFT = (-1, 1, -2, 2)
HALO = 8
RB = 256
R4 = RB // 4
NC = F // 512
NP = 49
EPS = 1e-5
NEG = -1000000000.0

VMEM_LIMIT = 127 * 1024 * 1024 + 896 * 1024

LAG_QK = 2
LAG_PV = 4
LAG_WO = 15
UNROLL = 2
ENC = 4
SIDE_AT = 4
SIDE_N = 72
LN_UNROLL = 4
W_UNROLL = 8
TIE_C = 384
IN_FENCE = (0, -1)
NORM_ROWS = 16
W4_AT = 5
W4_WO = 18
W4_SPLIT = (12, 0, 0, 0, 0, 16, 16, 16)
UP_ROWS = 32
NSPLIT = 5
KSPLIT = 5
POST_C = (1, 3, 5)
POST_N = 44
POST_LAG = 5
POST_P = (0, 6, 5)
assert (7 - W4_AT) * W4_WO + sum(W4_SPLIT) == 16 * (NC - 1)

bf16 = jnp.bfloat16
f32 = jnp.float32
u32 = jnp.uint32

SEM_X0, SEM_X, SEM_W1, SEM_W3, SEM_W4, SEM_WO, SEM_OUT, SEM_W = 0, 3, 4, 5, 6, 7, 11, 27
NSEM = SEM_W + 6

SA = (((0, 0), 1, (1, 1)), ((1, 0), 1, (1, 1)), ((0, 0),), ((1, 1),),
      ((0, 0), 1, (0, 1)), ((1, 0), -1, (0, 0)), ((0, 1), -1, (1, 1)))
SB = (((0, 0), 1, (1, 1)), ((0, 0),), ((0, 1), -1, (1, 1)), ((1, 0), -1, (0, 0)),
      ((1, 1),), ((0, 0), 1, (0, 1)), ((1, 0), 1, (1, 1)))
SC = ((((0, 0), 1), ((1, 1), 1)), (((1, 0), 1), ((1, 1), -1)),
      (((0, 1), 1), ((1, 1), 1)), (((0, 0), 1), ((1, 0), 1)),
      (((0, 0), -1), ((0, 1), 1)), (((1, 1), 1),), (((0, 0), 1),))
ORDER_A = (2, 3, 0, 4, 6, 1, 5)
ORDER_B = (1, 4, 0, 2, 5, 3, 6)
QUAD = ((0, 0), (0, 1), (1, 0), (1, 1))


def _mult(i, n):
    return i if isinstance(i, int) else pl.multiple_of(i, n)


def _ln(x):
    m = jnp.mean(x, axis=-1, keepdims=True)
    d = x - m
    v = jnp.mean(d * d, axis=-1, keepdims=True)
    return d * lax.rsqrt(v + EPS)


def _gelu2(x):
    c = 0.7978845608028654
    return x * jnp.tanh(x * (c + c * 0.044715 * (x * x))) + x


def _gelu(x):
    return 0.5 * _gelu2(x)


def _unpack(x):
    return pltpu.bitcast(x, bf16)


def _dot(a, b):
    return jnp.dot(a, b, preferred_element_type=f32)


def _zip(even, odd):
    return pltpu.bitcast(pltpu.pack_elementwise([even, odd], packed_dtype=bf16), u32)


def _unzip(w, k):
    return pltpu.unpack_elementwise(w, index=k, packed_dtype=bf16, unpacked_dtype=f32)


def _combine(get, term):
    if len(term) == 1:
        return get(*term[0])
    a, b = get(*term[0]), get(*term[2])
    return a + b if term[1] > 0 else a - b


def _encode7(tab, p, get):
    outer = [{(i, j): _combine(lambda a, b: get(k, 2 * a + i, 2 * b + j), tab[p])
              for i, j in QUAD} for k in range(2)]
    return [_zip(*[_combine(lambda a, b: o[a, b], tab[r]) for o in outer])
            for r in range(7)]


def _encode(tab, get):
    get = functools.cache(get)
    ops = {p: _encode7(tab, p, get) for p in (ORDER_A if tab is SA else ORDER_B)}
    return [w for p in range(7) for w in ops[p]]


def _encode1(tab, get):
    get = functools.cache(get)
    return [_zip(*[_combine(functools.partial(get, k), t) for k in range(2)]) for t in tab]


def _decode1(prods):
    out = {}
    for p in range(7):
        for key, sign in SC[p]:
            _accumulate(out, key, sign, prods[p])
    return out


def _accumulate(acc, key, sign, v):
    if key not in acc:
        acc[key] = v
    else:
        acc[key] = acc[key] + v if sign > 0 else acc[key] - v


def _decode7(p, prods, out):
    inner = _decode1(prods)
    for (a, b), sign in SC[p]:
        for (i, j), v in inner.items():
            _accumulate(out, (2 * a + i, 2 * b + j), sign, v)


def _decode(prods, r0):
    out = {}
    for p in range(7):
        _decode7(p, [pltpu.bitcast(m[r0:r0 + 8, :], f32) for m in prods[7 * p:7 * p + 7]],
                 out)
    return out


def _rows(ref, rows):
    return jnp.concatenate([ref[c, rows, :] for c in range(ref.shape[0])], axis=1)


def _set_rows(ref, rows, v):
    for c in range(ref.shape[0]):
        ref[c, rows, :] = v[:, c * 128:(c + 1) * 128]


class _Side:
    def __init__(self, zero, slots, *jobs):
        self.zero = zero
        self.slots = slots
        self.jobs = [[job, count, 0] for job, count in jobs]
        self.at = 0

    def tie(self, w, r0=0, c0=0):
        self.at += 1
        head = old = w[r0:r0 + 8, c0:c0 + 128]
        for job in self.jobs:
            while job[2] * self.slots < min(self.at, self.slots) * job[1]:
                job[2] += 1
                for ref, idx in next(job[0]):
                    row = pl.ds(pl.multiple_of(idx[-1] + 8 * self.zero, 8), 8)
                    seen = ref[idx[:-1] + (row, pl.ds(0, 128))]
                    head = jnp.where(self.zero == 0, head, pltpu.bitcast(seen, u32))
        if head is old:
            return w
        row = [v for v in (w[r0:r0 + 8, :c0] if c0 else None, head,
                           w[r0:r0 + 8, c0 + 128:] if c0 + 128 < w.shape[1] else None)
               if v is not None]
        rows = (w[:r0] if r0 else None, jnp.concatenate(row, axis=1),
                w[r0 + 8:] if r0 + 8 < w.shape[0] else None)
        return jnp.concatenate([v for v in rows if v is not None], axis=0)

    def after(self, ref, r):
        spare = pl.multiple_of(ref.shape[-2] - 8 - 8 * self.zero, 8)
        lead = tuple(n - 1 - self.zero for n in ref.shape[:-2])
        ref[lead + (pl.ds(spare, 8), pl.ds(0, 128))] = pltpu.bitcast(r[:8, :128], ref.dtype)


def _ln_job(load, store, rows, group=0, mean_ref=None, rstd_ref=None, zero=None):
    wide = lambda ref, r, n, k: jnp.concatenate(
        [ref[pl.ds(pl.multiple_of(r + 8 * k * zero, 8), n), :]] * (D // 128), axis=1)
    if not group:
        for r in range(0, rows, 16):
            x = load(r, 16, 0)
            yield store(r, x, _ln(x))
        return
    for r in range(0, rows + 2 * group, group):
        if r < rows:
            m = jnp.mean(load(r, group, 0), axis=-1, keepdims=True)
            mean_ref[pl.ds(r, group), :] = jnp.broadcast_to(m, (group, 128))
            yield [(mean_ref, (r,))]
        if 0 <= r - group < rows:
            d = load(r - group, group, 1) - wide(mean_ref, r - group, group, 1)
            v = jnp.mean(d * d, axis=-1, keepdims=True)
            rstd_ref[pl.ds(r - group, group), :] = jnp.broadcast_to(
                lax.rsqrt(v + EPS), (group, 128))
            yield [(rstd_ref, (r - group,))]
        for q in range(r - 2 * group, r - group, 16) if r >= 2 * group else ():
            x = load(q, 16, 2)
            yield store(q, x, (x - wide(mean_ref, q, 16, 2)) * wide(rstd_ref, q, 16, 2))


def _kernel(x_hbm, mem0_ref, wq_hbm, wk_hbm, wv_hbm, wo_hbm, w1_hbm, w2_hbm,
            w3_hbm, w4_hbm, out_hbm,
            wo_b, xs, hbuf, xg, w1e, we, sems, fence_sem, *bufs):
    stats, q_rings = bufs[:4], bufs[4:]
    w_hbm = (wq_hbm, wk_hbm, wv_hbm)
    q_r = [q_rings[h % 8].at[h // 8] for h in range(H)]

    def x0_copies(k):
        rows = ([pl.ds(P0 // 4 * a + P0 // 8 * k, P0 // 8) for a in range(4)] if k < 2
                else [pl.ds(P0, X0 - P0)])
        return [pltpu.make_async_copy(x_hbm.at[r], xs.at[r], sems.at[SEM_X0 + k])
                for r in rows]

    x_copy = pltpu.make_async_copy(x_hbm.at[pl.ds(X0, S - X0)], xs.at[pl.ds(X0, S - X0)],
                                   sems.at[SEM_X])

    def wo_copy(i):
        rows = pl.ds(_mult(i * 512, 512), 512)
        return pltpu.make_async_copy(wo_hbm.bitcast(u32).at[rows], wo_b.at[rows],
                                     sems.at[SEM_WO + i])

    w3_copies = [pltpu.make_async_copy(
        w3_hbm.bitcast(u32).at[:, pl.ds((4 * c + b) * 128, 128)],
        we.at[c, pl.ds(b * 512, 512)], sems.at[SEM_W3]) for c in range(NC) for b in range(4)]

    def w2_slot(p, j, r0=0, n=D // 4):
        return NC + p // 6, pl.ds(_mult(D * (p % 6) + D // 4 * j + r0, 8), n)

    def early_copies(j):
        return [pltpu.make_async_copy(
            src.bitcast(u32).at[pl.ds(D // 4 * a, D // 4),
                                pl.ds(_mult(D // 2 * b + 128 * j, 128), 128)],
            dst, sems.at[SEM_W1]) for a, b in QUAD for src, dst in (
                (w1_hbm, w1e.at[j, (1, 2, 3, 4)[2 * a + b]]),
                (w2_hbm, we.at[w2_slot(2 * a + b, j)]))] + [
            pltpu.make_async_copy(
                w4_hbm.bitcast(u32).at[0, a, :, pl.ds(_mult(C4 * j + 128 * k, 128), 128)],
                we.at[NC + 2, pl.ds(_mult(128 * (4 * j + a) + 64 * k, 64), 64)],
                sems.at[SEM_W1]) for a in range(4) for k in range(2)]

    def fence():
        pl.semaphore_signal(fence_sem, 1)
        pl.semaphore_wait(fence_sem, 1)

    def block_a(wq_s, wk_s, wv_s, ubuf, useq, tokbuf, lnbuf, *kv_rings):
        w_s = (wq_s, wk_s, wv_s)
        rings = tuple(q_rings) + tuple(kv_rings)
        ring = [[rings[m * 8 + h % 8].at[h // 8] for h in range(H)] for m in range(3)]
        k_r, v_r = ring[1:]

        xe = [we.at[3, pl.ds(128 * p, 128)] for p in range(NP)]
        w_op = (hbuf, xg)

        def start_chunk(g, m):
            for k in range(8):
                pltpu.make_async_copy(
                    w_hbm[m].bitcast(u32).at[:, 16 * (k % 2) + 4 * g + k // 2, :],
                    we.at[m, pl.ds(D // 2 * k, D // 2)],
                    sems.at[SEM_W + 2 * m + k // 4]).start()

        def wait_chunk(m, halves=(0, 1)):
            for half in halves:
                part = we.at[m, pl.ds(2 * D * half, 2 * D)]
                pltpu.make_async_copy(part, part, sems.at[SEM_W + 2 * m + half]).wait()

        def encode_unit(g, m, half, slices):
            h0 = 8 * g + 4 * half
            for i0 in slices:
                blk = {}

                def get(k, a, b):
                    if (k, a, b) not in blk:
                        for par in range(2):
                            w = we[m, pl.ds(_mult(D // 2 * (
                                4 * half + b - b % 2 + par) + 128 * a + i0, 8), 8), :]
                            for j in range(2):
                                blk[par, a, b - b % 2 + j] = _unzip(w, j)
                        for j in (b - b % 2, b - b % 2 + 1):
                            w_s[m][h0 + j, pl.ds(128 * a + i0, 8), :] = _zip(
                                blk[0, a, j], blk[1, a, j])
                    return blk[k, a, b]

                for p in ORDER_B:
                    known = len(blk)
                    for r, w in enumerate(_encode7(SB, p, get)):
                        q = 7 * p + r
                        if len(SB[p]) + len(SB[r]) > 2:
                            w_op[half][1 + q // 16, pl.ds(128 * (q % 16) + i0, 8), :] = (
                                pltpu.bitcast(w, f32))
                    yield [(w_op[half], (1, 0))] + [(w_s[m], (h0, 0))] * (len(blk) > known)

        def operand(g, m, half, q, zero):
            tp, tr = SB[q // 7], SB[q % 7]
            if len(tp) + len(tr) == 2:
                a, b = (2 * tp[0][n] + tr[0][n] for n in range(2))
                return w_s[m][8 * g + 4 * half + b, pl.ds(128 * a, 128), :]
            return w_op[half][1 + q // 16, pl.ds(
                pl.multiple_of(128 * (q % 16) + 8 * zero, 8), 128), :]

        def decode_unit(g, m, half, prods):
            for r0 in range(0, P0 // 4, 8):
                out = _decode(prods, r0)
                for i, j in QUAD:
                    for a, b in QUAD:
                        rings[8 * m + 4 * half + 2 * b + j][
                            g, pl.ds(P0 // 4 * (2 * a + i) + r0, 8), :] = out[2 * a + i, 2 * b + j]
                    yield [(rings[8 * m + 4 * half + 2 * b + j], (g, 0)) for b in range(2)]

        for cp in x0_copies(0) + x0_copies(1):
            cp.start()
        for m in range(3):
            start_chunk(0, m)
        x0_copies(2)[0].start()

        @pl.loop(0, NP)
        def _(p):
            we[4, pl.ds(pl.multiple_of(128 * p, 128), 128), :] = jnp.zeros((128, 128), u32)

        @pl.loop(0, P0 // 64 // LN_UNROLL)
        def _(i):
            for k in range(2):
                @pl.when(i == k * P0 // 128 // LN_UNROLL)
                def _():
                    for cp in x0_copies(k):
                        cp.wait()
            n = 16 * LN_UNROLL
            for a in range(4):
                rows = pl.ds(pl.multiple_of(P0 // 4 * a + n * i, 16), n)
                _set_rows(xg, rows, _ln(xs[rows, :].astype(f32)))
            for s in range(LN_UNROLL):
                for kt in range(2):
                    ops = _encode(SA, lambda k, a, b: xg[2 * b + kt, pl.ds(
                        P0 // 4 * a + n * i + 16 * s + k, 8, stride=2), :])
                    for p, w in enumerate(ops):
                        xe[p][pl.ds(pl.multiple_of(64 * kt + n // 2 * i + 8 * s, 8), 8), :] = w

        wait_chunk(0, (0,))

        @pl.loop(0, 16 // W_UNROLL)
        def _(i):
            list(encode_unit(0, 0, 0, [pl.multiple_of(8 * (W_UNROLL * i + k), 8)
                                       for k in range(W_UNROLL)]))

        wait_chunk(0, (1,))

        def transfers(g, g1, m, half):
            if half == 1:
                if m < 2:
                    wait_chunk(m + 1)
                else:
                    pl.when(g < 3)(functools.partial(wait_chunk, 0))
                pl.when(g < 3)(functools.partial(start_chunk, g1, m))
            elif m > 0:
                fence()
                for cp in early_copies(g) if m == 1 else [wo_copy(g)]:
                    cp.start()

        last = [we.at[4, pl.ds(128 * p, 128)] for p in range(NP)]

        @pl.loop(0, 4)
        def _(g):
            g1 = jnp.minimum(g + 1, 3)
            zero = g >> 2
            pending = decode_unit((g + 3) & 3, 2, 1, last)
            for m in range(3):
                for half in range(2):
                    nxt = (g1, 0, 0) if (m, half) == (2, 1) else (g, m + half, 1 - half)
                    side = _Side(zero, 8 * (NP - 1),
                                 (encode_unit(*nxt, range(0, 128, 8)), 7 * 16), (pending, 64))
                    prods = []
                    for p in range(NP):
                        if p == 1:
                            transfers(g, g1, m, half)
                        lhs = jnp.concatenate(
                            [xe[p][pl.ds(64 * kt, 64), :] for kt in range(2)], axis=1)
                        rhs = operand(g, m, half, p, zero)
                        for k in range(0, 64, 8) if p else ():
                            lhs = side.tie(lhs, k, 128)
                        prods.append(_dot(_unpack(lhs), _unpack(rhs)))
                    pending = decode_unit(g, m, half, prods)
            for p in range(NP):
                last[p][...] = pltpu.bitcast(prods[p], u32)

        list(decode_unit(3, 2, 1, last))

        x_copy.start()
        x0_copies(2)[0].wait()
        tokbuf[...] = _ln(xs[pl.ds(P0, UNROLL * TOK), :].astype(f32))
        _set_rows(xg, pl.ds(0, HALO), jnp.zeros((HALO, D), f32))
        _set_rows(xg, pl.ds(HALO + S, HALO), jnp.zeros((HALO, D), f32))
        _set_rows(hbuf, pl.ds(0, UNROLL * TOK), jnp.zeros((UNROLL * TOK, D), f32))
        _set_rows(useq, pl.ds(2 * TOK, 2 * TOK), jnp.zeros((2 * TOK, D), f32))
        for cp in w3_copies:
            cp.start()
        for i in range(4):
            for cp in early_copies(i):
                cp.wait()

        @pl.loop(0, 4)
        def _(j):
            for r in range(0, D // 4, 16):
                raw = {key: w1e[j, 1 + n, pl.ds(r, 16), :] for n, key in enumerate(QUAD)}
                ops = _encode1(SB, lambda k, a, b: _unzip(raw[a, b], k))
                for p in (0, 2, 3, 5, 6):
                    w1e[j, p, pl.ds(r, 16), :] = ops[p]

        for i in range(4):
            wo_copy(i).wait()

        def wrap(r):
            return jnp.where(r >= RING, r - RING, r)

        def step(s, carry, tok, side, last):
            mem, rp, ra, rw = carry
            ri = lax.broadcasted_iota(jnp.int32, (2 * MEM + SEG, 2 * L), 0)
            ci = lax.broadcasted_iota(jnp.int32, (2 * MEM + SEG, 2 * L), 1)
            key_b = ((ci >= MEM) & (ci < 2 * MEM)) | (ci >= 2 * MEM + SEG)
            same = key_b == ((ri >= MEM) & (ri < 2 * MEM))
            mask = same & ((ri < 2 * MEM) | (ri >= ci))
            fill = jnp.where(same, NEG, -jnp.inf)

            lhs = jnp.concatenate([mem, tok], axis=0).astype(bf16)
            rps = [pl.multiple_of(wrap(rp + 8 * i), 8) for i in range(3)]
            ra_ = pl.multiple_of(ra, SEG)
            rw_ = pl.multiple_of(rw, 8)

            col = s & 3
            group = jnp.maximum((s >> 2) - 1, 0)
            rb = pl.multiple_of(group * (4 * TOK), 8)

            mem_qkv = {}
            scores = {}
            o_mem = {}
            total = [None]

            def qkv(h):
                for m in range(3):
                    w = w_s[m][h]
                    r = _dot(lhs, _unpack(side.tie(w, D // 4) if h >= SIDE_AT else w))
                    for i in range(3):
                        ring[m][h][pl.ds(rps[i], 8), :] = r[8 + 8 * i:16 + 8 * i]
                    mem_qkv[m, h] = r[:MEM]

            def segment(m, pair):
                a, b = 2 * pair, 2 * pair + 1
                ma, mb = mem_qkv.pop((m, a)), mem_qkv.pop((m, b))
                xa, xb = (ring[m][h][pl.ds(ra_, SEG), :] for h in (a, b))
                if m == 0:
                    parts = ((ma, mb, xa), (xb,))
                else:
                    parts = ((ma, mb, xa, xb), (mb, ma, xb))
                return [jnp.concatenate(v, axis=0).astype(bf16) for v in parts]

            def qk(pair):
                q, k = segment(0, pair), segment(1, pair)
                for n in range(2):
                    scores[pair, n] = lax.dot_general(
                        q[n], k[n], (((1,), (1,)), ((), ())), preferred_element_type=f32)

            def pv(pair):
                v = segment(2, pair)
                for n in range(2):
                    sc = scores.pop((pair, n)) * (DH ** -0.5)
                    if n == 0:
                        sc = jnp.where(mask, sc, fill)
                    else:
                        sc = jnp.where(mask[2 * MEM:, :2 * MEM + SEG], sc,
                                       fill[2 * MEM:, :2 * MEM + SEG])
                    mx = jnp.max(sc, axis=1, keepdims=True)
                    e = jnp.exp(sc - mx)
                    den = jnp.sum(e, axis=1, keepdims=True)
                    inv = pl.reciprocal(den, approx=True)
                    inv = inv * (2.0 - den * inv)
                    o = _dot(e.astype(bf16), v[n]) * inv
                    q_r[2 * pair + n][pl.ds(ra_, SEG), :] = o[-SEG:]
                    if n == 0:
                        o_mem[2 * pair], o_mem[2 * pair + 1] = o[:MEM], o[MEM:2 * MEM]

            def wo(h):
                lo = jnp.concatenate([o_mem.pop(h), q_r[h][pl.ds(rw_, TOK), :]],
                                     axis=0).astype(bf16)
                r = _dot(lo, _unpack(wo_b[pl.ds(h * DH // 2, DH // 2), :]))
                total[0] = r if total[0] is None else total[0] + r

            npair = H // 2
            for t in range(npair + LAG_WO):
                if 0 <= t - LAG_QK < npair:
                    qk(t - LAG_QK)
                if 0 <= t - LAG_PV < npair:
                    pv(t - LAG_PV)
                if t < npair:
                    qkv(2 * t)
                    qkv(2 * t + 1)
                if 0 <= t - LAG_WO < npair:
                    wo(2 * (t - LAG_WO))
                    wo(2 * (t - LAG_WO) + 1)
            fills = [_dot(_unpack(ubuf[p]), _unpack(w1e[col, p])) for p in range(7)]
            for (a, b), v in _decode1(fills).items():
                xg[4 * b + col, pl.ds(HALO + rb + 2 * TOK * a, 2 * TOK), :] = (
                    v if last and a == b else _gelu(v))

            a = total[0]
            return (a[:MEM], wrap(rp + TOK), wrap(ra + SEG), wrap(rw + TOK)), a[MEM:]

        def late_gelu(s):
            rb = jnp.maximum((s >> 2) - 1, 0) * (4 * TOK)
            for a in range(2):
                at = (4 * a + (s & 3),
                      pl.ds(pl.multiple_of(HALO + rb + 2 * TOK * a, 8), 2 * TOK))
                xg[at] = _gelu(xg[at])
            yield [(xg, (s & 3, HALO + rb))]

        def steps(i, carry):
            n = UNROLL * TOK
            pl.when(i == 1)(x_copy.wait)

            @pl.when(i == 16 // ENC)
            def _():
                raw = we.at[pl.ds(0, NC), pl.ds(0, 4 * 512)]
                pltpu.make_async_copy(raw, raw, sems.at[SEM_W3]).wait()

            zero = i >> 5
            at = lambda r, m, k: pl.ds(pl.multiple_of(r + 16 * k * zero, 16), m)

            def norm_filler():
                prev = jnp.maximum(i - 1, 0)

                def first_norm(r, x, y):
                    lnbuf[pl.ds(r, 16), :] = y
                    return [(lnbuf, (r,))]

                def second_norm(r, x, y):
                    dst = pl.multiple_of(n * (prev & 3) + r, 8)
                    _set_rows(useq, pl.ds(dst, 16), y)
                    return [(useq, (0, dst))]

                yield from _ln_job(lambda r, m, k: _rows(hbuf, at(n * prev + r, m, k)),
                                   first_norm, n)
                yield from _ln_job(lambda r, m, k: lnbuf[at(r, m, k + 2), :],
                                   second_norm, n)
                base = (jnp.maximum((UNROLL * i >> 2) - 1, 0) & 1) * (2 * n)
                for r in range(0, n, 16):
                    for kt in range(4):
                        ops = _encode1(SA, lambda k, a, b: useq[
                            4 * b + kt, pl.ds(base + n * a + r + k, 8, stride=2), :])
                        for p, w in enumerate(ops):
                            ubuf[p, pl.ds(r // 2, 8), pl.ds(128 * kt, 128)] = w
                        if kt % 2:
                            yield [(ubuf, (0, 0))]

            def norm_tokens():
                def keep(r, x, y):
                    tokbuf[pl.ds(r, 16), :] = y
                    return [(tokbuf, (r,))]

                nxt = jnp.minimum(P0 + n * (i + 1), S - n)
                return _ln_job(lambda r, m, k: xs[at(nxt + r, m, k), :].astype(f32),
                               keep, n)

            def encode_b():
                for j in range(4):
                    raw = {(a, b): we[w2_slot(2 * a + b, j, 8 * i, 8)] for a, b in QUAD}
                    for p, w in enumerate(_encode1(SB, lambda k, a, b: _unzip(raw[a, b], k))):
                        we[w2_slot(p, j, 8 * i, 8)] = w
                    yield [(we, (NC, 8 * i))]
                for k in range(ENC):
                    j = ENC * i + k
                    grp, i0 = jnp.where(j < 16, NC + 2, (j >> 4) - 1), 8 * (j & 15)
                    slot = lambda q: (grp, pl.ds(pl.multiple_of(128 * q + i0, 8), 8))
                    raw = {(a, b): we[slot(4 * b + a)] for a in range(4) for b in range(4)}
                    get = functools.cache(lambda k, a, b: _unzip(raw[a, b], k))
                    for p in ORDER_B:
                        for r, w in enumerate(_encode7(SB, p, get)):
                            we[slot(7 * p + r)] = w
                        yield [(we, (grp, i0))]

            jobs = [[(norm_filler(), 4 * n // 16), (late_gelu(jnp.maximum(UNROLL * i - 1, 0)), 1)],
                    [(encode_b(), 4 + 7 * ENC), (norm_tokens(), n // 16)]]
            for k in range(UNROLL):
                s = i * UNROLL + k
                carry, o = step(s, carry, tokbuf[pl.ds(k * TOK, TOK), :],
                                _Side(zero, SIDE_N, *jobs[k]), k == UNROLL - 1)
                lo = k * TOK // 16 * 16
                xv = xs[pl.ds(pl.multiple_of(n * i + lo, 16), 32), :].astype(f32)
                _set_rows(hbuf, pl.ds(pl.multiple_of(TOK * s, 8), TOK),
                          xv[k * TOK - lo:(k + 1) * TOK - lo] + o)
            return carry

        carry = (mem0_ref[...].astype(f32), jnp.int32(P0), jnp.int32(0), jnp.int32(0))
        carry = lax.fori_loop(0, NSEG // UNROLL, steps, carry)
        list(late_gelu(jnp.int32(NSEG - 1)))
        return carry[1] >> 16

    zero = pl.run_scoped(
        block_a,
        *[pltpu.VMEM((H, D // 2, DH), u32)] * 3,
        pltpu.VMEM((7, TOK, D // 2), u32),
        pltpu.VMEM((D // 128, 8 * TOK, 128), f32),
        pltpu.VMEM((UNROLL * TOK, D), f32),
        pltpu.VMEM((UNROLL * TOK, D), f32),
        *[pltpu.VMEM((H // 8, RING, DH), f32)] * 16,
    )

    def tail(w4e, ye, ybuf, *bufs):
        woe, pool = bufs[:3], bufs[3:]
        w4_copies = [
            pltpu.make_async_copy(w4_hbm.bitcast(u32).at[pl.ds(1, NC - 1), a, :, pl.ds(b * C4, C4)],
                                  w4e.at[4 * a + b], sems.at[SEM_W4])
            for a in range(4) for b in range(4)]
        for cp in w4_copies:
            cp.start()
        done = TOK * NSEG
        first = 4 * TOK * (NSEG // 4 - 1)

        def later(rows, n):
            return pl.ds(pl.multiple_of(rows + 8 * zero, 8), n)

        def run(dots, ties, start, *jobs):
            side = _Side(zero, (len(dots) - max(start, 0)) * len(ties), *jobs)
            prods = []
            for load in dots:
                if len(prods) == start:
                    fence()
                lhs, rhs = load()
                for r0, c0 in ties if len(prods) >= start else ():
                    lhs = side.tie(lhs, r0, c0)
                prods.append(_dot(_unpack(lhs), _unpack(rhs)))
            return prods

        hk, hn, hm = H * DH // 4, D // 2, P0 // 2

        def wo_op(p, j):
            if p == 3:
                return pool[j], 0, 0
            if p in (1, 4):
                return wo_b, hk * (p // 4), hn * (p // 4) + C4 * j
            return woe[{0: 0, 2: 1, 5: 2, 6: 0}[p]], 0, C4 * j

        def encode_wo(ps):
            for i0 in range(0, hk, 8):
                for j in range(2):
                    get = functools.cache(lambda k, a, b: _unzip(wo_b[
                        later(hk * a + i0 + 8 * ps[0] * zero, 8), pl.ds(hn * b + C4 * j, C4)], k))
                    ops = [_zip(*[_combine(functools.partial(get, k), SB[p]) for k in range(2)])
                           for p in ps]
                    for p, w in zip(ps, ops):
                        ref, r0, c0 = wo_op(p, j)
                        ref[pl.ds(r0 + i0, 8), pl.ds(c0, C4)] = w
                    yield [(wo_op(p, j)[0], (0,)) for p in ps]

        def encode_o(n):
            for kt in range(H // 2):
                for s in range(hm // 16):
                    pool[n][pl.ds(hm // 2 * (kt // 2) + 8 * s, 8), pl.ds(kt % 2 * 128, 128)] = (
                        _zip(*[_combine(
                            lambda a, b: q_r[H // 2 * b + kt][pl.ds(
                                (done + hm * a + 16 * s) % RING + k + n * zero, 8, stride=2), :],
                            SA[ORDER_B[n]]) for k in range(2)]))
                    if s % 4 == 3:
                        yield [(pool[n], (0,))]

        def wo_dots(n):
            def load(j, i):
                ref, r0, c0 = wo_op(ORDER_B[n], j)
                lhs = [pool[n][later(hm // 2 * c + hm // 4 * i + 8 * j * zero, hm // 4), :]
                       for c in range(8)]
                return (jnp.concatenate(lhs, axis=1),
                        ref[later(r0 + 8 * i * zero, hk), pl.ds(c0, C4)])
            return [functools.partial(load, j, i) for j, i in QUAD]

        def decode_wo(n, prods):
            for (j, i), v in zip(QUAD, prods):
                for r in range(0, hm // 2, 16):
                    for (a, b), sign in SC[ORDER_B[n]]:
                        fresh = all(key != (a, b) for q in ORDER_B[:n] for key, _ in SC[q])
                        row = done + hm * a + hm // 2 * i + r
                        for k in range(2):
                            c = 4 * b + 2 * j + k
                            old = (xs[pl.ds(row, 16), pl.ds(128 * c, 128)].astype(f32) if fresh
                                   else hbuf[c, later(row + 8 * n * zero, 16), :])
                            new = v[r:r + 16, 128 * k:128 * (k + 1)]
                            hbuf[c, pl.ds(row, 16), :] = old + new if sign > 0 else old - new
                    yield [(hbuf, (0, 0))]

        hsb = wo_b

        def norm_in():
            def first_norm(r, x, y):
                woe[2][pl.ds(r, 16), :] = pltpu.bitcast(y[:, :hn], u32)
                woe[2][pl.ds(P0 + r, 16), :] = pltpu.bitcast(y[:, hn:], u32)
                return [(woe[2], (r,))]

            def second_norm(r, x, y):
                _set_rows(xg, pl.ds(HALO + done + r, 16), y)
                return [(xg, (0, HALO + done))]

            yield from _ln_job(
                lambda r, n, k: _rows(hbuf, later(done + r + 8 * (7 + k) * zero, n)),
                first_norm, P0, NORM_ROWS, *stats[:2], zero)
            yield from _ln_job(
                lambda r, n, k: pltpu.bitcast(jnp.concatenate(
                    [woe[2][later(r0 + r + 8 * k * zero, n), :] for r0 in (0, P0)], axis=1), f32),
                second_norm, P0, NORM_ROWS, *stats[2:], zero)

        def encode_rows(buf, r0, n, shift=(0, 0, 0, 0)):
            for r in range(0, n // 2, 16):
                for kt in range(4):
                    ops = _encode1(SA, lambda k, a, b: xg[4 * b + kt, pl.ds(
                        HALO + r0 + n // 2 * a + r + k + shift[2 * b + kt // 2],
                        8, stride=2), :])
                    for p, w in enumerate(ops):
                        buf[pl.ds(128 * p + 64 * (kt // 2) + r // 2, 8),
                            pl.ds(128 * (kt % 2), 128)] = w
                    yield [(buf, (0,))]

        def encode_g(i):
            return encode_rows(pool[i - 1], i * RB, RB, SHIFT)

        def mixer(buf, n, weights, store, start, pending, *jobs):
            def decode(j, prods):
                for r in range(0, n // 2, 8):
                    for (a, b), v in _decode1([m[r:r + 8] for m in prods]).items():
                        seen = store(n // 2 * a + r, 4 * b + j, v)
                    yield seen

            for j in range(4):
                dots = [lambda p=p: (
                    jnp.concatenate([buf[later(128 * p + 64 * k + 8 * j * zero, n // 4), :]
                                     for k in range(2)], axis=1),
                    weights(p, j)) for p in range(7)]
                prods = run(dots, [(r, TIE_C) for r in range(0, n // 4, 8)],
                            -1 if j else start, pending,
                            *[(job, count // 4) for job, count in jobs])
                pending = (decode(j, prods), n // 16)
            return pending

        def mixer_in(buf, r0, n, *args):
            def store(r, c, v):
                xg[c, pl.ds(HALO + r0 + r, 8), :] = _gelu(v)
                return [(xg, (0, HALO + r0))]

            return mixer(buf, n, lambda p, j: w1e[j, p, later(r0 * zero, D // 4), :],
                         store, *args)

        def mixer_out(i, *args):
            def store(r, c, v):
                hsb[pl.ds(i * RB + r, 8), pl.ds(128 * c, 128)] = pltpu.bitcast(v, u32)
                return [(hsb, (i * RB,))]

            return mixer(pool[i - 1], RB, lambda p, j: we[w2_slot(p, j, 8 * (i + 1) * zero)],
                         store, 0, *args)

        def encode_w4():
            for c in range(NC - 1):
                for i0 in range(0, 64, 8):
                    for j in range(2):
                        at = (c, pl.ds(i0, 8), pl.ds(128 * j, 128))
                        raw = {(a, b): w4e[(4 * a + b,) + at]
                               for a in range(4) for b in range(4)}
                        get = functools.cache(lambda k, a, b: _unzip(raw[a, b], k))
                        for p in ORDER_B:
                            for r, w in enumerate(_encode7(SB, p, get)):
                                w4e[(7 * p + r,) + at] = w
                            yield [(w4e, (0, c, i0))]

        def mixer_post(r0, zero, group):
            def first_norm(r, hv, y):
                rows = pl.ds(_mult(r0 + r, 8), 16)
                x1 = y + pltpu.bitcast(hsb[rows, :], f32)
                _set_rows(xg, rows, hv + x1)
                _set_rows(ybuf, pl.ds(r, 16), x1)
                return [(ybuf, (0, 0)), (xg, (0, r0))]

            def second_norm(r, x1, y):
                _set_rows(hbuf, pl.ds(_mult(r0 + r, 8), 16), y)
                return [(hbuf, (0, r0))]

            at = lambda r, n, k: pl.ds(pl.multiple_of(r + 8 * k * zero, 8), n)
            yield from _ln_job(lambda r, n, k: _rows(hbuf, at(r0 + r, n, k)),
                               first_norm, RB, group, *stats[:2], zero)
            yield from _ln_job(lambda r, n, k: _rows(ybuf, at(r, n, k + 1)),
                               second_norm, RB, group, *stats[2:], zero)
            for s in range(4):
                for kt in range(2):
                    get = functools.cache(lambda k, a, b: hbuf[2 * b + kt, pl.ds(
                        r0 + R4 * a + 4 * k + 2 * (s % 2) + s // 2, 8, stride=8), :])
                    for p in ORDER_A:
                        for r, w in enumerate(_encode7(SA, p, get)):
                            ye[7 * p + r, pl.ds(8 * s, 8), pl.ds(128 * kt, 128)] = w
                        if p in POST_P:
                            yield [(ye, (0, 8 * s))]

        def out_copies(i):
            rows = pl.ds(_mult(i * RB, RB), RB)
            return [pltpu.make_async_copy(
                woe[b].bitcast(bf16).at[rows], out_hbm.at[rows, pl.ds(hn * b, hn)],
                sems.at[SEM_OUT + 2 * i + b]) for b in range(2)]

        n_g, n_o = RB // 8, H // 2 * hm // 64
        n_post = RB // 8 + 8 * len(POST_P)
        wo_ties = [(r0, c0) for c0 in range(TIE_C, 2 * D, 512) for r0 in range(0, 64, 8)]
        w4_job = encode_w4()
        wo_jobs = [encode_wo(ps) for ps in ((0,), (2, 5), (3, 6))]

        _set_rows(xg, pl.ds(HALO + first, done - first),
                  _ln(_ln(_rows(hbuf, pl.ds(first, done - first)))))
        list(encode_rows(pool[7], first, done - first))
        pending = mixer_in(pool[7], first, done - first, -1, (None, 0), (encode_o(0), n_o))
        for n in range(7):
            jobs = [(encode_o(n + 1), n_o) if n < 6 else (encode_g(0), n_g), pending]
            if n < 5:
                jobs.append((wo_jobs[(n + 1) // 2], hk // 8 if n else hk // 4))
            if n == W4_AT:
                for cp in w4_copies:
                    cp.wait()
            if n >= W4_AT:
                jobs.append((w4_job, 7 * W4_WO))
            prods = run(wo_dots(n), wo_ties, 0, *jobs)
            pending = (decode_wo(n, prods), hm // 8)
        norm = norm_in()
        for i in range(5):
            jobs = [(w4_job, 7 * W4_SPLIT[i])]
            jobs.append((encode_g(i + 1) if i < 4 else encode_rows(pool[7], done, RB), n_g))
            if i > 0:
                jobs.append((norm, P0 // NORM_ROWS + P0 // 32))
            pending = mixer_out(i, pending, *jobs)
        post = (mixer_post(0, zero, NORM_ROWS), (n_post + 4 * RB // NORM_ROWS) // 2)
        pending = mixer_in(pool[7], done, RB, IN_FENCE[0], pending, post,
                           (encode_rows(pool[0], done + RB, RB), n_g))
        pending = mixer_in(pool[0], done + RB, RB, IN_FENCE[1], pending, post,
                           (encode_g(5), n_g))
        for i in range(5, 8):
            jobs = [(w4_job, 7 * W4_SPLIT[i])]
            if i < 7:
                jobs.append((encode_g(i + 1), n_g))
            pending = mixer_out(i, pending, *jobs)
        list(pending[0])

        def mlp_block(i, carry):
            te = []
            for c in range(NC):
                ops = []
                for r0 in range(0, R4, UP_ROWS):
                    prods = [_dot(_unpack(ye[p, pl.ds(r0 // 2, UP_ROWS // 2), :]), _unpack(
                        we[c, pl.ds(pl.multiple_of(128 * p + r0 * (i >> 3), 8), 128), :]))
                        for p in range(NP)]
                    for s in range(UP_ROWS // 16):
                        act = [{key: _gelu2(v) for key, v in _decode(
                            prods, 32 * (s // 2) + 16 * k + 8 * (s % 2)).items()}
                            for k in range(2)]
                        ops.append(_encode(SA, lambda k, a, b: act[k][a, b]))
                te.append([jnp.concatenate([o[p] for o in ops], axis=0) for p in range(NP)])

            def down(p, lo, hi, tie=lambda w: w):
                lhs = jnp.concatenate([tie(te[c][p]) if c in POST_C else te[c][p]
                                       for c in range(lo, hi)], axis=1)
                rhs = [w4e[p, c - 1] if c else jnp.concatenate(
                    [we[NC + 2, pl.ds(128 * p + 64 * k, 64), :] for k in range(2)], axis=1)
                    for c in range(lo, hi)]
                rhs = jnp.concatenate(rhs, axis=0)
                return _dot(_unpack(lhs), _unpack(rhs))

            prods = [down(p, 0, KSPLIT) for p in range(NSPLIT)]
            prods = [m + down(p, KSPLIT, NC) for p, m in enumerate(prods)]
            out = {}

            def finish(qa, qb):
                for a, b in ((2 * qa + n // 2, 2 * qb + n % 2) for n in range(4)):
                    for r in range(0, R4, 16):
                        row = i * RB + R4 * a + r
                        for j in range(2):
                            woe[qb][pl.ds(pl.multiple_of(row // 2, 8), 8),
                                    pl.ds(C4 * (b % 2) + 128 * j, 128)] = _zip(*[
                                        0.5 * out[a, b][32 * k + r // 2:32 * k + r // 2 + 8,
                                                  128 * j:128 * (j + 1)]
                                        + xg[2 * b + j, pl.ds(row + k, 8, stride=2), :]
                                        for k in range(2)])
                        yield [(woe[qb], (i * (RB // 2),))]

            side = _Side(i >> 3, POST_N * len(POST_C),
                         (mixer_post(((i + 1) & 7) * RB, i >> 3, 0), n_post))
            for p in range(7):
                done_quad = {4: (1, 0), 5: (0, 1), 6: (1, 1)}.get(p)
                store = _Side(i >> 3, 16, *([(finish(*done_quad), 16)] if done_quad else []))
                for q in range(len(prods), 7 * p + 7):
                    side.after(hbuf, prods[q - POST_LAG])
                    prods.append(down(q, 0, NC, side.tie if q % 7 == 0 else
                                      lambda w: store.tie(side.tie(w))))
                _decode7(p, prods[7 * p:7 * p + 7], out)
            list(finish(0, 0))
            for cp in out_copies(i):
                cp.start()
            return carry

        lax.fori_loop(0, S // RB, mlp_block, 0)
        for i in range(S // RB):
            for cp in out_copies(i):
                cp.wait()

    pl.run_scoped(
        tail,
        pltpu.VMEM((NP, NC - 1, 64, C4), u32),
        pltpu.VMEM((NP, R4 // 2, C4), u32),
        pltpu.VMEM((D // 128, RB, 128), f32),
        *[pltpu.VMEM((H * DH // 4, D // 2), u32)] * 3,
        *[pltpu.VMEM((D, C4), u32)] * 8,
    )


@jax.jit
def pallas_sequential_preLN__memory_aug_recurrent_mem_tr__mixer_s_mlp__prompt_kernel(
    A_x: jax.Array,
    A_mem0: jax.Array,
    A_Wq: jax.Array,
    A_Wk: jax.Array,
    A_Wv: jax.Array,
    A_Wo: jax.Array,
    A_seg_len: jax.Array,
    B_x: jax.Array,
    B_w1: jax.Array,
    B_w2: jax.Array,
    B_w3: jax.Array,
    B_w4: jax.Array,
):
    del A_seg_len, B_x
    hbm = pl.BlockSpec(memory_space=pl.ANY)
    vmem = pl.BlockSpec(memory_space=pltpu.VMEM)
    scratch = [
        pltpu.VMEM((H * DH // 2, D), u32),
        pltpu.VMEM((S, D), bf16),
        pltpu.VMEM((D // 128, S + 8, 128), f32),
        pltpu.VMEM((D // 128, S + 2 * HALO, 128), f32),
        pltpu.VMEM((4, 7, D // 4, 128), u32),
        pltpu.VMEM((NC + 3, NP * 128, 128), u32),
        pltpu.SemaphoreType.DMA((NSEM,)),
        pltpu.SemaphoreType.REGULAR,
    ] + [pltpu.VMEM((P0, 128), f32)] * 4 + [pltpu.VMEM((H // 8, RING, DH), f32)] * 8
    out = pl.pallas_call(
        _kernel,
        out_shape=jax.ShapeDtypeStruct((S, D), A_x.dtype),
        in_specs=[hbm, vmem] + [hbm] * 8,
        out_specs=hbm,
        scratch_shapes=scratch,
        compiler_params=pltpu.CompilerParams(vmem_limit_bytes=VMEM_LIMIT),
    )(A_x.reshape(S, D), A_mem0.reshape(MEM, D),
      A_Wq.reshape(D // 2, 2 * H, DH), A_Wk.reshape(D // 2, 2 * H, DH),
      A_Wv.reshape(D // 2, 2 * H, DH),
      A_Wo.reshape(H * DH, D), B_w1, B_w2, B_w3, B_w4.reshape(NC, 4, 128, D))
    return out.reshape(A_x.shape)
```

```python
import functools

import jax
import jax.numpy as jnp
from jax import lax
import jax.experimental.pallas as pl
import jax.experimental.pallas.tpu as pltpu

S = 2048
D = 1024
H = 32
DH = 128
MEM = 8
SEG = 32
F = 3584
NSEG = S // SEG
L = MEM + SEG
TOK = 24
P0 = S - TOK * NSEG
RING = 576
X0 = P0 + 128
C4 = D // 4
SHIFT = (-1, 1, -2, 2)
HALO = 8
RB = 256
R4 = RB // 4
NC = F // 512
NP = 49
EPS = 1e-5
NEG = -1000000000.0

VMEM_LIMIT = 127 * 1024 * 1024 + 896 * 1024

LAG_QK = 2
LAG_PV = 4
LAG_WO = 15
UNROLL = 2
ENC = 4
SIDE_AT = 4
SIDE_N = 73
SIDE_ROW = 256
TIE_C = 384
LN_UNROLL = 4
W_UNROLL = 8
IN_FENCE = (0, -1)
NORM_ROWS = 16
W4_AT = 5
W4_WO = 18
W4_SPLIT = (12, 0, 0, 0, 0, 16, 16, 16)
UP_ROWS = 32
NSPLIT = 5
KSPLIT = 5
POST_C = (1, 3, 5)
POST_N = 42
POST_LAG = 5
POST_P = (0, 6, 5)
assert (7 - W4_AT) * W4_WO + sum(W4_SPLIT) == 16 * (NC - 1)

bf16 = jnp.bfloat16
f32 = jnp.float32
u32 = jnp.uint32

SEM_X0, SEM_X, SEM_W1, SEM_W3, SEM_W4, SEM_WO, SEM_OUT, SEM_W = 0, 3, 4, 5, 6, 7, 11, 27
NSEM = SEM_W + 6

SA = (((0, 0), 1, (1, 1)), ((1, 0), 1, (1, 1)), ((0, 0),), ((1, 1),),
      ((0, 0), 1, (0, 1)), ((1, 0), -1, (0, 0)), ((0, 1), -1, (1, 1)))
SB = (((0, 0), 1, (1, 1)), ((0, 0),), ((0, 1), -1, (1, 1)), ((1, 0), -1, (0, 0)),
      ((1, 1),), ((0, 0), 1, (0, 1)), ((1, 0), 1, (1, 1)))
SC = ((((0, 0), 1), ((1, 1), 1)), (((1, 0), 1), ((1, 1), -1)),
      (((0, 1), 1), ((1, 1), 1)), (((0, 0), 1), ((1, 0), 1)),
      (((0, 0), -1), ((0, 1), 1)), (((1, 1), 1),), (((0, 0), 1),))
ORDER_A = (2, 3, 0, 4, 6, 1, 5)
ORDER_B = (1, 4, 0, 2, 5, 3, 6)
QUAD = ((0, 0), (0, 1), (1, 0), (1, 1))


def _mult(i, n):
    return i if isinstance(i, int) else pl.multiple_of(i, n)


def _ln(x):
    m = jnp.mean(x, axis=-1, keepdims=True)
    d = x - m
    v = jnp.mean(d * d, axis=-1, keepdims=True)
    return d * lax.rsqrt(v + EPS)


def _gelu2(x):
    c = 0.7978845608028654
    return x * jnp.tanh(x * (c + c * 0.044715 * (x * x))) + x


def _gelu(x):
    return 0.5 * _gelu2(x)


def _unpack(x):
    return pltpu.bitcast(x, bf16)


def _dot(a, b):
    return jnp.dot(a, b, preferred_element_type=f32)


def _zip(even, odd):
    return pltpu.bitcast(pltpu.pack_elementwise([even, odd], packed_dtype=bf16), u32)


def _unzip(w, k):
    return pltpu.unpack_elementwise(w, index=k, packed_dtype=bf16, unpacked_dtype=f32)


def _combine(get, term):
    if len(term) == 1:
        return get(*term[0])
    a, b = get(*term[0]), get(*term[2])
    return a + b if term[1] > 0 else a - b


def _encode7(tab, p, get):
    outer = [{(i, j): _combine(lambda a, b: get(k, 2 * a + i, 2 * b + j), tab[p])
              for i, j in QUAD} for k in range(2)]
    return [_zip(*[_combine(lambda a, b: o[a, b], tab[r]) for o in outer])
            for r in range(7)]


def _encode(tab, get):
    get = functools.cache(get)
    ops = {p: _encode7(tab, p, get) for p in (ORDER_A if tab is SA else ORDER_B)}
    return [w for p in range(7) for w in ops[p]]


def _encode1(tab, get):
    get = functools.cache(get)
    return [_zip(*[_combine(functools.partial(get, k), t) for k in range(2)]) for t in tab]


def _decode1(prods):
    out = {}
    for p in range(7):
        for key, sign in SC[p]:
            _accumulate(out, key, sign, prods[p])
    return out


def _accumulate(acc, key, sign, v):
    if key not in acc:
        acc[key] = v
    else:
        acc[key] = acc[key] + v if sign > 0 else acc[key] - v


def _decode7(p, prods, out):
    inner = _decode1(prods)
    for (a, b), sign in SC[p]:
        for (i, j), v in inner.items():
            _accumulate(out, (2 * a + i, 2 * b + j), sign, v)


def _decode(prods, r0):
    out = {}
    for p in range(7):
        _decode7(p, [pltpu.bitcast(m[r0:r0 + 8, :], f32) for m in prods[7 * p:7 * p + 7]],
                 out)
    return out


def _rows(ref, rows):
    return jnp.concatenate([ref[c, rows, :] for c in range(ref.shape[0])], axis=1)


def _set_rows(ref, rows, v):
    for c in range(ref.shape[0]):
        ref[c, rows, :] = v[:, c * 128:(c + 1) * 128]


class _Side:
    def __init__(self, zero, slots, *jobs):
        self.zero = zero
        self.slots = slots
        self.jobs = [[job, count, 0] for job, count in jobs]
        self.at = 0

    def tie(self, w, r0=0, c0=0):
        self.at += 1
        head = old = w[r0:r0 + 8, c0:c0 + 128]
        for job in self.jobs:
            while job[2] * self.slots < min(self.at, self.slots) * job[1]:
                job[2] += 1
                for ref, idx in next(job[0]):
                    row = pl.ds(pl.multiple_of(idx[-1] + 8 * self.zero, 8), 8)
                    seen = ref[idx[:-1] + (row, pl.ds(0, 128))]
                    head = jnp.where(self.zero == 0, head, pltpu.bitcast(seen, u32))
        if head is old:
            return w
        row = [v for v in (w[r0:r0 + 8, :c0] if c0 else None, head,
                           w[r0:r0 + 8, c0 + 128:] if c0 + 128 < w.shape[1] else None)
               if v is not None]
        rows = (w[:r0] if r0 else None, jnp.concatenate(row, axis=1),
                w[r0 + 8:] if r0 + 8 < w.shape[0] else None)
        return jnp.concatenate([v for v in rows if v is not None], axis=0)

    def after(self, ref, r):
        spare = pl.multiple_of(ref.shape[-2] - 8 - 8 * self.zero, 8)
        lead = tuple(n - 1 - self.zero for n in ref.shape[:-2])
        ref[lead + (pl.ds(spare, 8), pl.ds(0, 128))] = pltpu.bitcast(r[:8, :128], ref.dtype)


def _ln_job(load, store, rows, group=0, mean_ref=None, rstd_ref=None, zero=None):
    wide = lambda ref, r, n, k: jnp.concatenate(
        [ref[pl.ds(pl.multiple_of(r + 8 * k * zero, 8), n), :]] * (D // 128), axis=1)
    if not group:
        for r in range(0, rows, 16):
            x = load(r, 16, 0)
            yield store(r, x, _ln(x))
        return
    for r in range(0, rows + 2 * group, group):
        if r < rows:
            m = jnp.mean(load(r, group, 0), axis=-1, keepdims=True)
            mean_ref[pl.ds(r, group), :] = jnp.broadcast_to(m, (group, 128))
            yield [(mean_ref, (r,))]
        if 0 <= r - group < rows:
            d = load(r - group, group, 1) - wide(mean_ref, r - group, group, 1)
            v = jnp.mean(d * d, axis=-1, keepdims=True)
            rstd_ref[pl.ds(r - group, group), :] = jnp.broadcast_to(
                lax.rsqrt(v + EPS), (group, 128))
            yield [(rstd_ref, (r - group,))]
        for q in range(r - 2 * group, r - group, 16) if r >= 2 * group else ():
            x = load(q, 16, 2)
            yield store(q, x, (x - wide(mean_ref, q, 16, 2)) * wide(rstd_ref, q, 16, 2))


def _kernel(x_hbm, mem0_ref, wq_hbm, wk_hbm, wv_hbm, wo_hbm, w1_hbm, w2_hbm,
            w3_hbm, w4_hbm, out_hbm,
            wo_b, xs, hbuf, xg, w1e, we, sems, fence_sem, *bufs):
    stats, q_rings = bufs[:4], bufs[4:]
    w_hbm = (wq_hbm, wk_hbm, wv_hbm)
    q_r = [q_rings[h % 8].at[h // 8] for h in range(H)]

    def x0_copies(k):
        rows = ([pl.ds(P0 // 4 * a + P0 // 8 * k, P0 // 8) for a in range(4)] if k < 2
                else [pl.ds(P0, X0 - P0)])
        return [pltpu.make_async_copy(x_hbm.at[r], xs.at[r], sems.at[SEM_X0 + k])
                for r in rows]

    x_copy = pltpu.make_async_copy(x_hbm.at[pl.ds(X0, S - X0)], xs.at[pl.ds(X0, S - X0)],
                                   sems.at[SEM_X])

    def wo_copy(i):
        rows = pl.ds(_mult(i * 512, 512), 512)
        return pltpu.make_async_copy(wo_hbm.bitcast(u32).at[rows], wo_b.at[rows],
                                     sems.at[SEM_WO + i])

    w3_copies = [pltpu.make_async_copy(
        w3_hbm.bitcast(u32).at[:, pl.ds((4 * c + b) * 128, 128)],
        we.at[c, pl.ds(b * 512, 512)], sems.at[SEM_W3]) for c in range(NC) for b in range(4)]

    def w2_slot(p, j, r0=0, n=D // 4):
        return NC + p // 6, pl.ds(_mult(D * (p % 6) + D // 4 * j + r0, 8), n)

    def early_copies(j):
        return [pltpu.make_async_copy(
            src.bitcast(u32).at[pl.ds(D // 4 * a, D // 4),
                                pl.ds(_mult(D // 2 * b + 128 * j, 128), 128)],
            dst, sems.at[SEM_W1]) for a, b in QUAD for src, dst in (
                (w1_hbm, w1e.at[j, (1, 2, 3, 4)[2 * a + b]]),
                (w2_hbm, we.at[w2_slot(2 * a + b, j)]))] + [
            pltpu.make_async_copy(
                w4_hbm.bitcast(u32).at[0, a, :, pl.ds(_mult(C4 * j + 128 * k, 128), 128)],
                we.at[NC + 2, pl.ds(_mult(128 * (4 * j + a) + 64 * k, 64), 64)],
                sems.at[SEM_W1]) for a in range(4) for k in range(2)]

    def fence():
        pl.semaphore_signal(fence_sem, 1)
        pl.semaphore_wait(fence_sem, 1)

    def block_a(wq_s, wk_s, wv_s, ubuf, useq, tokbuf, lnbuf, *kv_rings):
        w_s = (wq_s, wk_s, wv_s)
        rings = tuple(q_rings) + tuple(kv_rings)
        ring = [[rings[m * 8 + h % 8].at[h // 8] for h in range(H)] for m in range(3)]
        k_r, v_r = ring[1:]

        xe = [we.at[3, pl.ds(128 * p, 128)] for p in range(NP)]
        w_op = (hbuf, xg)

        def start_chunk(g, m):
            for k in range(8):
                pltpu.make_async_copy(
                    w_hbm[m].bitcast(u32).at[:, 16 * (k % 2) + 4 * g + k // 2, :],
                    we.at[m, pl.ds(D // 2 * k, D // 2)],
                    sems.at[SEM_W + 2 * m + k // 4]).start()

        def wait_chunk(m, halves=(0, 1)):
            for half in halves:
                part = we.at[m, pl.ds(2 * D * half, 2 * D)]
                pltpu.make_async_copy(part, part, sems.at[SEM_W + 2 * m + half]).wait()

        def encode_unit(g, m, half, slices):
            h0 = 8 * g + 4 * half
            for i0 in slices:
                blk = {}

                def get(k, a, b):
                    if (k, a, b) not in blk:
                        for par in range(2):
                            w = we[m, pl.ds(_mult(D // 2 * (
                                4 * half + b - b % 2 + par) + 128 * a + i0, 8), 8), :]
                            for j in range(2):
                                blk[par, a, b - b % 2 + j] = _unzip(w, j)
                        for j in (b - b % 2, b - b % 2 + 1):
                            w_s[m][h0 + j, pl.ds(128 * a + i0, 8), :] = _zip(
                                blk[0, a, j], blk[1, a, j])
                    return blk[k, a, b]

                for p in ORDER_B:
                    known = len(blk)
                    for r, w in enumerate(_encode7(SB, p, get)):
                        q = 7 * p + r
                        if len(SB[p]) + len(SB[r]) > 2:
                            w_op[half][1 + q // 16, pl.ds(128 * (q % 16) + i0, 8), :] = (
                                pltpu.bitcast(w, f32))
                    yield [(w_op[half], (1, 0))] + [(w_s[m], (h0, 0))] * (len(blk) > known)

        def operand(g, m, half, q, zero):
            tp, tr = SB[q // 7], SB[q % 7]
            if len(tp) + len(tr) == 2:
                a, b = (2 * tp[0][n] + tr[0][n] for n in range(2))
                return w_s[m][8 * g + 4 * half + b, pl.ds(128 * a, 128), :]
            return w_op[half][1 + q // 16, pl.ds(
                pl.multiple_of(128 * (q % 16) + 8 * zero, 8), 128), :]

        def decode_unit(g, m, half, prods):
            for r0 in range(0, P0 // 4, 8):
                out = _decode(prods, r0)
                for i, j in QUAD:
                    for a, b in QUAD:
                        rings[8 * m + 4 * half + 2 * b + j][
                            g, pl.ds(P0 // 4 * (2 * a + i) + r0, 8), :] = out[2 * a + i, 2 * b + j]
                    yield [(rings[8 * m + 4 * half + 2 * b + j], (g, 0)) for b in range(2)]

        for cp in x0_copies(0) + x0_copies(1):
            cp.start()
        for m in range(3):
            start_chunk(0, m)
        x0_copies(2)[0].start()

        @pl.loop(0, NP)
        def _(p):
            we[4, pl.ds(pl.multiple_of(128 * p, 128), 128), :] = jnp.zeros((128, 128), u32)

        @pl.loop(0, P0 // 64 // LN_UNROLL)
        def _(i):
            for k in range(2):
                @pl.when(i == k * P0 // 128 // LN_UNROLL)
                def _():
                    for cp in x0_copies(k):
                        cp.wait()
            n = 16 * LN_UNROLL
            for a in range(4):
                rows = pl.ds(pl.multiple_of(P0 // 4 * a + n * i, 16), n)
                _set_rows(xg, rows, _ln(xs[rows, :].astype(f32)))
            for s in range(LN_UNROLL):
                for kt in range(2):
                    ops = _encode(SA, lambda k, a, b: xg[2 * b + kt, pl.ds(
                        P0 // 4 * a + n * i + 16 * s + k, 8, stride=2), :])
                    for p, w in enumerate(ops):
                        xe[p][pl.ds(pl.multiple_of(64 * kt + n // 2 * i + 8 * s, 8), 8), :] = w

        wait_chunk(0, (0,))

        @pl.loop(0, 16 // W_UNROLL)
        def _(i):
            list(encode_unit(0, 0, 0, [pl.multiple_of(8 * (W_UNROLL * i + k), 8)
                                       for k in range(W_UNROLL)]))

        wait_chunk(0, (1,))

        def transfers(g, g1, m, half):
            if half == 1:
                if m < 2:
                    wait_chunk(m + 1)
                else:
                    pl.when(g < 3)(functools.partial(wait_chunk, 0))
                pl.when(g < 3)(functools.partial(start_chunk, g1, m))
            elif m > 0:
                fence()
                for cp in early_copies(g) if m == 1 else [wo_copy(g)]:
                    cp.start()

        last = [we.at[4, pl.ds(128 * p, 128)] for p in range(NP)]

        @pl.loop(0, 4)
        def _(g):
            g1 = jnp.minimum(g + 1, 3)
            zero = g >> 2
            pending = decode_unit((g + 3) & 3, 2, 1, last)
            for m in range(3):
                for half in range(2):
                    nxt = (g1, 0, 0) if (m, half) == (2, 1) else (g, m + half, 1 - half)
                    side = _Side(zero, 8 * (NP - 1),
                                 (encode_unit(*nxt, range(0, 128, 8)), 7 * 16), (pending, 64))
                    prods = []
                    for p in range(NP):
                        if p == 1:
                            transfers(g, g1, m, half)
                        lhs = jnp.concatenate(
                            [xe[p][pl.ds(64 * kt, 64), :] for kt in range(2)], axis=1)
                        rhs = operand(g, m, half, p, zero)
                        for k in range(0, 64, 8) if p else ():
                            lhs = side.tie(lhs, k, 128)
                        prods.append(_dot(_unpack(lhs), _unpack(rhs)))
                    pending = decode_unit(g, m, half, prods)
            for p in range(NP):
                last[p][...] = pltpu.bitcast(prods[p], u32)

        list(decode_unit(3, 2, 1, last))

        x_copy.start()
        x0_copies(2)[0].wait()
        tokbuf[...] = _ln(xs[pl.ds(P0, UNROLL * TOK), :].astype(f32))
        _set_rows(xg, pl.ds(0, HALO), jnp.zeros((HALO, D), f32))
        _set_rows(xg, pl.ds(HALO + S, HALO), jnp.zeros((HALO, D), f32))
        _set_rows(hbuf, pl.ds(0, UNROLL * TOK), jnp.zeros((UNROLL * TOK, D), f32))
        _set_rows(useq, pl.ds(2 * TOK, 2 * TOK), jnp.zeros((2 * TOK, D), f32))
        for cp in w3_copies:
            cp.start()
        for i in range(4):
            for cp in early_copies(i):
                cp.wait()

        @pl.loop(0, 4)
        def _(j):
            for r in range(0, D // 4, 16):
                raw = {key: w1e[j, 1 + n, pl.ds(r, 16), :] for n, key in enumerate(QUAD)}
                ops = _encode1(SB, lambda k, a, b: _unzip(raw[a, b], k))
                for p in (0, 2, 3, 5, 6):
                    w1e[j, p, pl.ds(r, 16), :] = ops[p]

        for i in range(4):
            wo_copy(i).wait()

        def wrap(r):
            return jnp.where(r >= RING, r - RING, r)

        def step(s, carry, tok, side, last):
            mem, rp, ra, rw = carry
            ri = lax.broadcasted_iota(jnp.int32, (2 * MEM + SEG, 2 * L), 0)
            ci = lax.broadcasted_iota(jnp.int32, (2 * MEM + SEG, 2 * L), 1)
            key_b = ((ci >= MEM) & (ci < 2 * MEM)) | (ci >= 2 * MEM + SEG)
            same = key_b == ((ri >= MEM) & (ri < 2 * MEM))
            mask = same & ((ri < 2 * MEM) | (ri >= ci))
            fill = jnp.where(same, NEG, -jnp.inf)

            lhs = jnp.concatenate([mem, tok], axis=0).astype(bf16)
            rps = [pl.multiple_of(wrap(rp + 8 * i), 8) for i in range(3)]
            ra_ = pl.multiple_of(ra, SEG)
            rw_ = pl.multiple_of(rw, 8)

            col = s & 3
            group = jnp.maximum((s >> 2) - 1, 0)
            rb = pl.multiple_of(group * (4 * TOK), 8)

            mem_qkv = {}
            scores = {}
            o_mem = {}
            total = [None]

            def qkv(h):
                for m in range(3):
                    w = w_s[m][h]
                    r = _dot(lhs, _unpack(side.tie(w, SIDE_ROW) if h >= SIDE_AT else w))
                    for i in range(3):
                        ring[m][h][pl.ds(rps[i], 8), :] = r[8 + 8 * i:16 + 8 * i]
                    mem_qkv[m, h] = r[:MEM]

            def segment(m, pair):
                a, b = 2 * pair, 2 * pair + 1
                ma, mb = mem_qkv.pop((m, a)), mem_qkv.pop((m, b))
                xa, xb = (ring[m][h][pl.ds(ra_, SEG), :] for h in (a, b))
                if m == 0:
                    parts = ((ma, mb, xa), (xb,))
                else:
                    parts = ((ma, mb, xa, xb), (mb, ma, xb))
                return [jnp.concatenate(v, axis=0).astype(bf16) for v in parts]

            def qk(pair):
                q, k = segment(0, pair), segment(1, pair)
                for n in range(2):
                    scores[pair, n] = lax.dot_general(
                        q[n], k[n], (((1,), (1,)), ((), ())), preferred_element_type=f32)

            def pv(pair):
                v = segment(2, pair)
                for n in range(2):
                    sc = scores.pop((pair, n)) * (DH ** -0.5)
                    if n == 0:
                        sc = jnp.where(mask, sc, fill)
                    else:
                        sc = jnp.where(mask[2 * MEM:, :2 * MEM + SEG], sc,
                                       fill[2 * MEM:, :2 * MEM + SEG])
                    mx = jnp.max(sc, axis=1, keepdims=True)
                    e = jnp.exp(sc - mx)
                    den = jnp.sum(e, axis=1, keepdims=True)
                    inv = pl.reciprocal(den, approx=True)
                    inv = inv * (2.0 - den * inv)
                    o = _dot(e.astype(bf16), v[n]) * inv
                    q_r[2 * pair + n][pl.ds(ra_, SEG), :] = o[-SEG:]
                    if n == 0:
                        o_mem[2 * pair], o_mem[2 * pair + 1] = o[:MEM], o[MEM:2 * MEM]

            def wo(h):
                lo = jnp.concatenate([o_mem.pop(h), q_r[h][pl.ds(rw_, TOK), :]],
                                     axis=0).astype(bf16)
                r = _dot(lo, _unpack(wo_b[pl.ds(h * DH // 2, DH // 2), :]))
                total[0] = r if total[0] is None else total[0] + r

            npair = H // 2
            for t in range(npair + LAG_WO):
                if 0 <= t - LAG_QK < npair:
                    qk(t - LAG_QK)
                if 0 <= t - LAG_PV < npair:
                    pv(t - LAG_PV)
                if t < npair:
                    qkv(2 * t)
                    qkv(2 * t + 1)
                if 0 <= t - LAG_WO < npair:
                    wo(2 * (t - LAG_WO))
                    wo(2 * (t - LAG_WO) + 1)
            fills = [_dot(_unpack(ubuf[p]), _unpack(w1e[col, p])) for p in range(7)]
            for (a, b), v in _decode1(fills).items():
                xg[4 * b + col, pl.ds(HALO + rb + 2 * TOK * a, 2 * TOK), :] = (
                    v if last and a == b else _gelu(v))

            a = total[0]
            return (a[:MEM], wrap(rp + TOK), wrap(ra + SEG), wrap(rw + TOK)), a[MEM:]

        def late_gelu(s):
            rb = jnp.maximum((s >> 2) - 1, 0) * (4 * TOK)
            for a in range(2):
                at = (4 * a + (s & 3),
                      pl.ds(pl.multiple_of(HALO + rb + 2 * TOK * a, 8), 2 * TOK))
                xg[at] = _gelu(xg[at])
            yield [(xg, (s & 3, HALO + rb))]

        def steps(i, carry):
            n = UNROLL * TOK
            pl.when(i == 1)(x_copy.wait)

            @pl.when(i == 16 // ENC)
            def _():
                raw = we.at[pl.ds(0, NC), pl.ds(0, 4 * 512)]
                pltpu.make_async_copy(raw, raw, sems.at[SEM_W3]).wait()

            zero = i >> 5
            at = lambda r, m, k: pl.ds(pl.multiple_of(r + 16 * k * zero, 16), m)

            def norm_filler():
                prev = jnp.maximum(i - 1, 0)

                def first_norm(r, x, y):
                    lnbuf[pl.ds(r, 16), :] = y
                    return [(lnbuf, (r,))]

                def second_norm(r, x, y):
                    dst = pl.multiple_of(n * (prev & 3) + r, 8)
                    _set_rows(useq, pl.ds(dst, 16), y)
                    return [(useq, (0, dst))]

                yield from _ln_job(lambda r, m, k: _rows(hbuf, at(n * prev + r, m, k)),
                                   first_norm, n)
                yield from _ln_job(lambda r, m, k: lnbuf[at(r, m, k + 2), :],
                                   second_norm, n)
                base = (jnp.maximum((UNROLL * i >> 2) - 1, 0) & 1) * (2 * n)
                for r in range(0, n, 16):
                    for kt in range(4):
                        ops = _encode1(SA, lambda k, a, b: useq[
                            4 * b + kt, pl.ds(base + n * a + r + k, 8, stride=2), :])
                        for p, w in enumerate(ops):
                            ubuf[p, pl.ds(r // 2, 8), pl.ds(128 * kt, 128)] = w
                        if kt % 2:
                            yield [(ubuf, (0, 0))]

            def norm_tokens():
                def keep(r, x, y):
                    tokbuf[pl.ds(r, 16), :] = y
                    return [(tokbuf, (r,))]

                nxt = jnp.minimum(P0 + n * (i + 1), S - n)
                return _ln_job(lambda r, m, k: xs[at(nxt + r, m, k), :].astype(f32),
                               keep, n)

            def encode_b():
                for j in range(4):
                    raw = {(a, b): we[w2_slot(2 * a + b, j, 8 * i, 8)] for a, b in QUAD}
                    for p, w in enumerate(_encode1(SB, lambda k, a, b: _unzip(raw[a, b], k))):
                        we[w2_slot(p, j, 8 * i, 8)] = w
                    yield [(we, (NC, 8 * i))]
                for k in range(ENC):
                    j = ENC * i + k
                    grp, i0 = jnp.where(j < 16, NC + 2, (j >> 4) - 1), 8 * (j & 15)
                    slot = lambda q: (grp, pl.ds(pl.multiple_of(128 * q + i0, 8), 8))
                    raw = {(a, b): we[slot(4 * b + a)] for a in range(4) for b in range(4)}
                    get = functools.cache(lambda k, a, b: _unzip(raw[a, b], k))
                    for p in ORDER_B:
                        for r, w in enumerate(_encode7(SB, p, get)):
                            we[slot(7 * p + r)] = w
                        yield [(we, (grp, i0))]

            jobs = [[(norm_filler(), 4 * n // 16), (late_gelu(jnp.maximum(UNROLL * i - 1, 0)), 1)],
                    [(encode_b(), 4 + 7 * ENC), (norm_tokens(), n // 16)]]
            for k in range(UNROLL):
                s = i * UNROLL + k
                carry, o = step(s, carry, tokbuf[pl.ds(k * TOK, TOK), :],
                                _Side(zero, SIDE_N, *jobs[k]), k == UNROLL - 1)
                lo = k * TOK // 16 * 16
                xv = xs[pl.ds(pl.multiple_of(n * i + lo, 16), 32), :].astype(f32)
                _set_rows(hbuf, pl.ds(pl.multiple_of(TOK * s, 8), TOK),
                          xv[k * TOK - lo:(k + 1) * TOK - lo] + o)
            return carry

        carry = (mem0_ref[...].astype(f32), jnp.int32(P0), jnp.int32(0), jnp.int32(0))
        carry = lax.fori_loop(0, NSEG // UNROLL, steps, carry)
        list(late_gelu(jnp.int32(NSEG - 1)))
        return carry[1] >> 16

    zero = pl.run_scoped(
        block_a,
        *[pltpu.VMEM((H, D // 2, DH), u32)] * 3,
        pltpu.VMEM((7, TOK, D // 2), u32),
        pltpu.VMEM((D // 128, 8 * TOK, 128), f32),
        pltpu.VMEM((UNROLL * TOK, D), f32),
        pltpu.VMEM((UNROLL * TOK, D), f32),
        *[pltpu.VMEM((H // 8, RING, DH), f32)] * 16,
    )

    def tail(w4e, ye, ybuf, *bufs):
        woe, pool = bufs[:3], bufs[3:]
        w4_copies = [
            pltpu.make_async_copy(w4_hbm.bitcast(u32).at[pl.ds(1, NC - 1), a, :, pl.ds(b * C4, C4)],
                                  w4e.at[4 * a + b], sems.at[SEM_W4])
            for a in range(4) for b in range(4)]
        for cp in w4_copies:
            cp.start()
        done = TOK * NSEG
        first = 4 * TOK * (NSEG // 4 - 1)

        def later(rows, n):
            return pl.ds(pl.multiple_of(rows + 8 * zero, 8), n)

        def run(dots, ties, start, *jobs):
            side = _Side(zero, (len(dots) - max(start, 0)) * len(ties), *jobs)
            prods = []
            for load in dots:
                if len(prods) == start:
                    fence()
                lhs, rhs = load()
                for r0, c0 in ties if len(prods) >= start else ():
                    lhs = side.tie(lhs, r0, c0)
                prods.append(_dot(_unpack(lhs), _unpack(rhs)))
            return prods

        hk, hn, hm = H * DH // 4, D // 2, P0 // 2

        def wo_op(p, j):
            if p == 3:
                return pool[j], 0, 0
            if p in (1, 4):
                return wo_b, hk * (p // 4), hn * (p // 4) + C4 * j
            return woe[{0: 0, 2: 1, 5: 2, 6: 0}[p]], 0, C4 * j

        def encode_wo(ps):
            for i0 in range(0, hk, 8):
                for j in range(2):
                    get = functools.cache(lambda k, a, b: _unzip(wo_b[
                        later(hk * a + i0 + 8 * ps[0] * zero, 8), pl.ds(hn * b + C4 * j, C4)], k))
                    ops = [_zip(*[_combine(functools.partial(get, k), SB[p]) for k in range(2)])
                           for p in ps]
                    for p, w in zip(ps, ops):
                        ref, r0, c0 = wo_op(p, j)
                        ref[pl.ds(r0 + i0, 8), pl.ds(c0, C4)] = w
                    yield [(wo_op(p, j)[0], (0,)) for p in ps]

        def encode_o(n):
            for kt in range(H // 2):
                for s in range(hm // 16):
                    pool[n][pl.ds(hm // 2 * (kt // 2) + 8 * s, 8), pl.ds(kt % 2 * 128, 128)] = (
                        _zip(*[_combine(
                            lambda a, b: q_r[H // 2 * b + kt][pl.ds(
                                (done + hm * a + 16 * s) % RING + k + n * zero, 8, stride=2), :],
                            SA[ORDER_B[n]]) for k in range(2)]))
                    if s % 4 == 3:
                        yield [(pool[n], (0,))]

        def wo_dots(n):
            def load(j, i):
                ref, r0, c0 = wo_op(ORDER_B[n], j)
                lhs = [pool[n][later(hm // 2 * c + hm // 4 * i + 8 * j * zero, hm // 4), :]
                       for c in range(8)]
                return (jnp.concatenate(lhs, axis=1),
                        ref[later(r0 + 8 * i * zero, hk), pl.ds(c0, C4)])
            return [functools.partial(load, j, i) for j, i in QUAD]

        def decode_wo(n, prods):
            for (j, i), v in zip(QUAD, prods):
                for r in range(0, hm // 2, 16):
                    for (a, b), sign in SC[ORDER_B[n]]:
                        fresh = all(key != (a, b) for q in ORDER_B[:n] for key, _ in SC[q])
                        row = done + hm * a + hm // 2 * i + r
                        for k in range(2):
                            c = 4 * b + 2 * j + k
                            old = (xs[pl.ds(row, 16), pl.ds(128 * c, 128)].astype(f32) if fresh
                                   else hbuf[c, later(row + 8 * n * zero, 16), :])
                            new = v[r:r + 16, 128 * k:128 * (k + 1)]
                            hbuf[c, pl.ds(row, 16), :] = old + new if sign > 0 else old - new
                    yield [(hbuf, (0, 0))]

        hsb = wo_b

        def norm_in():
            def first_norm(r, x, y):
                woe[2][pl.ds(r, 16), :] = pltpu.bitcast(y[:, :hn], u32)
                woe[2][pl.ds(P0 + r, 16), :] = pltpu.bitcast(y[:, hn:], u32)
                return [(woe[2], (r,))]

            def second_norm(r, x, y):
                _set_rows(xg, pl.ds(HALO + done + r, 16), y)
                return [(xg, (0, HALO + done))]

            yield from _ln_job(
                lambda r, n, k: _rows(hbuf, later(done + r + 8 * (7 + k) * zero, n)),
                first_norm, P0, NORM_ROWS, *stats[:2], zero)
            yield from _ln_job(
                lambda r, n, k: pltpu.bitcast(jnp.concatenate(
                    [woe[2][later(r0 + r + 8 * k * zero, n), :] for r0 in (0, P0)], axis=1), f32),
                second_norm, P0, NORM_ROWS, *stats[2:], zero)

        def encode_rows(buf, r0, n, shift=(0, 0, 0, 0)):
            for r in range(0, n // 2, 16):
                for kt in range(4):
                    ops = _encode1(SA, lambda k, a, b: xg[4 * b + kt, pl.ds(
                        HALO + r0 + n // 2 * a + r + k + shift[2 * b + kt // 2],
                        8, stride=2), :])
                    for p, w in enumerate(ops):
                        buf[pl.ds(128 * p + 64 * (kt // 2) + r // 2, 8),
                            pl.ds(128 * (kt % 2), 128)] = w
                    yield [(buf, (0,))]

        def encode_g(i):
            return encode_rows(pool[i - 1], i * RB, RB, SHIFT)

        def mixer(buf, n, weights, store, start, pending, *jobs):
            def decode(j, prods):
                for r in range(0, n // 2, 8):
                    for (a, b), v in _decode1([m[r:r + 8] for m in prods]).items():
                        seen = store(n // 2 * a + r, 4 * b + j, v)
                    yield seen

            for j in range(4):
                dots = [lambda p=p: (
                    jnp.concatenate([buf[later(128 * p + 64 * k + 8 * j * zero, n // 4), :]
                                     for k in range(2)], axis=1),
                    weights(p, j)) for p in range(7)]
                prods = run(dots, [(r, TIE_C) for r in range(0, n // 4, 8)],
                            -1 if j else start, pending,
                            *[(job, count // 4) for job, count in jobs])
                pending = (decode(j, prods), n // 16)
            return pending

        def mixer_in(buf, r0, n, *args):
            def store(r, c, v):
                xg[c, pl.ds(HALO + r0 + r, 8), :] = _gelu(v)
                return [(xg, (0, HALO + r0))]

            return mixer(buf, n, lambda p, j: w1e[j, p, later(r0 * zero, D // 4), :],
                         store, *args)

        def mixer_out(i, *args):
            def store(r, c, v):
                hsb[pl.ds(i * RB + r, 8), pl.ds(128 * c, 128)] = pltpu.bitcast(v, u32)
                return [(hsb, (i * RB,))]

            return mixer(pool[i - 1], RB, lambda p, j: we[w2_slot(p, j, 8 * (i + 1) * zero)],
                         store, 0, *args)

        def encode_w4():
            for c in range(NC - 1):
                for i0 in range(0, 64, 8):
                    for j in range(2):
                        at = (c, pl.ds(i0, 8), pl.ds(128 * j, 128))
                        raw = {(a, b): w4e[(4 * a + b,) + at]
                               for a in range(4) for b in range(4)}
                        get = functools.cache(lambda k, a, b: _unzip(raw[a, b], k))
                        for p in ORDER_B:
                            for r, w in enumerate(_encode7(SB, p, get)):
                                w4e[(7 * p + r,) + at] = w
                            yield [(w4e, (0, c, i0))]

        def mixer_post(r0, zero, group):
            def first_norm(r, hv, y):
                rows = pl.ds(_mult(r0 + r, 8), 16)
                x1 = y + pltpu.bitcast(hsb[rows, :], f32)
                _set_rows(xg, rows, hv + x1)
                _set_rows(ybuf, pl.ds(r, 16), x1)
                return [(ybuf, (0, 0)), (xg, (0, r0))]

            def second_norm(r, x1, y):
                _set_rows(hbuf, pl.ds(_mult(r0 + r, 8), 16), y)
                return [(hbuf, (0, r0))]

            at = lambda r, n, k: pl.ds(pl.multiple_of(r + 8 * k * zero, 8), n)
            yield from _ln_job(lambda r, n, k: _rows(hbuf, at(r0 + r, n, k)),
                               first_norm, RB, group, *stats[:2], zero)
            yield from _ln_job(lambda r, n, k: _rows(ybuf, at(r, n, k + 1)),
                               second_norm, RB, group, *stats[2:], zero)
            for s in range(4):
                for kt in range(2):
                    get = functools.cache(lambda k, a, b: hbuf[2 * b + kt, pl.ds(
                        r0 + R4 * a + 4 * k + 2 * (s % 2) + s // 2, 8, stride=8), :])
                    for p in ORDER_A:
                        for r, w in enumerate(_encode7(SA, p, get)):
                            ye[7 * p + r, pl.ds(8 * s, 8), pl.ds(128 * kt, 128)] = w
                        if p in POST_P:
                            yield [(ye, (0, 8 * s))]

        def out_copies(i):
            rows = pl.ds(_mult(i * RB, RB), RB)
            return [pltpu.make_async_copy(
                woe[b].bitcast(bf16).at[rows], out_hbm.at[rows, pl.ds(hn * b, hn)],
                sems.at[SEM_OUT + 2 * i + b]) for b in range(2)]

        n_g, n_o = RB // 8, H // 2 * hm // 64
        n_post = RB // 8 + 8 * len(POST_P)
        wo_ties = [(r0, c0) for c0 in range(TIE_C, 2 * D, 512) for r0 in range(0, 64, 8)]
        w4_job = encode_w4()
        wo_jobs = [encode_wo(ps) for ps in ((0,), (2, 5), (3, 6))]

        _set_rows(xg, pl.ds(HALO + first, done - first),
                  _ln(_ln(_rows(hbuf, pl.ds(first, done - first)))))
        list(encode_rows(pool[7], first, done - first))
        pending = mixer_in(pool[7], first, done - first, -1, (None, 0), (encode_o(0), n_o))
        for n in range(7):
            jobs = [(encode_o(n + 1), n_o) if n < 6 else (encode_g(0), n_g), pending]
            if n < 5:
                jobs.append((wo_jobs[(n + 1) // 2], hk // 8 if n else hk // 4))
            if n == W4_AT:
                for cp in w4_copies:
                    cp.wait()
            if n >= W4_AT:
                jobs.append((w4_job, 7 * W4_WO))
            prods = run(wo_dots(n), wo_ties, 0, *jobs)
            pending = (decode_wo(n, prods), hm // 8)
        norm = norm_in()
        for i in range(5):
            jobs = [(w4_job, 7 * W4_SPLIT[i])]
            jobs.append((encode_g(i + 1) if i < 4 else encode_rows(pool[7], done, RB), n_g))
            if i > 0:
                jobs.append((norm, P0 // NORM_ROWS + P0 // 32))
            pending = mixer_out(i, pending, *jobs)
        post = (mixer_post(0, zero, NORM_ROWS), (n_post + 4 * RB // NORM_ROWS) // 2)
        pending = mixer_in(pool[7], done, RB, IN_FENCE[0], pending, post,
                           (encode_rows(pool[0], done + RB, RB), n_g))
        pending = mixer_in(pool[0], done + RB, RB, IN_FENCE[1], pending, post,
                           (encode_g(5), n_g))
        for i in range(5, 8):
            jobs = [(w4_job, 7 * W4_SPLIT[i])]
            if i < 7:
                jobs.append((encode_g(i + 1), n_g))
            pending = mixer_out(i, pending, *jobs)
        list(pending[0])

        def mlp_block(i, carry):
            te = []
            for c in range(NC):
                ops = []
                for r0 in range(0, R4, UP_ROWS):
                    prods = [_dot(_unpack(ye[p, pl.ds(r0 // 2, UP_ROWS // 2), :]), _unpack(
                        we[c, pl.ds(pl.multiple_of(128 * p + r0 * (i >> 3), 8), 128), :]))
                        for p in range(NP)]
                    for s in range(UP_ROWS // 16):
                        act = [{key: _gelu2(v) for key, v in _decode(
                            prods, 32 * (s // 2) + 16 * k + 8 * (s % 2)).items()}
                            for k in range(2)]
                        ops.append(_encode(SA, lambda k, a, b: act[k][a, b]))
                te.append([jnp.concatenate([o[p] for o in ops], axis=0) for p in range(NP)])

            def down(p, lo, hi, tie=lambda w: w):
                lhs = jnp.concatenate([tie(te[c][p]) if c in POST_C else te[c][p]
                                       for c in range(lo, hi)], axis=1)
                rhs = [w4e[p, c - 1] if c else jnp.concatenate(
                    [we[NC + 2, pl.ds(128 * p + 64 * k, 64), :] for k in range(2)], axis=1)
                    for c in range(lo, hi)]
                rhs = jnp.concatenate(rhs, axis=0)
                return _dot(_unpack(lhs), _unpack(rhs))

            prods = [down(p, 0, KSPLIT) for p in range(NSPLIT)]
            prods = [m + down(p, KSPLIT, NC) for p, m in enumerate(prods)]
            out = {}

            def finish(qa, qb):
                for a, b in ((2 * qa + n // 2, 2 * qb + n % 2) for n in range(4)):
                    for r in range(0, R4, 16):
                        row = i * RB + R4 * a + r
                        for j in range(2):
                            woe[qb][pl.ds(pl.multiple_of(row // 2, 8), 8),
                                    pl.ds(C4 * (b % 2) + 128 * j, 128)] = _zip(*[
                                        0.5 * out[a, b][32 * k + r // 2:32 * k + r // 2 + 8,
                                                  128 * j:128 * (j + 1)]
                                        + xg[2 * b + j, pl.ds(row + k, 8, stride=2), :]
                                        for k in range(2)])
                        yield [(woe[qb], (i * (RB // 2),))]

            side = _Side(i >> 3, POST_N * len(POST_C),
                         (mixer_post(((i + 1) & 7) * RB, i >> 3, 0), n_post))
            for p in range(7):
                done_quad = {4: (1, 0), 5: (0, 1), 6: (1, 1)}.get(p)
                store = _Side(i >> 3, 16, *([(finish(*done_quad), 16)] if done_quad else []))
                for q in range(len(prods), 7 * p + 7):
                    side.after(hbuf, prods[q - POST_LAG])
                    prods.append(down(q, 0, NC, side.tie if q % 7 == 0 else
                                      lambda w: store.tie(side.tie(w))))
                _decode7(p, prods[7 * p:7 * p + 7], out)
            list(finish(0, 0))
            for cp in out_copies(i):
                cp.start()
            return carry

        lax.fori_loop(0, S // RB, mlp_block, 0)
        for i in range(S // RB):
            for cp in out_copies(i):
                cp.wait()

    pl.run_scoped(
        tail,
        pltpu.VMEM((NP, NC - 1, 64, C4), u32),
        pltpu.VMEM((NP, R4 // 2, C4), u32),
        pltpu.VMEM((D // 128, RB, 128), f32),
        *[pltpu.VMEM((H * DH // 4, D // 2), u32)] * 3,
        *[pltpu.VMEM((D, C4), u32)] * 8,
    )


@jax.jit
def pallas_sequential_preLN__memory_aug_recurrent_mem_tr__mixer_s_mlp__prompt_kernel(
    A_x: jax.Array,
    A_mem0: jax.Array,
    A_Wq: jax.Array,
    A_Wk: jax.Array,
    A_Wv: jax.Array,
    A_Wo: jax.Array,
    A_seg_len: jax.Array,
    B_x: jax.Array,
    B_w1: jax.Array,
    B_w2: jax.Array,
    B_w3: jax.Array,
    B_w4: jax.Array,
):
    del A_seg_len, B_x
    hbm = pl.BlockSpec(memory_space=pl.ANY)
    vmem = pl.BlockSpec(memory_space=pltpu.VMEM)
    scratch = [
        pltpu.VMEM((H * DH // 2, D), u32),
        pltpu.VMEM((S, D), bf16),
        pltpu.VMEM((D // 128, S + 8, 128), f32),
        pltpu.VMEM((D // 128, S + 2 * HALO, 128), f32),
        pltpu.VMEM((4, 7, D // 4, 128), u32),
        pltpu.VMEM((NC + 3, NP * 128, 128), u32),
        pltpu.SemaphoreType.DMA((NSEM,)),
        pltpu.SemaphoreType.REGULAR,
    ] + [pltpu.VMEM((P0, 128), f32)] * 4 + [pltpu.VMEM((H // 8, RING, DH), f32)] * 8
    out = pl.pallas_call(
        _kernel,
        out_shape=jax.ShapeDtypeStruct((S, D), A_x.dtype),
        in_specs=[hbm, vmem] + [hbm] * 8,
        out_specs=hbm,
        scratch_shapes=scratch,
        compiler_params=pltpu.CompilerParams(vmem_limit_bytes=VMEM_LIMIT),
    )(A_x.reshape(S, D), A_mem0.reshape(MEM, D),
      A_Wq.reshape(D // 2, 2 * H, DH), A_Wk.reshape(D // 2, 2 * H, DH),
      A_Wv.reshape(D // 2, 2 * H, DH),
      A_Wo.reshape(H * DH, D), B_w1, B_w2, B_w3, B_w4.reshape(NC, 4, 128, D))
    return out.reshape(A_x.shape)
```
